```python
import jax
import jax.numpy as jnp

def _softmax(x, axis=-1):
    return jax.nn.softmax(x, axis=axis)

def _gelu(x):
    return jax.nn.gelu(x, approximate=True)

def _silu(x):
    return jax.nn.silu(x)

def _sigmoid(x):
    return jax.nn.sigmoid(x)

def _layernorm(x, axis=-1, eps=1e-05):
    m = jnp.mean(x, axis=axis, keepdims=True)
    v = jnp.var(x, axis=axis, keepdims=True)
    return (x - m) / jnp.sqrt(v + eps)

def _scatter_add(tgt, idx, src, axis=0):
    return tgt.at[idx].add(src)

def _segment_sum(src, seg, n):
    return jax.ops.segment_sum(src, seg, n)

class _Rng:

    def __init__(self, key):
        self._k = key

    def _next(self):
        self._k, sub = jax.random.split(self._k)
        return sub

    def normal(self, shape):
        return jax.random.normal(self._next(), shape, dtype=jnp.bfloat16)

    def randint(self, lo, hi, shape):
        return jax.random.randint(self._next(), shape, lo, hi, dtype=jnp.int32)

    def uniform(self, shape, lo=0.0, hi=1.0):
        return jax.random.uniform(self._next(), shape, jnp.bfloat16, lo, hi)

    def permutation(self, n):
        return jax.random.permutation(self._next(), n)
kernel_name = 'parallel_sum__memory_aug_infini_attn__moe_arch_mod__prompt'

def setup_inputs():
    _rng = _Rng(jax.random.key(int.from_bytes(__import__("os").urandom(4), "little")))
    _w = lambda a: (lambda t: t.astype(jnp.bfloat16) if jnp.issubdtype(t.dtype, jnp.floating) else t)(jnp.asarray(a))

    def _A_setup():
        B, S, D, H = (1, 2048, 576, 32)
        N = 4
        L = max(1, S // N)
        sc = D ** (-0.5)
        return {'x': _w((lambda *s: _rng.normal(s) * 0.05)(B, N * L, D)), 'wq': _w((lambda *s: _rng.normal(s) * 0.05)(D, D) * sc), 'wk': _w((lambda *s: _rng.normal(s) * 0.05)(D, D) * sc), 'wv': _w((lambda *s: _rng.normal(s) * 0.05)(D, D) * sc), 'wo': _w((lambda *s: _rng.normal(s) * 0.05)(D, D) * sc), 'beta': _w((lambda *s: _rng.normal(s) * 0.05)(H))}
    _A_in = _A_setup()

    def _B_setup():
        B, S, D, F, C = (1, 2048, 576, 4608, 2)
        return {'x': _w((lambda *s: _rng.normal(s) * 0.05)(B, S, D)), 'w_r': _w((lambda *s: _rng.normal(s) * 0.05)(D)), 'w_gate': _w((lambda *s: _rng.normal(s) * 0.05)(D, F)), 'w_up': _w((lambda *s: _rng.normal(s) * 0.05)(D, F)), 'w_down': _w((lambda *s: _rng.normal(s) * 0.05)(F, D))}
    _B_in = _B_setup()
    return {'A_x': _A_in['x'], 'A_wq': _A_in['wq'], 'A_wk': _A_in['wk'], 'A_wv': _A_in['wv'], 'A_wo': _A_in['wo'], 'A_beta': _A_in['beta'], 'B_x': _B_in['x'], 'B_w_r': _B_in['w_r'], 'B_w_gate': _B_in['w_gate'], 'B_w_up': _B_in['w_up'], 'B_w_down': _B_in['w_down']}

def reference(A_x, A_wq, A_wk, A_wv, A_wo, A_beta, B_x, B_w_r, B_w_gate, B_w_up, B_w_down):

    def _A_ref(x, wq, wk, wv, wo, beta):
        B, S, D = x.shape
        H = 32
        Dh = D // H
        N = 4
        L = S // N
        q = (lambda x, *d: x.transpose(*d))((x @ wq).reshape(B, S, H, Dh), 0, 2, 1, 3).reshape(B, H, N, L, Dh)
        k = (lambda x, *d: x.transpose(*d))((x @ wk).reshape(B, S, H, Dh), 0, 2, 1, 3).reshape(B, H, N, L, Dh)
        v = (lambda x, *d: x.transpose(*d))((x @ wv).reshape(B, S, H, Dh), 0, 2, 1, 3).reshape(B, H, N, L, Dh)
        phi = lambda t: jnp.where(t > 0, t + 1.0, jnp.exp(t))
        scale = Dh ** (-0.5)
        ar = jnp.arange(L)
        mask = (lambda x, dt: x.astype(dt))(ar[:, None] < ar[None, :], x.dtype) * -1000000000.0
        g = _sigmoid(beta).reshape(1, H, 1, 1)
        M = jnp.einsum('bhd,bhe->bhde', q[:, :, 0, 0, :] * 0.0, q[:, :, 0, 0, :] * 0.0)
        z = q[:, :, 0, 0, :] * 0.0
        outs = []
        for s in range(N):
            qs, ks, vs = (q[:, :, s].copy(), k[:, :, s].copy(), v[:, :, s].copy())
            logits = jnp.einsum('bhqd,bhkd->bhqk', qs, ks) * scale + mask
            p = _softmax(logits, axis=-1)
            a_dot = jnp.einsum('bhqk,bhkd->bhqd', p, vs)
            pq = phi(qs)
            num = jnp.einsum('bhld,bhde->bhle', pq, M)
            den = jnp.einsum('bhld,bhd->bhl', pq, z)[..., None] + 1e-06
            a_mem = num / den
            o = g * a_mem + (1.0 - g) * a_dot
            outs.append(o)
            pk = phi(ks)
            M = M + jnp.einsum('bhld,bhle->bhde', pk, vs)
            z = z + jnp.einsum('bhld->bhd', pk)
        o = (lambda x, *d: x.transpose(*d))(jnp.stack(outs, 2).reshape(B, H, S, Dh), 0, 2, 1, 3).reshape(B, S, D)
        return o @ wo

    def _B_ref(x, w_r, w_gate, w_up, w_down):
        B, S, D = x.shape
        C = 2
        r = x @ w_r
        idx = jnp.argsort(-r, axis=-1)[:, :C]
        idx_e = jnp.repeat(idx.reshape(B, C, 1), D, axis=2)
        x_sel = jnp.take_along_axis(x, idx_e, axis=1)
        g = _silu(x_sel @ w_gate)
        u = x_sel @ w_up
        y = g * u @ w_down
        r_sel = _sigmoid(jnp.take_along_axis(r, idx, axis=1))
        y = y * r_sel.reshape(B, C, 1)
        b_off = (jnp.arange(B) * S).reshape(B, 1)
        flat_idx = (idx + b_off).reshape(B * C)
        zero = (x * 0.0).reshape(B * S, D)
        upd = _scatter_add(zero, flat_idx, y.reshape(B * C, D), axis=0)
        return x + upd.reshape(B, S, D)
    x = A_x
    xn = _layernorm(x, axis=-1)
    return x + _A_ref(xn, A_wq, A_wk, A_wv, A_wo, A_beta) + _B_ref(xn, B_w_r, B_w_gate, B_w_up, B_w_down)
```

```python
import jax
import jax.numpy as jnp
import jax.experimental.pallas as pl
import jax.experimental.pallas.tpu as pltpu

S, D, H, DH, NSEG, L, F = 2048, 576, 32, 18, 4, 512, 4608
DP = 640
G = 4 * DH
NG = H // 4
T = 128
LOG2E = 1.4426950408889634
QSCALE = DH ** -0.5 * LOG2E
NEG = -1e30

f32, bf16 = jnp.float32, jnp.bfloat16
NT = (((1,), (1,)), ((), ()))


def _dot(a, b):
    return jnp.dot(a, b, preferred_element_type=f32)


def _dot_nt(a, b):
    return jax.lax.dot_general(a, b, NT, preferred_element_type=f32)


def _rnd(a):
    return a.astype(bf16).astype(f32)


def _iota(shape, axis):
    return jax.lax.broadcasted_iota(jnp.int32, shape, axis)


def _phi(t):
    return jnp.where(t > 0, t + 1.0, jnp.exp(t))


def _head_of(i):
    return ((i >= DH).astype(jnp.int32) + (i >= 2 * DH).astype(jnp.int32)
            + (i >= 3 * DH).astype(jnp.int32) + (i >= 4 * DH).astype(jnp.int32))


def _kernel(x_hbm, wq_hbm, wk_hbm, wv_hbm, wo_hbm, beta_ref, wr_ref, wg_hbm, wu_hbm,
            wd_hbm, o_hbm,
            x_v, w_v, wg_v, wu_v, wd_v, wt, wrt, xn_v, base, qm, vl, kn, ot, mst, gcol,
            r_v, o_v, sem, osem):
    x_cp = [pltpu.make_async_copy(x_hbm.at[:, pl.ds(s * L, L)], x_v.at[s], sem.at[s])
            for s in range(NSEG)]
    w_cp = [pltpu.make_async_copy(w, w_v.at[i], sem.at[4 + i])
            for i, w in enumerate((wq_hbm, wk_hbm, wv_hbm, wo_hbm))]
    f_cp = [pltpu.make_async_copy(a, b, sem.at[8 + i])
            for i, (a, b) in enumerate(((wg_hbm, wg_v), (wu_hbm, wu_v), (wd_hbm, wd_v)))]
    o_cp = [pltpu.make_async_copy(o_v.at[s], o_hbm.at[:, pl.ds(s * L, L)], osem.at[s])
            for s in range(NSEG)]

    x_cp[0].start()
    for c in w_cp[:3]:
        c.start()
    for c in x_cp[1:]:
        c.start()
    w_cp[3].start()

    gate = jax.nn.sigmoid(beta_ref[...].astype(f32))
    row = _iota((D, H), 0)
    col = _iota((D, H), 1) * DH
    gsel = jnp.where((row >= col) & (row < col + DH), gate, 0.0)
    gcol[...] = jnp.broadcast_to(jnp.sum(gsel, axis=1, keepdims=True), (D, T))
    wr = jnp.concatenate([wr_ref[...].astype(f32).reshape(1, D), jnp.zeros((1, DP - D), f32)], axis=1)
    wrt[...] = jnp.broadcast_to(wr, (16, DP)).astype(bf16)
    mst[...] = jnp.zeros(mst.shape, f32)

    def transpose_w(i):
        w = jnp.concatenate([w_v[i], jnp.zeros((DP - D, D), bf16)], axis=0)
        wt[i] = w.T

    def layernorm(s):
        eps = _rnd(jnp.full((1, T), 1e-5, f32))
        for c in range(L // T):
            x = x_v[s, :, c * T:(c + 1) * T].astype(f32)
            mean = jnp.sum(x, axis=0, keepdims=True) * (1.0 / D)
            xc = x - mean
            var = jnp.sum(xc * xc, axis=0, keepdims=True) * (1.0 / D)
            sd = _rnd(jnp.sqrt(_rnd(_rnd(var) + eps)))
            xn = (_rnd(x - _rnd(mean)) * (1.0 / sd)).astype(bf16)
            xn_v[s * (L // T) + c] = jnp.concatenate([xn, jnp.zeros((DP - D, T), bf16)], axis=0)
            base[s * (L // T) + c] = x + xn.astype(f32)

    def project(s):
        xs = jnp.concatenate([xn_v[s * (L // T) + c] for c in range(L // T)], axis=1)
        r_v[s] = _rnd(_dot(wrt[...], xs)[:8])
        r8 = _iota((8, L), 0)
        ones8 = jnp.ones((8, L), f32)
        zpad = jnp.zeros((T - G, L), f32)
        mrow = _iota((G + 8, T), 0)
        mkeep = jnp.where(mrow < G, _head_of(mrow), mrow - G) == _head_of(_iota((G + 8, T), 1))
        for p in range(NG // 2):
            rows = pl.ds(p * 2 * G, 2 * G)
            q2 = _dot(wt[0, rows, :], xs)
            k2 = _dot(wt[1, rows, :], xs)
            v2 = _dot(wt[2, rows, :], xs)
            for e in range(2):
                g = 2 * p + e
                q, k, v = (a[e * G:(e + 1) * G] for a in (q2, k2, v2))
                qs = q * QSCALE
                vls = []
                for h in range(4):
                    lo = 16 * h
                    a0, a1, a2 = qs[lo:lo + 8], qs[lo + 8:lo + 16], qs[lo + 16:lo + 24]
                    if h > 0:
                        a0 = jnp.where(r8 >= 2 * h, a0, 0.0)
                    if h < 3:
                        a2 = jnp.where(r8 < 2 * h + 2, a2, 0.0)
                    qm[s, 4 * g + h] = jnp.concatenate(
                        [a0, a1, a2, jnp.zeros((8, L), f32)], axis=0).astype(bf16)
                    vh = jnp.concatenate([v[lo:lo + 24], ones8], axis=0).astype(bf16)
                    vl[s, 4 * g + h] = vh
                    vls.append(vh)
                kn[s, g] = jnp.concatenate([k, zpad], axis=0).astype(bf16).T
                state = mst[g]
                pq = jnp.concatenate([_phi(q), zpad], axis=0).astype(bf16)
                nd = _dot(jnp.where(mkeep, state, 0.0).astype(bf16), pq)
                inv = 1.0 / (nd[G:] + 1e-6)
                ib = [jnp.broadcast_to(inv[h:h + 1], (8, L)) for h in range(4)]
                iv = jnp.concatenate(
                    [ib[0], ib[0], jnp.where(r8 < 2, ib[0], ib[1]), ib[1],
                     jnp.where(r8 < 4, ib[1], ib[2]), ib[2],
                     jnp.where(r8 < 6, ib[2], ib[3]), ib[3], ib[3]], axis=0)
                gg = gcol[g * G:(g + 1) * G, :]
                ot[s, g * G:(g + 1) * G, :] = nd[:G] * iv * jnp.concatenate([gg] * (L // T), axis=1)
                pk = jnp.concatenate([_phi(k), zpad], axis=0).astype(bf16)
                v80 = jnp.concatenate([vls[0][:16], vls[1][:16], vls[2][:16], vls[3]], axis=0)
                mst[g] = state + _dot_nt(v80, pk)

    def attention(s):
        keep = _iota((T, T), 0) <= _iota((T, T), 1)
        r8 = _iota((8, T), 0)
        units = [(g, i, j) for g in range(NG) for i in range(L // T) for j in range(i + 1)]
        run = {}

        def scores(g, i, j):
            w = []
            for h in range(4):
                parts = [qm[s, 4 * g + h, :, i * T:(i + 1) * T]]
                if h > 0:
                    parts.insert(0, jnp.zeros((16 * h, T), bf16))
                parts.append(jnp.zeros((T - 32 - 16 * h, T), bf16))
                w.append(jnp.concatenate(parts, axis=0))
            st = _dot(kn[s, g, j * T:(j + 1) * T, :], jnp.concatenate(w, axis=1))
            ps, alphas = [], []
            for h in range(4):
                sh = st[:, h * T:(h + 1) * T]
                if i == j:
                    sh = jnp.where(keep, sh, NEG)
                m = jnp.max(sh, axis=0, keepdims=True)
                if j > 0:
                    m = jnp.maximum(m, run[h])
                    alphas.append(jnp.exp2(run[h] - m))
                run[h] = m
                ps.append(jnp.exp2(sh - m).astype(bf16))
            return ps, alphas

        def values(g, i, j, ps, alphas, acc):
            new = [_dot(vl[s, 4 * g + h, :, j * T:(j + 1) * T], ps[h]) for h in range(4)]
            if j > 0:
                new = [a * al + b for a, al, b in zip(acc, alphas, new)]
            if j < i:
                return new
            o = []
            for h in range(4):
                inv = 1.0 / new[h][24:32]
                o.append([new[h][8 * c:8 * c + 8] * inv for c in range(3)])
            a_dot = jnp.concatenate(
                [o[0][0], o[0][1], jnp.where(r8 < 2, o[0][2], o[1][0]), o[1][1],
                 jnp.where(r8 < 4, o[1][2], o[2][0]), o[2][1],
                 jnp.where(r8 < 6, o[2][2], o[3][0]), o[3][1], o[3][2]], axis=0)
            dst = (s, slice(g * G, (g + 1) * G), slice(i * T, (i + 1) * T))
            ot[dst] = ot[dst] + (1.0 - gcol[g * G:(g + 1) * G, :]) * a_dot
            return None

        lag, pend, acc = 2, {}, None
        for t in range(len(units) + lag):
            if t < len(units):
                pend[t] = scores(*units[t])
            if t >= lag:
                acc = values(*units[t - lag], *pend.pop(t - lag), acc)

    def out_proj(s):
        o = jnp.concatenate([ot[s], jnp.zeros((DP - D, L), f32)], axis=0).astype(bf16)
        a = _dot(wt[3], o)
        for c in range(L // T):
            o_v[s, :, c * T:(c + 1) * T] = (
                base[s * (L // T) + c] + a[:, c * T:(c + 1) * T]).astype(bf16)

    def routed_ffn():
        r = r_v[...]
        idx = _iota(r.shape, 0) * L + _iota(r.shape, 2)
        m1 = jnp.max(r)
        i1 = jnp.minimum(jnp.min(jnp.where(r == m1, idx, S)), S - 1)
        r = jnp.where(idx == i1, -jnp.inf, r)
        m2 = jnp.max(r)
        i2 = jnp.minimum(jnp.min(jnp.where((r == m2) & (idx != i1), idx, S)), S - 1)
        picks = ((i1, m1), (i2, m2))
        xsel = jnp.zeros((16, D), f32)
        for n, (i, _) in enumerate(picks):
            hot = (_iota((16, T), 0) == n) & (_iota((16, T), 1) == (i & (T - 1)))
            xsel = xsel + _dot_nt(hot.astype(f32).astype(bf16), xn_v[i >> 7, 0:D, :])
        xsel = xsel.astype(bf16)
        for c in f_cp:
            c.wait()
        gt = _dot(xsel, wg_v[...])
        up = _dot(xsel, wu_v[...])
        y = _dot_nt((gt * jax.nn.sigmoid(gt) * up).astype(bf16), wd_v[...])
        lane = _iota((D, T), 1)
        for n, (i, m) in enumerate(picks):
            yn = y[n:n + 1] * jax.nn.sigmoid(jnp.full((1, D), m, f32))
            yn = jnp.concatenate([yn, jnp.zeros((1, DP - D), f32)], axis=1)
            col = jnp.broadcast_to(yn, (T, DP)).T[0:D]
            base[i >> 7] = base[i >> 7] + jnp.where(lane == (i & (T - 1)), col, 0.0)

    x_cp[0].wait()
    layernorm(0)
    for i in range(3):
        w_cp[i].wait()
        transpose_w(i)
    for c in f_cp:
        c.start()
    for c in x_cp[1:]:
        c.wait()

    def proj_step(s, carry):
        project(s)
        layernorm(s + 1)
        return carry

    jax.lax.fori_loop(0, NSEG - 1, proj_step, 0)
    w_cp[3].wait()
    project(NSEG - 1)
    transpose_w(3)
    routed_ffn()

    def attn_step(s, carry):
        attention(s)
        out_proj(s)
        r0 = pl.multiple_of(s * L, L)
        pltpu.make_async_copy(o_v.at[s], o_hbm.at[:, pl.ds(r0, L)], osem.at[s]).start()
        return carry

    jax.lax.fori_loop(0, NSEG, attn_step, 0)
    for c in o_cp:
        c.wait()


@jax.jit
def pallas_parallel_sum__memory_aug_infini_attn__moe_arch_mod__prompt_kernel(
    A_x: jax.Array,
    A_wq: jax.Array,
    A_wk: jax.Array,
    A_wv: jax.Array,
    A_wo: jax.Array,
    A_beta: jax.Array,
    B_x: jax.Array,
    B_w_r: jax.Array,
    B_w_gate: jax.Array,
    B_w_up: jax.Array,
    B_w_down: jax.Array,
):
    del B_x
    hbm = pl.BlockSpec(memory_space=pltpu.HBM)
    vmem = pl.BlockSpec(memory_space=pltpu.VMEM)
    out = pl.pallas_call(
        _kernel,
        out_shape=jax.ShapeDtypeStruct((D, S), A_x.dtype),
        in_specs=[hbm, hbm, hbm, hbm, hbm, vmem, vmem, hbm, hbm, hbm],
        out_specs=hbm,
        scratch_shapes=[
            pltpu.VMEM((NSEG, D, L), bf16),
            pltpu.VMEM((4, D, D), bf16),
            pltpu.VMEM((D, F), bf16),
            pltpu.VMEM((D, F), bf16),
            pltpu.VMEM((D, F), bf16),
            pltpu.VMEM((4, D, DP), bf16),
            pltpu.VMEM((16, DP), bf16),
            pltpu.VMEM((S // T, DP, T), bf16),
            pltpu.VMEM((S // T, D, T), f32),
            pltpu.VMEM((NSEG, H, 32, L), bf16),
            pltpu.VMEM((NSEG, H, 32, L), bf16),
            pltpu.VMEM((NSEG, NG, L, T), bf16),
            pltpu.VMEM((NSEG, D, L), f32),
            pltpu.VMEM((NG, G + 8, T), f32),
            pltpu.VMEM((D, T), f32),
            pltpu.VMEM((NSEG, 8, L), f32),
            pltpu.VMEM((NSEG, D, L), bf16),
            pltpu.SemaphoreType.DMA((11,)),
            pltpu.SemaphoreType.DMA((NSEG,)),
        ],
        compiler_params=pltpu.CompilerParams(vmem_limit_bytes=100 * 2**20),
    )(A_x.reshape(S, D).T, A_wq, A_wk, A_wv, A_wo, A_beta.reshape(1, H), B_w_r,
      B_w_gate, B_w_up, B_w_down.T)
    return out.T.reshape(A_x.shape)
```

```python
import jax
import jax.numpy as jnp
import jax.experimental.pallas as pl
import jax.experimental.pallas.tpu as pltpu

S, D, H, DH, NSEG, L, F = 2048, 576, 32, 18, 4, 512, 4608
DP = 640
G = 4 * DH
NG = H // 4
T = 128
NT = L // T
NP = NG // 2
LNROWS = 144
LOG2E = 1.4426950408889634
QSCALE = DH ** -0.5 * LOG2E
NEG = -1e30

f32, bf16 = jnp.float32, jnp.bfloat16


def _dot(a, b):
    return jnp.dot(a, b, preferred_element_type=f32)


def _dot_nt(a, b):
    return jax.lax.dot_general(a, b, (((1,), (1,)), ((), ())), preferred_element_type=f32)


def _rnd(a):
    return a.astype(bf16).astype(f32)


def _iota(shape, axis):
    return jax.lax.broadcasted_iota(jnp.int32, shape, axis)


def _phi(t):
    return jnp.where(t > 0, t + 1.0, jnp.exp(t))


def _head_of(i):
    return ((i >= DH).astype(jnp.int32) + (i >= 2 * DH).astype(jnp.int32)
            + (i >= 3 * DH).astype(jnp.int32) + (i >= 4 * DH).astype(jnp.int32))


def _kernel(x_hbm, wq_hbm, wk_hbm, wv_hbm, wo_hbm, beta_hbm, wr_hbm, wg_hbm, wu_hbm,
            wd_hbm, o_hbm,
            x_v, w_v, beta_v, wr_v, wg_v, wu_v, wd_v, wt, wrc, xn_v, base, qm, vl, kn, ot, mst,
            gcol, r_v, o_v, sem, osem):
    x_cp = [pltpu.make_async_copy(x_hbm.at[:, pl.ds(s * L, L)], x_v.at[s], sem.at[s])
            for s in range(NSEG)]
    w_cp = [pltpu.make_async_copy(w, w_v.at[i], sem.at[4 + i])
            for i, w in enumerate((wq_hbm, wk_hbm, wv_hbm, wo_hbm))]
    f_cp = [pltpu.make_async_copy(a, b, sem.at[8 + i])
            for i, (a, b) in enumerate(((wg_hbm, wg_v), (wu_hbm, wu_v), (wd_hbm, wd_v)))]
    c_cp = [pltpu.make_async_copy(a, b, sem.at[11 + i])
            for i, (a, b) in enumerate(((wr_hbm, wr_v), (beta_hbm, beta_v)))]
    o_cp = [[pltpu.make_async_copy(o_v.at[s, pl.ds(p * 2 * G, 2 * G)],
                                   o_hbm.at[pl.ds(p * 2 * G, 2 * G), pl.ds(s * L, L)],
                                   osem.at[s * NP + p]) for p in range(NP)] for s in range(NSEG)]

    fillers = []

    def fill():
        while fillers:
            if next(fillers[0], False):
                return
            fillers.pop(0)

    def drain():
        while fillers:
            fill()

    def gate_column():
        gate = jax.nn.sigmoid(beta_v[...].astype(f32))
        gate = jnp.concatenate([gate, jnp.zeros((1, T - H), f32)], axis=1)
        gate = jnp.broadcast_to(gate, (T, T)).T
        r8 = _iota((8, T), 0)
        for v in range(D // 8):
            h0, h1 = (8 * v) // DH, (8 * v + 7) // DH
            gv = jnp.broadcast_to(gate[h0:h0 + 1], (8, T))
            if h1 != h0:
                gv = jnp.where(r8 < h1 * DH - 8 * v, gv, jnp.broadcast_to(gate[h1:h1 + 1], (8, T)))
            gcol[8 * v:8 * v + 8, :] = gv
            if v % 9 == 8:
                yield True

    def router_column():
        wr = wr_v[...].astype(f32).reshape(1, D)
        wr = jnp.concatenate([wr, jnp.zeros((1, DP - D), f32)], axis=1)
        wrc[...] = jnp.broadcast_to(wr, (T, DP)).T[0:D]

    def transpose_w(i):
        for c in range(0, D, T):
            n = min(T, D - c)
            w = jnp.concatenate([w_v[i, :, c:c + n], jnp.zeros((DP - D, n), bf16)], axis=0)
            wt[i, c:c + n, :] = w.T
            yield True

    def layernorm(s, c):
        b = s * NT + c
        step = LNROWS

        def tree(v):
            return sum(v[8 * k:8 * k + 8] for k in range(1, v.shape[0] // 8)) + v[0:8]

        acc = None
        for r in range(0, D, step):
            x = x_v[s, r:r + step, c * T:(c + 1) * T].astype(f32)
            base[b, r:r + step, :] = x
            acc = tree(x) if acc is None else acc + tree(x)
            yield True
        mean = jnp.sum(acc, axis=0, keepdims=True) * (1.0 / D)
        acc = None
        for r in range(0, D, step):
            xc = base[b, r:r + step, :] - mean
            acc = tree(xc * xc) if acc is None else acc + tree(xc * xc)
            yield True
        var = jnp.sum(acc, axis=0, keepdims=True) * (1.0 / D)
        sd = _rnd(jnp.sqrt(_rnd(_rnd(var) + _rnd(jnp.full((1, T), 1e-5, f32)))))
        inv, mean = 1.0 / sd, _rnd(mean)
        acc = None
        for r in range(0, D, step):
            x = base[b, r:r + step, :]
            xn = (_rnd(x - mean) * inv).astype(bf16)
            xn_v[b, r:r + step, :] = xn
            xf = xn.astype(f32)
            base[b, r:r + step, :] = x + xf
            t = tree(xf * wrc[r:r + step, :])
            acc = t if acc is None else acc + t
            yield True
        xn_v[b, D:DP, :] = jnp.zeros((DP - D, T), bf16)
        r_v[b] = jnp.broadcast_to(_rnd(jnp.sum(acc, axis=0, keepdims=True)), (8, T))

    def proj(i, s, p):
        acc = None
        for k in range(0, DP, T):
            xs = jnp.concatenate([xn_v[s * NT + c, k:k + T, :] for c in range(NT)], axis=1)
            d = _dot(wt[i, p * 2 * G:(p + 1) * 2 * G, k:k + T], xs)
            acc = d if acc is None else acc + d
            fill()
        return acc

    def project_q(s, p):
        q2 = proj(0, s, p)
        r8 = _iota((8, L), 0)
        mrow = _iota((G + 8, T), 0)
        mkeep = jnp.where(mrow < G, _head_of(mrow), mrow - G) == _head_of(_iota((G + 8, T), 1))
        for e in range(2):
            g = 2 * p + e
            q = q2[e * G:(e + 1) * G]
            qs = q * QSCALE
            for h in range(4):
                lo = 16 * h
                a0, a1, a2 = qs[lo:lo + 8], qs[lo + 8:lo + 16], qs[lo + 16:lo + 24]
                if h > 0:
                    a0 = jnp.where(r8 >= 2 * h, a0, 0.0)
                if h < 3:
                    a2 = jnp.where(r8 < 2 * h + 2, a2, 0.0)
                qm[s, 4 * g + h] = jnp.concatenate(
                    [a0, a1, a2, jnp.zeros((8, L), f32)], axis=0).astype(bf16)
            if s > 0:
                pq = jnp.concatenate([_phi(q), jnp.zeros((T - G, L), f32)], axis=0).astype(bf16)
                nd = _dot(jnp.where(mkeep, mst[g], 0.0).astype(bf16), pq)
                inv = 1.0 / (nd[G:] + 1e-6)
                ib = [jnp.broadcast_to(inv[h:h + 1], (8, L)) for h in range(4)]
                iv = jnp.concatenate(
                    [ib[0], ib[0], jnp.where(r8 < 2, ib[0], ib[1]), ib[1],
                     jnp.where(r8 < 4, ib[1], ib[2]), ib[2],
                     jnp.where(r8 < 6, ib[2], ib[3]), ib[3], ib[3]], axis=0)
                gg = gcol[g * G:(g + 1) * G, :]
                ot[s, g * G:(g + 1) * G, :] = nd[:G] * iv * jnp.concatenate([gg] * NT, axis=1)

    def project_k(s, p):
        k2 = proj(1, s, p)
        pks = []
        for e in range(2):
            k = k2[e * G:(e + 1) * G]
            zpad = jnp.zeros((T - G, L), f32)
            kn[s, 2 * p + e] = jnp.concatenate([k, zpad], axis=0).astype(bf16).T
            if s < NSEG - 1:
                pks.append(jnp.concatenate([_phi(k), zpad], axis=0).astype(bf16))
        return pks

    def project_v(s, p, pks):
        v2 = proj(2, s, p)
        for e in range(2):
            g = 2 * p + e
            v = v2[e * G:(e + 1) * G]
            vls = []
            for h in range(4):
                vh = jnp.concatenate([v[16 * h:16 * h + 24], jnp.ones((8, L), f32)], axis=0)
                vls.append(vh.astype(bf16))
                vl[s, 4 * g + h] = vls[h]
            if pks:
                v80 = jnp.concatenate([vls[0][:16], vls[1][:16], vls[2][:16], vls[3]], axis=0)
                upd = _dot_nt(v80, pks[e])
                mst[g] = upd if s == 0 else mst[g] + upd

    def attention(extra):
        keep = _iota((T, T), 0) <= _iota((T, T), 1)
        r8 = _iota((8, T), 0)
        units = [(s, g, i, j) for s in range(NSEG) for g in range(NG)
                 for i in range(NT) for j in range(i + 1)]
        run = {}

        def scores(s, g, i, j):
            w = []
            for h in range(4):
                parts = [qm[s, 4 * g + h, :, i * T:(i + 1) * T]]
                if h > 0:
                    parts.insert(0, jnp.zeros((16 * h, T), bf16))
                parts.append(jnp.zeros((T - 32 - 16 * h, T), bf16))
                w.append(jnp.concatenate(parts, axis=0))
            st = _dot(kn[s, g, j * T:(j + 1) * T, :], jnp.concatenate(w, axis=1))
            ps, alphas = [], []
            for h in range(4):
                sh = st[:, h * T:(h + 1) * T]
                if i == j:
                    sh = jnp.where(keep, sh, NEG)
                m = jnp.max(sh, axis=0, keepdims=True)
                if j > 0:
                    m = jnp.maximum(m, run[h])
                    alphas.append(jnp.exp2(run[h] - m))
                run[h] = m
                ps.append(jnp.exp2(sh - m).astype(bf16))
            return ps, alphas

        def values(s, g, i, j, ps, alphas, acc):
            new = [_dot(vl[s, 4 * g + h, :, j * T:(j + 1) * T], ps[h]) for h in range(4)]
            if j > 0:
                new = [a * al + b for a, al, b in zip(acc, alphas, new)]
            if j < i:
                return new
            o = []
            for h in range(4):
                inv = 1.0 / new[h][24:32]
                o.append([new[h][8 * c:8 * c + 8] * inv for c in range(3)])
            a_dot = jnp.concatenate(
                [o[0][0], o[0][1], jnp.where(r8 < 2, o[0][2], o[1][0]), o[1][1],
                 jnp.where(r8 < 4, o[1][2], o[2][0]), o[2][1],
                 jnp.where(r8 < 6, o[2][2], o[3][0]), o[3][1], o[3][2]], axis=0)
            dst = (s, slice(g * G, (g + 1) * G), slice(i * T, (i + 1) * T))
            mix = (1.0 - gcol[g * G:(g + 1) * G, :]) * a_dot
            ot[dst] = ot[dst] + mix if s > 0 else mix
            return None

        lag, pend, acc = 2, {}, None
        for t in range(len(units) + lag):
            if t < len(units):
                pend[t] = scores(*units[t])
            if t >= lag:
                acc = values(*units[t - lag], *pend.pop(t - lag), acc)
            fill()
            extra(t)

    def out_proj(s):
        o = jnp.concatenate([ot[s], jnp.zeros((DP - D, L), f32)], axis=0).astype(bf16)
        for p in range(NP):
            rows = slice(p * 2 * G, (p + 1) * 2 * G)
            a = _dot(wt[3, rows, :], o)
            for c in range(NT):
                o_v[s, rows, c * T:(c + 1) * T] = (
                    base[s * NT + c, rows, :] + a[:, c * T:(c + 1) * T]).astype(bf16)
            o_cp[s][p].start()

    def route():
        r = r_v[...]
        idx = _iota(r.shape, 0) * T + _iota(r.shape, 2)
        m1 = jnp.max(r)
        i1 = jnp.minimum(jnp.min(jnp.where(r == m1, idx, S)), S - 1)
        r = jnp.where(idx == i1, -jnp.inf, r)
        m2 = jnp.max(r)
        i2 = jnp.minimum(jnp.min(jnp.where((r == m2) & (idx != i1), idx, S)), S - 1)
        picks = ((i1, m1), (i2, m2))
        xsel = jnp.zeros((16, DP), f32)
        for n, (i, _) in enumerate(picks):
            hot = (_iota((16, T), 0) == n) & (_iota((16, T), 1) == (i & (T - 1)))
            xsel = xsel + _dot_nt(hot.astype(f32).astype(bf16), xn_v[i >> 7])
        return picks, xsel.astype(bf16)

    def ffn(picks, xsel):
        ys = [None] * (DP // T)
        for n in range(0, F, L):
            gu = []
            for w_ref in (wg_v, wu_v):
                acc = None
                for k in range(0, D, T):
                    w = w_ref[k:min(k + T, D), n:n + L]
                    if k + T > D:
                        w = jnp.concatenate([w, jnp.zeros((DP - D, L), bf16)], axis=0)
                    d = _dot(xsel[:, k:k + T], w)
                    acc = d if acc is None else acc + d
                    yield True
                gu.append(acc)
            hid = (gu[0] * jax.nn.sigmoid(gu[0]) * gu[1]).astype(bf16)
            for c, k in enumerate(range(0, D, T)):
                w = wd_v[k:min(k + T, D), n:n + L]
                if k + T > D:
                    w = jnp.concatenate([w, jnp.zeros((DP - D, L), bf16)], axis=0)
                d = _dot_nt(hid, w)
                ys[c] = d if ys[c] is None else ys[c] + d
                yield True
        lane = _iota((T, T), 1)
        for n, (i, m) in enumerate(picks):
            wgt = jax.nn.sigmoid(jnp.full((1, T), m, f32))
            for c, k in enumerate(range(0, D, T)):
                rows = min(T, D - k)
                col = jnp.broadcast_to(ys[c][n:n + 1] * wgt, (T, T)).T
                upd = jnp.where(lane == (i & (T - 1)), col, 0.0)[0:rows]
                base[i >> 7, k:k + rows, :] = base[i >> 7, k:k + rows, :] + upd
                yield True

    for c in (c_cp[0], x_cp[0], w_cp[0], w_cp[1], w_cp[2], c_cp[1], x_cp[1]):
        c.start()
    c_cp[0].wait()
    router_column()
    x_cp[0].wait()
    fillers.extend(layernorm(0, c) for c in range(NT))
    drain()
    w_cp[0].wait()
    fillers.append(transpose_w(0))
    drain()
    for s in range(NSEG):
        if s == 0:
            for p in range(NP):
                project_q(s, p)
                if p == 1:
                    w_cp[1].wait()
                    fillers.append(transpose_w(1))
            drain()
            w_cp[2].wait()
            fillers.append(transpose_w(2))
            pks = [project_k(s, p) for p in range(NP)]
            drain()
            c_cp[1].wait()
            x_cp[1].wait()
            for c in (x_cp[2], x_cp[3], w_cp[3], *f_cp):
                c.start()
            fillers.extend(layernorm(1, c) for c in range(NT))
            fillers.append(gate_column())
            for p in range(NP):
                project_v(s, p, pks[p])
            drain()
            continue
        if s + 1 < NSEG:
            x_cp[s + 1].wait()
            fillers.extend(layernorm(s + 1, c) for c in range(NT))
        else:
            w_cp[3].wait()
            fillers.append(transpose_w(3))
        for p in range(NP):
            project_q(s, p)
            project_v(s, p, project_k(s, p))
            if s == NSEG - 1 and p == 1:
                picks, xsel = route()
        drain()
    for c in f_cp:
        c.wait()
    fillers.append(ffn(picks, xsel))

    per_seg = NG * NT * (NT + 1) // 2

    def extra(t):
        if t == 2 * per_seg + 3:
            drain()
            out_proj(0)
        elif t == 2 * per_seg + 40:
            out_proj(1)
        elif t == 3 * per_seg + 3:
            out_proj(2)

    attention(extra)
    out_proj(NSEG - 1)
    for cs in o_cp:
        for c in cs:
            c.wait()


@jax.jit
def pallas_parallel_sum__memory_aug_infini_attn__moe_arch_mod__prompt_kernel(
    A_x: jax.Array,
    A_wq: jax.Array,
    A_wk: jax.Array,
    A_wv: jax.Array,
    A_wo: jax.Array,
    A_beta: jax.Array,
    B_x: jax.Array,
    B_w_r: jax.Array,
    B_w_gate: jax.Array,
    B_w_up: jax.Array,
    B_w_down: jax.Array,
):
    del B_x
    hbm = pl.BlockSpec(memory_space=pltpu.HBM)
    out = pl.pallas_call(
        _kernel,
        out_shape=jax.ShapeDtypeStruct((D, S), A_x.dtype),
        in_specs=[hbm] * 10,
        out_specs=hbm,
        scratch_shapes=[
            pltpu.VMEM((NSEG, D, L), bf16),
            pltpu.VMEM((4, D, D), bf16),
            pltpu.VMEM((1, H), bf16),
            pltpu.VMEM((D,), bf16),
            pltpu.VMEM((D, F), bf16),
            pltpu.VMEM((D, F), bf16),
            pltpu.VMEM((D, F), bf16),
            pltpu.VMEM((4, D, DP), bf16),
            pltpu.VMEM((D, T), f32),
            pltpu.VMEM((S // T, DP, T), bf16),
            pltpu.VMEM((S // T, D, T), f32),
            pltpu.VMEM((NSEG, H, 32, L), bf16),
            pltpu.VMEM((NSEG, H, 32, L), bf16),
            pltpu.VMEM((NSEG, NG, L, T), bf16),
            pltpu.VMEM((NSEG, D, L), f32),
            pltpu.VMEM((NG, G + 8, T), f32),
            pltpu.VMEM((D, T), f32),
            pltpu.VMEM((S // T, 8, T), f32),
            pltpu.VMEM((NSEG, D, L), bf16),
            pltpu.SemaphoreType.DMA((13,)),
            pltpu.SemaphoreType.DMA((NSEG * NP,)),
        ],
        compiler_params=pltpu.CompilerParams(vmem_limit_bytes=100 * 2**20),
    )(A_x.reshape(S, D).T, A_wq, A_wk, A_wv, A_wo, A_beta.reshape(1, H), B_w_r,
      B_w_gate, B_w_up, B_w_down.T)
    return out.T.reshape(A_x.shape)
```

```python
import functools

import jax
import jax.numpy as jnp
import jax.experimental.pallas as pl
import jax.experimental.pallas.tpu as pltpu

S, D, H, DH, NSEG, L, F = 2048, 576, 32, 18, 4, 512, 4608
DP = 640
G = 4 * DH
NG = H // 4
T = 128
NT = L // T
NP = NG // 2
LATE = 1
DEFER_K = 2
PIN_P = 5
PIN_G = 2
PIN_A = 2
DIAG = True
LAG = 3
ORDER = ((3, 2), (3, 3), (3, 0), (0, 0), (3, 1), (2, 1), (2, 2), (2, 0), (1, 0), (1, 1))
SLOTS = ((0, 1, 2, 3, 4), (3, 4,), (2, 3, 4))
LNROWS = 192
LOG2E = 1.4426950408889634
QSCALE = DH ** -0.5 * LOG2E
NEG = -1e30
ONES_ROW = (23, 23, 0, 0)
XPARTS = ((0, 256), (256, 256), (512, 512), (1024, 1024))
RANGES = ((0, 32), (32, 64), (64, 96), (96, 128), (32, 128), (0, 64), (64, 128))

f32, bf16, u32 = jnp.float32, jnp.bfloat16, jnp.uint32
ALL = slice(None)


def _dot(a, b):
    return jnp.dot(a, b, preferred_element_type=f32)


def _dot_nt(a, b):
    return jax.lax.dot_general(a, b, (((1,), (1,)), ((), ())), preferred_element_type=f32)


def _rnd(a):
    return a.astype(bf16).astype(f32)


def _rcp(a):
    return pltpu.reciprocal(a, full_range=False)


def _iota(shape, axis):
    return jax.lax.broadcasted_iota(jnp.int32, shape, axis)


def _pad_to_tile(a):
    if a.shape[1] < T:
        a = jnp.concatenate([a, jnp.zeros((a.shape[0], T - a.shape[1]), a.dtype)], axis=1)
    if a.shape[0] < T:
        a = jnp.concatenate([a, jnp.zeros((T - a.shape[0], T), a.dtype)], axis=0)
    return a


def _phi(t):
    return jnp.where(t > 0, t + 1.0, jnp.exp(t))


def _head_of(i):
    return ((i >= DH).astype(jnp.int32) + (i >= 2 * DH).astype(jnp.int32)
            + (i >= 3 * DH).astype(jnp.int32) + (i >= 4 * DH).astype(jnp.int32))


class _Packed:
    def __init__(self, ref):
        self.words = ref

    def _index(self, idx):
        *lead, rows, cols = idx
        start, stop, _ = rows.indices(2 * self.words.shape[-2])
        return (*lead, slice(start // 2, stop // 2), cols)

    def __getitem__(self, idx):
        return pltpu.bitcast(self.words[self._index(idx)], bf16)

    def __setitem__(self, idx, value):
        self.words[self._index(idx)] = pltpu.bitcast(value, u32)


def _kernel(x_hbm, wq_hbm, wk_hbm, wv_hbm, wo_hbm, beta_hbm, wr_hbm, wg_hbm, wu_hbm,
            wd_hbm, o_hbm,
            x_v, w_v, beta_v, wr_v, wg_v, wu_v, wd_v, wt, wrc, xn_v, qm, vl, kn, ot, mst,
            gcol, r_v, o_v, causal, lanes, sem):
    wt, xn_v, qm, kn = (_Packed(r) for r in (wt, xn_v, qm, kn))
    x_cp = [pltpu.make_async_copy(x_hbm.at[:, pl.ds(t, n)], x_v.at[:, pl.ds(t, n)], sem.at[7 + i])
            for i, (t, n) in enumerate(XPARTS)]
    w_cp = [pltpu.make_async_copy(w, w_v.at[i], sem.at[i])
            for i, w in enumerate((wq_hbm, wk_hbm, wv_hbm, wo_hbm))]
    f_cp = [pltpu.make_async_copy(a, b, sem.at[4])
            for i, (a, b) in enumerate(((wg_hbm, wg_v), (wu_hbm, wu_v), (wd_hbm, wd_v)))]
    c_cp = [pltpu.make_async_copy(a, b, sem.at[5])
            for i, (a, b) in enumerate(((wr_hbm, wr_v), (beta_hbm, beta_v)))]
    o_cp = [[pltpu.make_async_copy(o_v.at[s, pl.ds(p * 2 * G, 2 * G)],
                                   o_hbm.at[pl.ds(p * 2 * G, 2 * G), pl.ds(s * L, L)],
                                   sem.at[6]) for p in range(NP)] for s in range(NSEG)]

    fillers = []

    lane8 = _iota((8, T), 1)
    never = lane8 < jnp.min(lane8, axis=1, keepdims=True)
    zero = jnp.min(lane8)
    link = [None, None]
    pins = []

    def opaque(ref, idx):
        ax = -1 if ref.shape[-1] > T else -2
        n = idx[ax].stop - idx[ax].start
        idx = list(idx)
        idx[ax] = pl.ds(pl.multiple_of(idx[ax].start + zero * n, n), n)
        return tuple(idx)

    def pin(ref, idx, steps):
        ref = ref.words if isinstance(ref, _Packed) else ref
        rows = 16 if ref.dtype == bf16 else 8
        pins.append([steps, ref, opaque(ref, (*idx, slice(0, rows), slice(0, T)))])

    def pinned_operand(a):
        for p in pins:
            p[0] -= 1
        due = [p for p in pins if p[0] < 0]
        if not due:
            return a
        pins[:] = [p for p in pins if p[0] >= 0]
        t = pltpu.bitcast(a[-16:, -T:], u32)
        for _, ref, idx in due:
            t = tie(t, pltpu.bitcast(ref[idx], u32))
        t = pltpu.bitcast(t, bf16)
        if a.shape[1] > T:
            t = jnp.concatenate([a[-16:, :-T], t], axis=1)
        return jnp.concatenate([a[:-16], t], axis=0)

    def tie(a, b):
        return a if b is None else jnp.where(never, b, a)

    def fill(after=None):
        link[0], link[1] = after, None
        while fillers:
            if next(fillers[0], False):
                break
            fillers.pop(0)
        return link[1]

    def drain():
        while fillers:
            fill()

    def gate_column():
        gate = jax.nn.sigmoid(beta_v[...].astype(f32))
        gate = jnp.concatenate([gate, jnp.zeros((1, T - H), f32)], axis=1)
        gate = jnp.broadcast_to(gate, (T, T)).T
        r8 = _iota((8, T), 0)
        for v in range(D // 8):
            h0, h1 = (8 * v) // DH, (8 * v + 7) // DH
            gv = jnp.broadcast_to(gate[h0:h0 + 1], (8, T))
            if h1 != h0:
                gv = jnp.where(r8 < h1 * DH - 8 * v, gv, jnp.broadcast_to(gate[h1:h1 + 1], (8, T)))
            gcol[8 * v:8 * v + 8, :] = gv
            if v % 9 == 8:
                yield True

    def router_column():
        wr = wr_v[...].astype(f32).reshape(1, D)
        wr = jnp.concatenate([wr, jnp.zeros((1, DP - D), f32)], axis=1)
        wrc[...] = jnp.broadcast_to(wr, (T, DP)).T[0:D]

    def transpose_w(i, tied=False):
        for c in range(0, D, T):
            n = min(T, D - c)
            if not tied:
                w = jnp.concatenate([w_v[i, :, c:c + n], jnp.zeros((DP - D, n), bf16)], axis=0)
                wt[i, c:c + n, :] = w.T
                yield True
                continue
            for k in range(0, D, T):
                w = _pad_to_tile(w_v[i, k:min(k + T, D), c:c + n].astype(f32))
                w = jnp.concatenate([tie(w[r:r + 8], link[0]) for r in range(0, T, 8)], axis=0).T
                wt[i, c:c + n, k:k + T] = w[0:n].astype(bf16)
                if k + T >= D:
                    pin(wt, (i,), PIN_P)
                yield True

    normed = [0]

    def layernorm(b, step):

        def chain(acc, v):
            h = v.shape[0] // 16 * 8
            a, c = v[0:8], v[h:h + 8]
            for k in range(8, h, 8):
                a, c = a + v[k:k + 8], c + v[h + k:h + k + 8]
            return a + c if acc is None else acc + (a + c)

        def rows(v):
            return jnp.concatenate([tie(v, link[0])] * (step // 8), axis=0)

        def bcast(v):
            return jnp.broadcast_to(v, (8, T))

        acc = jnp.zeros((8, T), f32)
        for r in range(0, D, step):
            x = x_v[r:r + step, b * T:(b + 1) * T].astype(f32)
            link[1] = acc = chain(tie(acc, link[0]), x)
            yield True
        mean = bcast(jnp.sum(acc, axis=0, keepdims=True) * (1.0 / D))
        acc = None
        for r in range(0, D, step):
            xc = x_v[r:r + step, b * T:(b + 1) * T].astype(f32) - rows(mean)
            link[1] = acc = chain(acc, xc * xc)
            yield True
        var = bcast(jnp.sum(acc, axis=0, keepdims=True) * (1.0 / D))
        sd = _rnd(jnp.sqrt(_rnd(_rnd(var) + _rnd(jnp.full((8, T), 1e-5, f32)))))
        inv, mean = jnp.concatenate([1.0 / sd] * (step // 8), axis=0), _rnd(mean)
        acc = None
        for r in range(0, D, step):
            x = x_v[r:r + step, b * T:(b + 1) * T].astype(f32)
            xn = (_rnd(x - rows(mean)) * inv).astype(bf16)
            xn_v[b, r:r + step, :] = xn
            link[1] = acc = chain(acc, xn.astype(f32) * wrc[r:r + step, :])
            yield True
        xn_v[b, D:DP, :] = jnp.zeros((DP - D, T), bf16)
        r_v[b] = jnp.broadcast_to(_rnd(jnp.sum(acc, axis=0, keepdims=True)), (8, T))
        normed[0] += 1

    late = [None] * LATE
    deferred = []

    def flush():
        while deferred:
            deferred.pop(0)()

    def proj(i, s, p, slots):
        acc = None
        for k in range(0, DP, T):
            xs = jnp.concatenate([xn_v[s * NT + c, k:k + T, :] for c in range(NT)], axis=1)
            w = wt[i, p * 2 * G:(p + 1) * 2 * G, k:k + T]
            d = _dot(pinned_operand(w), xs)
            done = late.pop(0)
            top = tie(d[-8:, :T], done)
            d = jnp.concatenate([d[:-8], jnp.concatenate([top, d[-8:, T:]], axis=1)], axis=0)
            acc = d if acc is None else acc + d
            late.append(fill(d[0:8, 0:T]) if k // T in slots else None)
            if k == DEFER_K * T:
                flush()
        return acc

    def project_q(s, p):
        q2 = proj(0, s, p, SLOTS[0] if s else (0, 1, 2, 3, 4))
        r8 = _iota((8, L), 0)
        for e in range(2):
            g = 2 * p + e
            q = q2[e * G:(e + 1) * G]
            qs = q * QSCALE
            for h in range(4):
                lo = 16 * h
                a0, a1, a2 = qs[lo:lo + 8], qs[lo + 8:lo + 16], qs[lo + 16:lo + 24]
                if h > 0:
                    a0 = jnp.where(r8 >= 2 * h, a0, 0.0)
                if h < 3:
                    a2 = jnp.where(r8 < 2 * h + 2, a2, 0.0)
                qm[s, 4 * g + h, :, :] = jnp.concatenate(
                    [a0, a1, a2, jnp.zeros((8, L), f32)], axis=0).astype(bf16)
            if s > 0:
                pq = jnp.concatenate([_phi(q), jnp.zeros((T - G, L), f32)], axis=0).astype(bf16)
                deferred.append(functools.partial(memory_read, s, g, pq))

    def memory_read(s, g, pq):
        r8 = _iota((8, L), 0)
        mrow = _iota((G + 8, T), 0)
        mkeep = jnp.where(mrow < G, _head_of(mrow), mrow - G) == _head_of(_iota((G + 8, T), 1))
        nd = _dot(jnp.where(mkeep, mst[g], 0.0).astype(bf16), pq)
        inv = _rcp(nd[G:] + 1e-6)
        ib = [jnp.broadcast_to(inv[h:h + 1], (8, L)) for h in range(4)]
        iv = jnp.concatenate(
            [ib[0], ib[0], jnp.where(r8 < 2, ib[0], ib[1]), ib[1],
             jnp.where(r8 < 4, ib[1], ib[2]), ib[2],
             jnp.where(r8 < 6, ib[2], ib[3]), ib[3], ib[3]], axis=0)
        gg = gcol[g * G:(g + 1) * G, :]
        ot[s, g * G:(g + 1) * G, :] = nd[:G] * iv * jnp.concatenate([gg] * NT, axis=1)

    def memory_update(s, g, v80, pk):
        upd = _dot_nt(v80, pk)
        mst[g] = upd if s == 0 else mst[g] + upd

    def project_k(s, p):
        k2 = proj(1, s, p, SLOTS[1] if s else (2, 3, 4))
        pks = []
        for e in range(2):
            k = k2[e * G:(e + 1) * G]
            zpad = jnp.zeros((T - G, L), f32)
            kn[s, 2 * p + e, :, :] = jnp.concatenate([k, zpad], axis=0).astype(bf16).T
            if s < NSEG - 1:
                pks.append(jnp.concatenate([_phi(k), zpad], axis=0).astype(bf16))
        return pks

    def project_v(s, p, pks):
        v2 = proj(2, s, p, SLOTS[2] if s or not p else (0, 1, 2, 3, 4))
        for e in range(2):
            g = 2 * p + e
            v = v2[e * G:(e + 1) * G]
            for h in range(4):
                a = [v[16 * h + c:16 * h + c + 8] for c in (0, 8, 16)]
                c, r = divmod(ONES_ROW[h], 8)
                a[c] = jnp.where(_iota((8, L), 0) == r, 1.0, a[c])
                vl[s, 4 * g + h] = jnp.concatenate(a, axis=0)
            if pks:
                v80 = jnp.concatenate([v, jnp.ones((8, L), f32)], axis=0).astype(bf16)
                deferred.append(functools.partial(memory_update, s, g, v80, pks[e]))
        pin(qm, (s, 8 * p), PIN_P)
        pin(kn, (s, 2 * p), PIN_P)
        pin(vl, (s, 8 * p), PIN_P)
        if s:
            pin(ot, (s,), PIN_P)

    def attention(segs, extra):
        r8 = _iota((8, T), 0)
        units = [(s, g, i, j) for s in segs for g in range(NG) for i, j in ORDER]
        run, accs = {}, {}

        lane32 = _iota((32, T), 1)
        carry = {}

        def own_queries(s, g, i):
            w = []
            for h in range(4):
                parts = [qm[s, 4 * g + h, :, i * T:(i + 1) * T]]
                if h > 0:
                    parts.insert(0, jnp.zeros((16 * h, T), bf16))
                parts.append(jnp.zeros((T - 32 - 16 * h, T), bf16))
                w.append(jnp.concatenate(parts, axis=0))
            return jnp.concatenate(w, axis=1)

        def shared_queries(qw, *parts):
            slots = [None] * 8
            for h, shift, lo, hi in parts:
                q = pltpu.roll(qw[h], shift, 1) if shift else qw[h]
                for e in range(2):
                    t = q[8 * e:8 * e + 8] & lanes[RANGES.index((lo, hi))]
                    slots[h + e] = t if slots[h + e] is None else t | slots[h + e]
            slots = [jnp.zeros((8, T), u32) if t is None else t for t in slots]
            return pltpu.bitcast(jnp.concatenate(slots, axis=0), bf16)

        def diagonal_scores(s, g, i):
            k0 = i * T
            own = carry.pop("own") if i else _dot(kn[s, g, 0:32, :], own_queries(s, g, 0))
            qw = [qm.words[s, 4 * g + h, :, k0:k0 + T] for h in range(4)]
            x = _dot(kn[s, g, k0 + 32:k0 + 64, :], jnp.concatenate(
                [shared_queries(qw, (h, 0, 32, T), (3, 96 - 32 * h, 0, 32)) for h in range(3)],
                axis=1))
            y = _dot(kn[s, g, k0 + 64:k0 + 96, :], jnp.concatenate(
                [shared_queries(qw, (h, 0, 64, T), (h + 1, 64, 0, 64)) for h in (0, 2)], axis=1))
            z = _dot(kn[s, g, k0 + 96:k0 + T, :], shared_queries(
                qw, *[(h, (32 * h + 32) % T, 32 * h, 32 * h + 32) for h in range(4)]))
            xs = [x[:, h * T:(h + 1) * T] for h in range(3)]
            xr = [pltpu.roll(xs[h], 32 * h + 32, 1) for h in range(3)]
            xs.append(jnp.where(lane32 < 64, xr[0], jnp.where(lane32 < 96, xr[1], xr[2])))
            ys = [y[:, :T], pltpu.roll(y[:, :T], 64, 1), y[:, T:], pltpu.roll(y[:, T:], 64, 1)]
            zs = [pltpu.roll(z, 96 - 32 * h, 1) for h in range(3)] + [z]
            return [jnp.concatenate([own[:, h * T:(h + 1) * T], xs[h], ys[h], zs[h]], axis=0)
                    for h in range(4)]

        def scores(s, g, i, j):
            if DIAG and i == j:
                shs = diagonal_scores(s, g, i)
            else:
                more = 32 if DIAG and j == i - 1 else 0
                st = _dot(pinned_operand(kn[s, g, j * T:(j + 1) * T + more, :]),
                          own_queries(s, g, i))
                if more:
                    carry["own"] = st[T:]
                shs = [st[:T, h * T:(h + 1) * T] for h in range(4)]
            ps, alphas = [], []
            later = any(a == i for a, _ in ORDER[:ORDER.index((i, j))])
            for h in range(4):
                sh = shs[h]
                if i == j:
                    sh = sh + causal[...]
                m = jnp.max(sh, axis=0, keepdims=True)
                if later:
                    m = jnp.maximum(m, run[i, h])
                    alphas.append(jnp.exp2(run[i, h] - m))
                run[i, h] = m
                ps.append(jnp.exp2(sh - m).astype(bf16))
            return ps, alphas

        def values(s, g, i, j, ps, alphas):
            new = [_dot(vl[s, 4 * g + h, :, j * T:(j + 1) * T], ps[h]) for h in range(4)]
            if alphas:
                new = [a * al + b for a, al, b in zip(accs.pop(i), alphas, new)]
            if any(a == i for a, _ in ORDER[ORDER.index((i, j)) + 1:]):
                accs[i] = new
                return
            o = []
            for h in range(4):
                inv = _rcp(jnp.broadcast_to(new[h][ONES_ROW[h]:ONES_ROW[h] + 1], (8, T)))
                o.append([new[h][8 * c:8 * c + 8] * inv for c in range(3)])
            a_dot = jnp.concatenate(
                [o[0][0], o[0][1], jnp.where(r8 < 2, o[0][2], o[1][0]), o[1][1],
                 jnp.where(r8 < 4, o[1][2], o[2][0]), o[2][1],
                 jnp.where(r8 < 6, o[2][2], o[3][0]), o[3][1], o[3][2]], axis=0)
            dst = (s, slice(g * G, (g + 1) * G), slice(i * T, (i + 1) * T))
            mix = (1.0 - gcol[g * G:(g + 1) * G, :]) * a_dot
            ot[dst] = ot[dst] + mix if s > 0 else mix
            if (i, j) == ORDER[-1] and g % PIN_G == PIN_G - 1:
                pin(ot, (s,), PIN_A)

        pend = {}
        for t in range(len(units) + LAG):
            if t < len(units):
                pend[t] = scores(*units[t])
            if t >= LAG:
                values(*units[t - LAG], *pend.pop(t - LAG))
            extra(t)

    def out_proj(s):
        o = jnp.concatenate([ot[s], jnp.zeros((DP - D, L), f32)], axis=0).astype(bf16)
        for p in range(NP):
            rows = slice(p * 2 * G, (p + 1) * 2 * G)
            a = _dot(pinned_operand(wt[3, rows, :]), o)
            for c in range(NT):
                b = s * NT + c
                res = x_v[rows, b * T:(b + 1) * T].astype(f32) + xn_v[b, rows, :].astype(f32)
                o_v[s, rows, c * T:(c + 1) * T] = (res + a[:, c * T:(c + 1) * T]).astype(bf16)
            o_cp[s][p].start()
            spare = (NSEG, slice(0, 16), slice(0, T))
            o_v[opaque(o_v, spare)] = jnp.zeros((16, T), bf16)
            pin(o_v, (NSEG,), 1)

    def route():
        r = r_v[...]
        idx = _iota(r.shape, 0) * T + _iota(r.shape, 2)
        m1 = jnp.max(r)
        i1 = jnp.minimum(jnp.min(jnp.where(r == m1, idx, S)), S - 1)
        r = jnp.where(idx == i1, -jnp.inf, r)
        m2 = jnp.max(r)
        i2 = jnp.minimum(jnp.min(jnp.where((r == m2) & (idx != i1), idx, S)), S - 1)
        picks = ((i1, m1), (i2, m2))
        xsel = jnp.zeros((8, DP), f32)
        for n, (i, _) in enumerate(picks):
            hot = (_iota((8, T), 0) == n) & (_iota((8, T), 1) == (i & (T - 1)))
            xsel = xsel + _dot_nt(hot.astype(f32), xn_v[i >> 7, :, :])
        return picks, xsel

    def ffn(picks, xsel):
        ys = [None] * (DP // T)
        for n in range(0, F, L):
            gu = []
            for w_ref in (wg_v, wu_v):
                acc = None
                for k in range(0, D, T):
                    w = w_ref[k:min(k + T, D), n:n + L]
                    if k + T > D:
                        w = jnp.concatenate([w, jnp.zeros((DP - D, L), bf16)], axis=0)
                    d = _dot(xsel[:, k:k + T], w)
                    acc = d if acc is None else acc + d
                    yield True
                gu.append(acc)
            hid = gu[0] * jax.nn.sigmoid(gu[0]) * gu[1]
            for c, k in enumerate(range(0, D, T)):
                w = wd_v[k:min(k + T, D), n:n + L]
                if k + T > D:
                    w = jnp.concatenate([w, jnp.zeros((DP - D, L), bf16)], axis=0)
                d = _dot_nt(hid, w)
                ys[c] = d if ys[c] is None else ys[c] + d
                yield True
        lane = _iota((T, T), 1)
        for n, (i, m) in enumerate(picks):
            wgt = jax.nn.sigmoid(jnp.full((1, T), m, f32))
            for c, k in enumerate(range(0, D, T)):
                rows = min(T, D - k)
                col = jnp.broadcast_to(ys[c][n:n + 1] * wgt, (T, T)).T
                upd = jnp.where(lane == (i & (T - 1)), col, 0.0)[0:rows]
                dst = (slice(k, k + rows), pl.ds(pl.multiple_of((i >> 7) << 7, T), T))
                x_v[dst] = (x_v[dst].astype(f32) + upd).astype(bf16)
                yield True
            pin(x_v, (), PIN_A)

    for c in (*c_cp, *x_cp[:2], *w_cp[:3]):
        c.start()
    causal[...] = jnp.where(_iota((T, T), 0) <= _iota((T, T), 1), 0.0, NEG)
    for n, (lo, hi) in enumerate(RANGES):
        lanes[n] = pltpu.bitcast(jnp.where((lane8 >= lo) & (lane8 < hi), -1, 0), u32)
    for c in c_cp:
        c.wait()
    router_column()
    for _ in gate_column():
        pass
    for b in range(NT):
        if b % 2 == 0:
            x_cp[b // 2].wait()
        fillers.append(layernorm(b, D))
        drain()
    x_cp[2].start()
    w_cp[0].wait()
    fillers.append(transpose_w(0))
    drain()
    for p in range(NP):
        if p == NP - 1:
            for c in (x_cp[3], w_cp[3]):
                c.start()
            w_cp[1].wait()
            fillers.append(transpose_w(1))
            drain()
        project_q(0, p)
    pks = []
    for p in range(NP):
        if p == 2:
            for ref in (wg_v, wu_v, wd_v):
                ref[0:16, 0:T] = kn[0, 0, 0:16, :]
            for c in f_cp:
                c.start()
            for c in (w_cp[2], x_cp[2]):
                c.wait()
            fillers.append(transpose_w(2))
            drain()
            fillers.extend(layernorm(b, D // 2) for b in range(NT, 2 * NT))
        pks.append(project_k(0, p))
    for p in range(NP):
        project_v(0, p, pks[p])
    drain()
    for s in range(1, NSEG):
        while normed[0] < (s + 1) * NT:
            assert s > 1
            fill()
        if s == NSEG - 1:
            attention([0], lambda t: None)
        for p in range(NP):
            project_q(s, p)
            if s == 1 and p == 0:
                for c in (x_cp[3], w_cp[3]):
                    c.wait()
                fillers.extend(layernorm(b, LNROWS) for b in range(2 * NT, S // T))
                fillers.append(transpose_w(3, True))
            if s == NSEG - 1 and p == NP - 1:
                for c in f_cp:
                    c.wait()
            project_v(s, p, project_k(s, p))
            if s == NSEG - 1 and p == 1:
                picks, xsel = route()
    drain()
    flush()
    fillers.append(ffn(picks, xsel))
    per_seg = NG * NT * (NT + 1) // 2

    def extra(t):
        fill()
        if t == 2 * per_seg:
            drain()
            out_proj(0)
        elif t == 2 * per_seg + 20:
            out_proj(1)
        elif t == 2 * per_seg + 40:
            out_proj(2)

    attention(range(1, NSEG), extra)
    out_proj(NSEG - 1)
    for cs in o_cp:
        for c in cs:
            c.wait()


@jax.jit
def pallas_parallel_sum__memory_aug_infini_attn__moe_arch_mod__prompt_kernel(
    A_x: jax.Array,
    A_wq: jax.Array,
    A_wk: jax.Array,
    A_wv: jax.Array,
    A_wo: jax.Array,
    A_beta: jax.Array,
    B_x: jax.Array,
    B_w_r: jax.Array,
    B_w_gate: jax.Array,
    B_w_up: jax.Array,
    B_w_down: jax.Array,
):
    del B_x
    hbm = pl.BlockSpec(memory_space=pltpu.HBM)
    out = pl.pallas_call(
        _kernel,
        out_shape=jax.ShapeDtypeStruct((D, S), A_x.dtype),
        in_specs=[hbm] * 10,
        out_specs=hbm,
        scratch_shapes=[
            pltpu.VMEM((D, S), bf16),
            pltpu.VMEM((4, D, D), bf16),
            pltpu.VMEM((1, H), bf16),
            pltpu.VMEM((D,), bf16),
            pltpu.VMEM((D, F), bf16),
            pltpu.VMEM((D, F), bf16),
            pltpu.VMEM((D, F), bf16),
            pltpu.VMEM((4, D // 2, DP), u32),
            pltpu.VMEM((D, T), f32),
            pltpu.VMEM((S // T, DP // 2, T), u32),
            pltpu.VMEM((NSEG, H, 16, L), u32),
            pltpu.VMEM((NSEG, H, 24, L), f32),
            pltpu.VMEM((NSEG, NG, L // 2, T), u32),
            pltpu.VMEM((NSEG, D, L), f32),
            pltpu.VMEM((NG, G + 8, T), f32),
            pltpu.VMEM((D, T), f32),
            pltpu.VMEM((S // T, 8, T), f32),
            pltpu.VMEM((NSEG + 1, D, L), bf16),
            pltpu.VMEM((T, T), f32),
            pltpu.VMEM((len(RANGES), 8, T), u32),
            pltpu.SemaphoreType.DMA((7 + len(XPARTS),)),
        ],
        compiler_params=pltpu.CompilerParams(vmem_limit_bytes=100 * 2**20),
    )(A_x.reshape(S, D).T, A_wq, A_wk, A_wv, A_wo, A_beta.reshape(1, H), B_w_r,
      B_w_gate, B_w_up, B_w_down.T)
    return out.T.reshape(A_x.shape)
```

```python
import functools

import jax
import jax.numpy as jnp
import jax.experimental.pallas as pl
import jax.experimental.pallas.tpu as pltpu

S, D, H, DH, NSEG, L, F = 2048, 576, 32, 18, 4, 512, 4608
DP = 640
G = 4 * DH
NG = H // 4
T = 128
NT = L // T
NP = NG // 2
LATE = 2
DEFER_K = 2
PIN_P = 12
SLOTS3 = (0, 1, 2, 3, 4)
ROUTE_WAIT = 8
LNROWS0 = 144
LNROWS1 = 192
PIN_G = 2
PIN_A = 3
DIAG = True
LAG = 3
ORDER = ((3, 2), (3, 3), (3, 0), (0, 0), (3, 1), (2, 1), (2, 2), (2, 0), (1, 0), (1, 1))
SLOTS = ((0, 1, 2, 3, 4), (3, 4,), (2, 3, 4))
LNROWS = 96
LOG2E = 1.4426950408889634
QSCALE = DH ** -0.5 * LOG2E
NEG = -1e30
ONES_ROW = (23, 23, 0, 0)
XPARTS = ((0, 256), (256, 256), (512, 512), (1024, 1024))
RANGES = ((0, 32), (32, 64), (64, 96), (96, 128), (32, 128), (0, 64), (64, 128))

f32, bf16, u32 = jnp.float32, jnp.bfloat16, jnp.uint32
ALL = slice(None)


def _dot(a, b):
    return jnp.dot(a, b, preferred_element_type=f32)


def _dot_nt(a, b):
    return jax.lax.dot_general(a, b, (((1,), (1,)), ((), ())), preferred_element_type=f32)


def _rnd(a):
    return a.astype(bf16).astype(f32)


def _rcp(a):
    return pltpu.reciprocal(a, full_range=False)


def _iota(shape, axis):
    return jax.lax.broadcasted_iota(jnp.int32, shape, axis)


def _pad_to_tile(a):
    if a.shape[1] < T:
        a = jnp.concatenate([a, jnp.zeros((a.shape[0], T - a.shape[1]), a.dtype)], axis=1)
    if a.shape[0] < T:
        a = jnp.concatenate([a, jnp.zeros((T - a.shape[0], T), a.dtype)], axis=0)
    return a


def _phi(t):
    return jnp.where(t > 0, t + 1.0, jnp.exp(t))


def _head_of(i):
    return ((i >= DH).astype(jnp.int32) + (i >= 2 * DH).astype(jnp.int32)
            + (i >= 3 * DH).astype(jnp.int32) + (i >= 4 * DH).astype(jnp.int32))


class _Packed:
    def __init__(self, ref):
        self.words = ref

    def _index(self, idx):
        *lead, rows, cols = idx
        start, stop, _ = rows.indices(2 * self.words.shape[-2])
        return (*lead, slice(start // 2, stop // 2), cols)

    def __getitem__(self, idx):
        return pltpu.bitcast(self.words[self._index(idx)], bf16)

    def __setitem__(self, idx, value):
        self.words[self._index(idx)] = pltpu.bitcast(value, u32)


def run(gen):
    try:
        while True:
            next(gen)
    except StopIteration as stop:
        return stop.value


def _kernel(x_hbm, wq_hbm, wk_hbm, wv_hbm, wo_hbm, beta_hbm, wr_hbm, wg_hbm, wu_hbm,
            wd_hbm, o_hbm,
            x_v, w_v, beta_v, wr_v, wg_v, wu_v, wd_v, wt, wrc, xn_v, qm, vl, kn, ot, mst,
            gcol, r_v, hot, o_v, causal, lanes, sem):
    xn_v, qm, kn = (_Packed(r) for r in (xn_v, qm, kn))
    x_cp = [pltpu.make_async_copy(x_hbm.at[:, pl.ds(t, n)], x_v.at[:, pl.ds(t, n)], sem.at[7 + i])
            for i, (t, n) in enumerate(XPARTS)]
    w_cp = [pltpu.make_async_copy(w, w_v.at[i], sem.at[i]) if i else None
            for i, w in enumerate((wq_hbm, wk_hbm, wv_hbm, wo_hbm))]
    wq_cp = [pltpu.make_async_copy(wq_hbm.at[:, pl.ds(c, n)], w_v.at[0, :, pl.ds(c, n)], sm)
             for c, n, sm in ((0, 2 * T, sem.at[0]), (2 * T, D - 2 * T, sem.at[7 + len(XPARTS)]))]
    f_cp = [pltpu.make_async_copy(a, b, sem.at[4])
            for i, (a, b) in enumerate(((wg_hbm, wg_v), (wu_hbm, wu_v), (wd_hbm, wd_v)))]
    c_cp = [pltpu.make_async_copy(a, b, sem.at[5])
            for i, (a, b) in enumerate(((wr_hbm, wr_v), (beta_hbm, beta_v)))]
    o_cp = [[pltpu.make_async_copy(o_v.at[s, pl.ds(p * 2 * G, 2 * G)],
                                   o_hbm.at[pl.ds(p * 2 * G, 2 * G), pl.ds(s * L, L)],
                                   sem.at[6]) for p in range(NP)] for s in range(NSEG)]

    fillers = []

    lane8 = _iota((8, T), 1)
    never = lane8 < jnp.min(lane8, axis=1, keepdims=True)
    zero = jnp.min(lane8)
    link = [None, None]
    pins = []

    def opaque(ref, idx):
        ax = -1 if ref.shape[-1] > T else -2
        n = idx[ax].stop - idx[ax].start
        idx = list(idx)
        idx[ax] = pl.ds(pl.multiple_of(idx[ax].start + zero * n, n), n)
        return tuple(idx)

    def pin(ref, idx, steps):
        ref = ref.words if isinstance(ref, _Packed) else ref
        rows = 16 if ref.dtype == bf16 else 8
        pins.append([steps, ref, opaque(ref, (*idx, slice(0, rows), slice(0, T)))])

    def pinned_operand(a):
        for p in pins:
            p[0] -= 1
        due = [p for p in pins if p[0] < 0]
        if not due:
            return a
        pins[:] = [p for p in pins if p[0] >= 0]
        n = 16 if a.dtype == bf16 else 8
        t = pltpu.bitcast(a[-n:, -T:], u32)
        for _, ref, idx in due:
            t = tie(t, pltpu.bitcast(ref[idx], u32))
        return jnp.concatenate([a[:-n], pltpu.bitcast(t, a.dtype)], axis=0)

    def tie(a, b):
        return a if b is None else jnp.where(never, b, a)

    def fill(after=None):
        link[0], link[1] = after, None
        while fillers:
            if next(fillers[0], False):
                break
            fillers.pop(0)
        return link[1]

    def drain():
        while fillers:
            fill()

    def gate_column():
        gate = jax.nn.sigmoid(beta_v[...].astype(f32))
        gate = jnp.concatenate([gate, jnp.zeros((1, T - H), f32)], axis=1)
        gate = jnp.broadcast_to(gate, (T, T)).T
        r8 = _iota((8, T), 0)
        for v in range(D // 8):
            h0, h1 = (8 * v) // DH, (8 * v + 7) // DH
            gv = jnp.broadcast_to(gate[h0:h0 + 1], (8, T))
            if h1 != h0:
                gv = jnp.where(r8 < h1 * DH - 8 * v, gv, jnp.broadcast_to(gate[h1:h1 + 1], (8, T)))
            gcol[8 * v:8 * v + 8, :] = gv
            if v % 9 == 8:
                yield True

    def router_column():
        wr = wr_v[...].astype(f32).reshape(1, D)
        wr = jnp.concatenate([wr, jnp.zeros((1, DP - D), f32)], axis=1)
        wrc[...] = jnp.broadcast_to(wr, (T, DP)).T[0:D]

    def transpose_w(i, lo=0, hi=D):
        for c in range(lo, hi, T):
            n = min(T, D - c)
            for k in range(0, D, T):
                w = _pad_to_tile(w_v[i, k:min(k + T, D), c:c + n].astype(f32))
                w = jnp.concatenate([tie(w[r:r + 8], link[0]) for r in range(0, T, 8)], axis=0).T
                wt[i, c:c + n, k:k + T] = w[0:n]
                if k + T >= D and i == 3:
                    pin(wt, (i,), PIN_P)
                yield True

    normed = [0]

    def layernorm(b, step):

        def chain(acc, v):
            h = v.shape[0] // 16 * 8
            a, c = v[0:8], v[h:h + 8]
            for k in range(8, h, 8):
                a, c = a + v[k:k + 8], c + v[h + k:h + k + 8]
            return a + c if acc is None else acc + (a + c)

        def rows(v):
            return jnp.concatenate([tie(v, link[0])] * (step // 8), axis=0)

        def bcast(v):
            return jnp.broadcast_to(v, (8, T))

        def load(r, n):
            return x_v[r:r + step, pl.ds(pl.multiple_of((b + n * zero) * T, T), T)].astype(f32)

        acc = jnp.zeros((8, T), f32)
        for r in range(0, D, step):
            x = load(r, 0)
            link[1] = acc = chain(tie(acc, link[0]), x)
            yield True
        mean = bcast(jnp.sum(acc, axis=0, keepdims=True) * (1.0 / D))
        acc = None
        for r in range(0, D, step):
            xc = load(r, 1) - rows(mean)
            link[1] = acc = chain(acc, xc * xc)
            yield True
        var = bcast(jnp.sum(acc, axis=0, keepdims=True) * (1.0 / D))
        sd = _rnd(jnp.sqrt(_rnd(_rnd(var) + _rnd(jnp.full((8, T), 1e-5, f32)))))
        inv, mean = jnp.concatenate([1.0 / sd] * (step // 8), axis=0), _rnd(mean)
        acc = None
        for r in range(0, D, step):
            x = load(r, 2)
            xn = (_rnd(x - rows(mean)) * inv).astype(bf16)
            xn_v[b, r:r + step, :] = xn
            link[1] = acc = chain(acc, xn.astype(f32) * wrc[r:r + step, :])
            if r + step == D:
                xn_v[b, D:DP, :] = jnp.zeros((DP - D, T), bf16)
                r_v[b:b + 1, :] = _rnd(jnp.sum(acc, axis=0, keepdims=True))
                normed[0] += 1
            yield True

    late = [None] * LATE
    deferred = []

    def flush():
        while deferred:
            deferred.pop(0)()

    def proj(i, s, g, slots):
        acc = None
        for k in range(0, DP, T):
            xs = jnp.concatenate([xn_v[s * NT + c, k:k + T, :] for c in range(NT)], axis=1)
            w = wt[i, g * G:(g + 1) * G, k:k + T]
            d = _dot(pinned_operand(w), xs)
            done = late.pop(0)
            top = tie(d[-8:, :T], done)
            d = jnp.concatenate([d[:-8], jnp.concatenate([top, d[-8:, T:]], axis=1)], axis=0)
            acc = d if acc is None else acc + d
            late.append(fill(d[0:8, 0:T]) if k // T in slots else None)
        yield 5 * G
        while deferred:
            deferred.pop(0)()
            yield G + 8
        return acc

    def project_q(s, g):
        q = yield from proj(0, s, g, SLOTS[0] if s < 3 else SLOTS3)
        r8 = _iota((8, L), 0)
        qs = q * QSCALE
        for h in range(4):
            lo = 16 * h
            a0, a1, a2 = qs[lo:lo + 8], qs[lo + 8:lo + 16], qs[lo + 16:lo + 24]
            if h > 0:
                a0 = jnp.where(r8 >= 2 * h, a0, 0.0)
            if h < 3:
                a2 = jnp.where(r8 < 2 * h + 2, a2, 0.0)
            qm[s, 4 * g + h, :, :] = jnp.concatenate(
                [a0, a1, a2, jnp.zeros((8, L), f32)], axis=0).astype(bf16)
        if s > 0:
            pq = jnp.concatenate([_phi(q), jnp.zeros((T - G, L), f32)], axis=0).astype(bf16)
            deferred.append(functools.partial(memory_read, s, g, pq))

    def memory_read(s, g, pq):
        r8 = _iota((8, L), 0)
        mrow = _iota((G + 8, T), 0)
        mkeep = jnp.where(mrow < G, _head_of(mrow), mrow - G) == _head_of(_iota((G + 8, T), 1))
        nd = _dot(jnp.where(mkeep, mst[g], 0.0).astype(bf16), pq)
        inv = _rcp(nd[G:] + 1e-6)
        ib = [jnp.broadcast_to(inv[h:h + 1], (8, L)) for h in range(4)]
        iv = jnp.concatenate(
            [ib[0], ib[0], jnp.where(r8 < 2, ib[0], ib[1]), ib[1],
             jnp.where(r8 < 4, ib[1], ib[2]), ib[2],
             jnp.where(r8 < 6, ib[2], ib[3]), ib[3], ib[3]], axis=0)
        gg = gcol[g * G:(g + 1) * G, :]
        ot[s, g * G:(g + 1) * G, :] = nd[:G] * iv * jnp.concatenate([gg] * NT, axis=1)

    def memory_update(s, g, v80, pk):
        upd = _dot_nt(v80, pk)
        mst[g] = upd if s == 0 else mst[g] + upd

    def project_k(s, g):
        k = yield from proj(1, s, g, SLOTS3 if s == 3 else SLOTS[1] if s else SLOTS[2])
        zpad = jnp.zeros((T - G, L), f32)
        kn[s, g, :, :] = jnp.concatenate([k, zpad], axis=0).astype(bf16).T
        if s < NSEG - 1:
            return jnp.concatenate([_phi(k), zpad], axis=0).astype(bf16)

    def project_v(s, g, pk):
        v = yield from proj(2, s, g, SLOTS3 if s == 3 else SLOTS[2] if s else SLOTS[0])
        for h in range(4):
            a = [v[16 * h + c:16 * h + c + 8] for c in (0, 8, 16)]
            c, r = divmod(ONES_ROW[h], 8)
            a[c] = jnp.where(_iota((8, L), 0) == r, 1.0, a[c])
            vl[s, 4 * g + h] = jnp.concatenate(a, axis=0)
        if pk is not None:
            v80 = jnp.concatenate([v, jnp.ones((8, L), f32)], axis=0)
            deferred.append(functools.partial(memory_update, s, g, v80, pk))
        if g % PIN_G == PIN_G - 1:
            for ref in (qm, kn, vl):
                pin(ref, (s, 0), PIN_P)
            if s:
                pin(ot, (s,), PIN_P)

    def attention():
        r8 = _iota((8, T), 0)
        units = [(s, g, i, j) for s in range(NSEG) for g in range(NG) for i, j in ORDER]
        run, accs = {}, {}

        lane32 = _iota((32, T), 1)
        carry = {}

        def own_queries(s, g, i):
            w = []
            for h in range(4):
                parts = [qm[s, 4 * g + h, :, i * T:(i + 1) * T]]
                if h > 0:
                    parts.insert(0, jnp.zeros((16 * h, T), bf16))
                parts.append(jnp.zeros((T - 32 - 16 * h, T), bf16))
                w.append(jnp.concatenate(parts, axis=0))
            return jnp.concatenate(w, axis=1)

        def shared_queries(qw, *parts):
            slots = [None] * 8
            for h, shift, lo, hi in parts:
                q = pltpu.roll(qw[h], shift, 1) if shift else qw[h]
                for e in range(2):
                    t = q[8 * e:8 * e + 8] & lanes[RANGES.index((lo, hi))]
                    slots[h + e] = t if slots[h + e] is None else t | slots[h + e]
            slots = [jnp.zeros((8, T), u32) if t is None else t for t in slots]
            return pltpu.bitcast(jnp.concatenate(slots, axis=0), bf16)

        def diagonal_scores(s, g, i):
            k0 = i * T
            own = carry.pop("own") if i else _dot(kn[s, g, 0:32, :], own_queries(s, g, 0))
            qw = [qm.words[s, 4 * g + h, :, k0:k0 + T] for h in range(4)]
            x = _dot(kn[s, g, k0 + 32:k0 + 64, :], jnp.concatenate(
                [shared_queries(qw, (h, 0, 32, T), (3, 96 - 32 * h, 0, 32)) for h in range(3)],
                axis=1))
            y = _dot(kn[s, g, k0 + 64:k0 + 96, :], jnp.concatenate(
                [shared_queries(qw, (h, 0, 64, T), (h + 1, 64, 0, 64)) for h in (0, 2)], axis=1))
            z = _dot(kn[s, g, k0 + 96:k0 + T, :], shared_queries(
                qw, *[(h, (32 * h + 32) % T, 32 * h, 32 * h + 32) for h in range(4)]))
            xs = [x[:, h * T:(h + 1) * T] for h in range(3)]
            xr = [pltpu.roll(xs[h], 32 * h + 32, 1) for h in range(3)]
            xs.append(jnp.where(lane32 < 64, xr[0], jnp.where(lane32 < 96, xr[1], xr[2])))
            ys = [y[:, :T], pltpu.roll(y[:, :T], 64, 1), y[:, T:], pltpu.roll(y[:, T:], 64, 1)]
            zs = [pltpu.roll(z, 96 - 32 * h, 1) for h in range(3)] + [z]
            return [jnp.concatenate([own[:, h * T:(h + 1) * T], xs[h], ys[h], zs[h]], axis=0)
                    for h in range(4)]

        def scores(s, g, i, j):
            if DIAG and i == j:
                shs = diagonal_scores(s, g, i)
            else:
                more = 32 if DIAG and j == i - 1 else 0
                st = _dot(pinned_operand(kn[s, g, j * T:(j + 1) * T + more, :]),
                          own_queries(s, g, i))
                if more:
                    carry["own"] = st[T:]
                shs = [st[:T, h * T:(h + 1) * T] for h in range(4)]
            ps, alphas = [], []
            later = any(a == i for a, _ in ORDER[:ORDER.index((i, j))])
            for h in range(4):
                sh = shs[h]
                if i == j:
                    sh = sh + causal[...]
                m = jnp.max(sh, axis=0, keepdims=True)
                if later:
                    m = jnp.maximum(m, run[i, h])
                    alphas.append(jnp.exp2(run[i, h] - m))
                run[i, h] = m
                ps.append(jnp.exp2(sh - m).astype(bf16))
            return ps, alphas

        def values(s, g, i, j, ps, alphas):
            new = [_dot(vl[s, 4 * g + h, :, j * T:(j + 1) * T], ps[h]) for h in range(4)]
            if alphas:
                new = [a * al + b for a, al, b in zip(accs.pop(i), alphas, new)]
            if any(a == i for a, _ in ORDER[ORDER.index((i, j)) + 1:]):
                accs[i] = new
                return
            o = []
            for h in range(4):
                inv = _rcp(jnp.broadcast_to(new[h][ONES_ROW[h]:ONES_ROW[h] + 1], (8, T)))
                o.append([new[h][8 * c:8 * c + 8] * inv for c in range(3)])
            a_dot = jnp.concatenate(
                [o[0][0], o[0][1], jnp.where(r8 < 2, o[0][2], o[1][0]), o[1][1],
                 jnp.where(r8 < 4, o[1][2], o[2][0]), o[2][1],
                 jnp.where(r8 < 6, o[2][2], o[3][0]), o[3][1], o[3][2]], axis=0)
            dst = (s, slice(g * G, (g + 1) * G), slice(i * T, (i + 1) * T))
            mix = (1.0 - gcol[g * G:(g + 1) * G, :]) * a_dot
            ot[dst] = ot[dst] + mix if s > 0 else mix
            if (i, j) == ORDER[-1] and g % PIN_G == PIN_G - 1:
                pin(ot, (s,), PIN_A)

        pend = {}
        for t in range(len(units) + LAG):
            if t < len(units):
                pend[t] = scores(*units[t])
            if t >= LAG:
                values(*units[t - LAG], *pend.pop(t - LAG))
            yield t < len(units) and units[t][2] != units[t][3]

    def out_proj(s):
        o = jnp.concatenate(
            [ot[s], hot[:, s * L:(s + 1) * L], jnp.zeros((DP - D - 8, L), f32)], axis=0).astype(bf16)
        for p in range(NP):
            rows = slice(p * 2 * G, (p + 1) * 2 * G)
            halves = []
            for g in (2 * p, 2 * p + 1):
                a = None
                for k in range(0, DP, T):
                    d = _dot(pinned_operand(wt[3, g * G:(g + 1) * G, k:k + T]), o[k:k + T])
                    a = d if a is None else a + d
                halves.append(a)
                yield 5 * G
            a = jnp.concatenate(halves, axis=0)
            for c in range(NT):
                b = s * NT + c
                res = x_v[rows, b * T:(b + 1) * T].astype(f32) + xn_v[b, rows, :].astype(f32)
                o_v[s, rows, c * T:(c + 1) * T] = (res + a[:, c * T:(c + 1) * T]).astype(bf16)
            o_cp[s][p].start()
            spare = (NSEG, slice(0, 16), slice(0, T))
            o_v[opaque(o_v, spare)] = jnp.zeros((16, T), bf16)
            pin(o_v, (NSEG,), PIN_P)

    routed = {}

    def row_block(ref, k, cols):
        w = ref[k:min(k + T, D), cols]
        if k + T > D:
            w = jnp.concatenate([w, jnp.zeros((DP - D, w.shape[1]), bf16)], axis=0)
        return w

    def route():
        def both(op, a):
            return op(op(a, axis=0, keepdims=True), axis=1, keepdims=True)

        r = r_v[...]
        idx = (_iota(r.shape, 0) * T + _iota(r.shape, 1)).astype(f32)
        m1 = both(jnp.max, r)
        i1 = both(jnp.min, jnp.where(r == m1, idx, S))
        r = jnp.where(idx == i1, -jnp.inf, r)
        m2 = both(jnp.max, r)
        i2 = both(jnp.min, jnp.where((r == m2) & (idx != i1), idx, S))
        row = _iota((8, T), 0)
        routed["w"] = jax.nn.sigmoid(jnp.where(row == 0, m1, m2))
        pick = jnp.where(row == 0, i1, jnp.where(row == 1, i2, -1.0))
        for b in range(S // T):
            hot[:, b * T:(b + 1) * T] = (pick == (lane8 + b * T).astype(f32)).astype(f32)
        blocks = [jnp.clip(jnp.max(i).astype(jnp.int32) >> 7, 0, S // T - 1) for i in (i1, i2)]
        for _ in range(ROUTE_WAIT):
            yield True
        x = None
        for n, b in enumerate(blocks):
            pick = jnp.where(row == n, hot[:, pl.ds(pl.multiple_of(b * T, T), T)], 0.0)
            d = _dot_nt(pick, xn_v[b, :, :])
            x = d if x is None else x + d
            yield True
        routed["x"] = [x[:, k:k + T] for k in range(0, DP, T)]

    def ffn_hidden():
        routed["h"] = []
        for n in range(0, F, L):
            gu = []
            for w_ref in (wg_v, wu_v):
                acc = None
                for c, k in enumerate(range(0, D, T)):
                    d = _dot(routed["x"][c], row_block(w_ref, k, slice(n, n + L)))
                    acc = d if acc is None else acc + d
                    yield True
                gu.append(acc)
            routed["h"].append(gu[0] * jax.nn.sigmoid(gu[0]) * gu[1])

    def ffn_down():
        for k in range(0, D, T):
            acc = None
            for c, n in enumerate(range(0, F, L)):
                d = _dot_nt(routed["h"][c], row_block(wd_v, k, slice(n, n + L)))
                acc = d if acc is None else acc + d
                yield
            y = jnp.concatenate([jnp.zeros((D - 4 * T, T), f32), acc * routed["w"],
                                 jnp.zeros((DP - D - 8, T), f32)], axis=0).T
            dst = (3, slice(k, min(k + T, D)), slice(4 * T, DP))
            wt[dst] = wt[dst] + y[0:min(T, D - k)]
            pin(wt, (3,), PIN_A)

    for c in (*c_cp, *x_cp[:2], *wq_cp, *w_cp[1:3]):
        c.start()
    causal[...] = jnp.where(_iota((T, T), 0) <= _iota((T, T), 1), 0.0, NEG)
    for n, (lo, hi) in enumerate(RANGES):
        lanes[n] = pltpu.bitcast(jnp.where((lane8 >= lo) & (lane8 < hi), -1, 0), u32)
    for c in c_cp:
        c.wait()
    router_column()
    for _ in gate_column():
        pass
    for b in range(NT):
        if b % 2 == 0:
            x_cp[b // 2].wait()
        fillers.append(layernorm(b, LNROWS0))
        prev = [None, None]
        while fillers:
            prev.append(fill(prev.pop(0)))
    x_cp[2].start()
    wq_cp[0].wait()
    fillers.append(transpose_w(0, 0, 2 * T))
    drain()
    for p in range(NG):
        if p == 2:
            wq_cp[1].wait()
            fillers.append(transpose_w(0, 2 * T))
            drain()
        if p == NG - 1:
            for c in (x_cp[3], w_cp[3]):
                c.start()
            w_cp[1].wait()
            fillers.append(transpose_w(1))
            drain()
        run(project_q(0, p))
    pks = []
    for p in range(NG):
        if p == NG - 1:
            for ref in (wg_v, wu_v, wd_v):
                ref[0:16, 0:T] = kn[0, 0, 0:16, :]
            for c in f_cp:
                c.start()
            for c in (w_cp[2], x_cp[2]):
                c.wait()
            fillers.append(transpose_w(2))
            drain()
            fillers.extend(layernorm(b, LNROWS1) for b in range(NT, 2 * NT))
        pks.append(run(project_k(0, p)))
    for p in range(NG):
        run(project_v(0, p, pks[p]))
    drain()
    def dense(s):
        while normed[0] < (s + 1) * NT:
            fill()
        for p in range(NG):
            yield from project_q(s, p)
            if s == 1 and p == 0:
                for c in (x_cp[3], w_cp[3]):
                    c.wait()
                fillers.extend(layernorm(b, LNROWS) for b in range(2 * NT, S // T))
                fillers.append(transpose_w(3))
            if s == NSEG - 1 and p == 0:
                fillers.append(route())
            if s == NSEG - 1 and p == 1:
                drain()
                for c in f_cp:
                    c.wait()
                fillers.append(ffn_hidden())
            yield from project_v(s, p, (yield from project_k(s, p)))

    def weave(main, steps, other, rows, extra=iter(())):
        done = 0
        for t in range(steps):
            if next(main):
                next(extra, None)
            while done < (t + 1) * rows // steps:
                done += next(other, rows)
        run(other)

    per_seg = NG * len(ORDER)
    seg_rows = NP * (15 * 2 * G + 4 * (G + 8))
    att = attention()
    run(dense(1))
    run(dense(2))
    while normed[0] < S // T:
        fill()
    weave(att, per_seg, iter(()), 0)
    run(dense(3))
    drain()
    steps = ffn_down()
    weave(att, per_seg, iter(()), 0, steps)
    run(steps)
    outs = (n for s in range(NSEG - 1) for n in out_proj(s))
    weave(att, 2 * per_seg + LAG, outs, 3 * NP * 5 * 2 * G - 15 * G)
    run(out_proj(NSEG - 1))
    for cs in o_cp:
        for c in cs:
            c.wait()


@jax.jit
def pallas_parallel_sum__memory_aug_infini_attn__moe_arch_mod__prompt_kernel(
    A_x: jax.Array,
    A_wq: jax.Array,
    A_wk: jax.Array,
    A_wv: jax.Array,
    A_wo: jax.Array,
    A_beta: jax.Array,
    B_x: jax.Array,
    B_w_r: jax.Array,
    B_w_gate: jax.Array,
    B_w_up: jax.Array,
    B_w_down: jax.Array,
):
    del B_x
    hbm = pl.BlockSpec(memory_space=pltpu.HBM)
    out = pl.pallas_call(
        _kernel,
        out_shape=jax.ShapeDtypeStruct((D, S), A_x.dtype),
        in_specs=[hbm] * 10,
        out_specs=hbm,
        scratch_shapes=[
            pltpu.VMEM((D, S), bf16),
            pltpu.VMEM((4, D, D), bf16),
            pltpu.VMEM((1, H), bf16),
            pltpu.VMEM((D,), bf16),
            pltpu.VMEM((D, F), bf16),
            pltpu.VMEM((D, F), bf16),
            pltpu.VMEM((D, F), bf16),
            pltpu.VMEM((4, D, DP), f32),
            pltpu.VMEM((D, T), f32),
            pltpu.VMEM((S // T, DP // 2, T), u32),
            pltpu.VMEM((NSEG, H, 16, L), u32),
            pltpu.VMEM((NSEG, H, 24, L), f32),
            pltpu.VMEM((NSEG, NG, L // 2, T), u32),
            pltpu.VMEM((NSEG, D, L), f32),
            pltpu.VMEM((NG, G + 8, T), f32),
            pltpu.VMEM((D, T), f32),
            pltpu.VMEM((S // T, T), f32),
            pltpu.VMEM((8, S), f32),
            pltpu.VMEM((NSEG + 1, D, L), bf16),
            pltpu.VMEM((T, T), f32),
            pltpu.VMEM((len(RANGES), 8, T), u32),
            pltpu.SemaphoreType.DMA((8 + len(XPARTS),)),
        ],
        compiler_params=pltpu.CompilerParams(vmem_limit_bytes=100 * 2**20),
    )(A_x.reshape(S, D).T, A_wq, A_wk, A_wv, A_wo, A_beta.reshape(1, H), B_w_r,
      B_w_gate, B_w_up, B_w_down.T)
    return out.T.reshape(A_x.shape)
```

```python
import functools

import jax
import jax.numpy as jnp
import jax.experimental.pallas as pl
import jax.experimental.pallas.tpu as pltpu

S, D, H, DH, NSEG, L, F = 2048, 576, 32, 18, 4, 512, 4608
DP = 640
G = 4 * DH
NG = H // 4
T = 128
NT = L // T
NP = NG // 2
LATE = 2
FWAIT = 1
SLOTS2 = ((), (2,), (1,))
TAIL = 30
DEFER_K = 2
PIN_P = 12
SLOTS3 = (0, 1, 2, 3, 4)
ROUTE_WAIT = 5
LNROWS0 = 144
LNROWS1 = 192
PIN_G = 8
PIN_A = 7
DIAG = True
LAG = 3
ORDER = ((3,0),(0,0),(3,1),(1,0),(1,1),(2,0),(3,2),(3,3),(2,1),(2,2))
SLOTS = ((0, 1, 2, 3, 4), (3, 4,), (2, 3, 4))
LNROWS = 96
LOG2E = 1.4426950408889634
QSCALE = DH ** -0.5 * LOG2E
NEG = -1e30
ONES_ROW = (23, 23, 0, 0)
XPARTS = ((0, 256), (256, 256), (512, 512), (1024, 1024))
RANGES = ((0, 32), (32, 64), (64, 96), (96, 128), (32, 128), (0, 64), (64, 128))

f32, bf16, u32 = jnp.float32, jnp.bfloat16, jnp.uint32
ALL = slice(None)


def _dot(a, b):
    return jnp.dot(a, b, preferred_element_type=f32)


def _dot_nt(a, b):
    return jax.lax.dot_general(a, b, (((1,), (1,)), ((), ())), preferred_element_type=f32)


def _rnd(a):
    return a.astype(bf16).astype(f32)


def _rcp(a):
    return pltpu.reciprocal(a, full_range=False)


def _iota(shape, axis):
    return jax.lax.broadcasted_iota(jnp.int32, shape, axis)


def _pad_to_tile(a):
    if a.shape[1] < T:
        a = jnp.concatenate([a, jnp.zeros((a.shape[0], T - a.shape[1]), a.dtype)], axis=1)
    if a.shape[0] < T:
        a = jnp.concatenate([a, jnp.zeros((T - a.shape[0], T), a.dtype)], axis=0)
    return a


def _phi(t):
    return jnp.where(t > 0, t + 1.0, jnp.exp(t))


def _head_of(i):
    return ((i >= DH).astype(jnp.int32) + (i >= 2 * DH).astype(jnp.int32)
            + (i >= 3 * DH).astype(jnp.int32) + (i >= 4 * DH).astype(jnp.int32))


class _Packed:
    def __init__(self, ref):
        self.words = ref

    def _index(self, idx):
        *lead, rows, cols = idx
        start, stop, _ = rows.indices(2 * self.words.shape[-2])
        return (*lead, slice(start // 2, stop // 2), cols)

    def __getitem__(self, idx):
        return pltpu.bitcast(self.words[self._index(idx)], bf16)

    def __setitem__(self, idx, value):
        self.words[self._index(idx)] = pltpu.bitcast(value, u32)


def run(gen):
    try:
        while True:
            next(gen)
    except StopIteration as stop:
        return stop.value


def _kernel(x_hbm, wq_hbm, wk_hbm, wv_hbm, wo_hbm, beta_hbm, wr_hbm, wg_hbm, wu_hbm,
            wd_hbm, o_hbm,
            x_v, w_v, beta_v, wr_v, wg_v, wu_v, wd_v, wt, wrc, xn_v, qm, vl, kn, ot, mst,
            gcol, r_v, hot, o_v, causal, lanes, sem):
    xn_v, qm, kn = (_Packed(r) for r in (xn_v, qm, kn))
    x_cp = [pltpu.make_async_copy(x_hbm.at[:, pl.ds(t, n)], x_v.at[:, pl.ds(t, n)], sem.at[7 + i])
            for i, (t, n) in enumerate(XPARTS)]
    w_cp = [pltpu.make_async_copy(w, w_v.at[i], sem.at[i]) if i else None
            for i, w in enumerate((wq_hbm, wk_hbm, wv_hbm, wo_hbm))]
    wq_cp = [pltpu.make_async_copy(wq_hbm.at[:, pl.ds(c, n)], w_v.at[0, :, pl.ds(c, n)], sm)
             for c, n, sm in ((0, 2 * T, sem.at[0]), (2 * T, D - 2 * T, sem.at[7 + len(XPARTS)]))]
    f_cp = [pltpu.make_async_copy(a, b, sem.at[4])
            for i, (a, b) in enumerate(((wg_hbm, wg_v), (wu_hbm, wu_v), (wd_hbm, wd_v)))]
    c_cp = [pltpu.make_async_copy(a, b, sem.at[5])
            for i, (a, b) in enumerate(((wr_hbm, wr_v), (beta_hbm, beta_v)))]
    o_cp = [[pltpu.make_async_copy(o_v.at[s, pl.ds(p * 2 * G, 2 * G)],
                                   o_hbm.at[pl.ds(p * 2 * G, 2 * G), pl.ds(s * L, L)],
                                   sem.at[6]) for p in range(NP)] for s in range(NSEG)]

    fillers = []

    lane8 = _iota((8, T), 1)
    never = lane8 < jnp.min(lane8, axis=1, keepdims=True)
    zero = jnp.min(lane8)
    link = [None, None]
    pins = []

    def opaque(ref, idx):
        ax = -1 if ref.shape[-1] > T else -2
        n = idx[ax].stop - idx[ax].start
        idx = list(idx)
        idx[ax] = pl.ds(pl.multiple_of(idx[ax].start + zero * n, n), n)
        return tuple(idx)

    def pin(ref, idx, steps):
        ref = ref.words if isinstance(ref, _Packed) else ref
        rows = 16 if ref.dtype == bf16 else 8
        pins.append([steps, ref, opaque(ref, (*idx, slice(0, rows), slice(0, T)))])

    def pinned_operand(a):
        for p in pins:
            p[0] -= 1
        due = [p for p in pins if p[0] < 0]
        if not due:
            return a
        pins[:] = [p for p in pins if p[0] >= 0]
        n = 16 if a.dtype == bf16 else 8
        t = pltpu.bitcast(a[-n:, -T:], u32)
        for _, ref, idx in due:
            t = tie(t, pltpu.bitcast(ref[idx], u32))
        return jnp.concatenate([a[:-n], pltpu.bitcast(t, a.dtype)], axis=0)

    def tie(a, b):
        return a if b is None else jnp.where(never, b, a)

    def fill(after=None):
        link[0], link[1] = after, None
        while fillers:
            if next(fillers[0], False):
                break
            fillers.pop(0)
        return link[1]

    def drain():
        while fillers:
            fill()

    def gate_column():
        gate = jax.nn.sigmoid(beta_v[...].astype(f32))
        gate = jnp.concatenate([gate, jnp.zeros((1, T - H), f32)], axis=1)
        gate = jnp.broadcast_to(gate, (T, T)).T
        r8 = _iota((8, T), 0)
        for v in range(D // 8):
            h0, h1 = (8 * v) // DH, (8 * v + 7) // DH
            gv = jnp.broadcast_to(gate[h0:h0 + 1], (8, T))
            if h1 != h0:
                gv = jnp.where(r8 < h1 * DH - 8 * v, gv, jnp.broadcast_to(gate[h1:h1 + 1], (8, T)))
            gcol[8 * v:8 * v + 8, :] = gv
            if v % 9 == 8:
                yield True

    def router_column():
        wr = wr_v[...].astype(f32).reshape(1, D)
        wr = jnp.concatenate([wr, jnp.zeros((1, DP - D), f32)], axis=1)
        wrc[...] = jnp.broadcast_to(wr, (T, DP)).T[0:D]

    def transpose_w(i, lo=0, hi=D):
        for c in range(lo, hi, T):
            n = min(T, D - c)
            for k in range(0, D, T):
                w = _pad_to_tile(w_v[i, k:min(k + T, D), c:c + n].astype(f32))
                w = jnp.concatenate([tie(w[r:r + 8], link[0]) for r in range(0, T, 8)], axis=0).T
                wt[i, c:c + n, k:k + T] = w[0:n]
                if k + T >= D and i == 3:
                    pin(wt, (i,), PIN_P)
                yield True

    normed = [0]

    def layernorm(b, step):

        def chain(acc, v):
            h = v.shape[0] // 16 * 8
            a, c = v[0:8], v[h:h + 8]
            for k in range(8, h, 8):
                a, c = a + v[k:k + 8], c + v[h + k:h + k + 8]
            return a + c if acc is None else acc + (a + c)

        def rows(v):
            return jnp.concatenate([tie(v, link[0])] * (step // 8), axis=0)

        def bcast(v):
            return jnp.broadcast_to(v, (8, T))

        def load(r, n):
            return x_v[r:r + step, pl.ds(pl.multiple_of((b + n * zero) * T, T), T)].astype(f32)

        acc = jnp.zeros((8, T), f32)
        for r in range(0, D, step):
            x = load(r, 0)
            link[1] = acc = chain(tie(acc, link[0]), x)
            yield True
        mean = bcast(jnp.sum(acc, axis=0, keepdims=True) * (1.0 / D))
        acc = None
        for r in range(0, D, step):
            xc = load(r, 1) - rows(mean)
            link[1] = acc = chain(acc, xc * xc)
            yield True
        var = bcast(jnp.sum(acc, axis=0, keepdims=True) * (1.0 / D))
        sd = _rnd(jnp.sqrt(_rnd(_rnd(var) + _rnd(jnp.full((8, T), 1e-5, f32)))))
        inv, mean = jnp.concatenate([1.0 / sd] * (step // 8), axis=0), _rnd(mean)
        acc = None
        for r in range(0, D, step):
            x = load(r, 2)
            xn = (_rnd(x - rows(mean)) * inv).astype(bf16)
            xn_v[b, r:r + step, :] = xn
            link[1] = acc = chain(acc, xn.astype(f32) * wrc[r:r + step, :])
            if r + step == D:
                xn_v[b, D:DP, :] = jnp.zeros((DP - D, T), bf16)
                r_v[b:b + 1, :] = _rnd(jnp.sum(acc, axis=0, keepdims=True))
                normed[0] += 1
            yield True

    late = [None] * LATE
    deferred = []
    small = []

    def flush():
        while deferred:
            deferred.pop(0)()

    def proj(i, s, g, slots):
        acc = None
        for k in range(0, DP, T):
            xs = jnp.concatenate([xn_v[s * NT + c, k:k + T, :] for c in range(NT)], axis=1)
            w = wt[i, g * G:(g + 1) * G, k:k + T]
            d = _dot(pinned_operand(w), xs)
            done = late.pop(0)
            top = tie(d[-8:, :T], done)
            d = jnp.concatenate([d[:-8], jnp.concatenate([top, d[-8:, T:]], axis=1)], axis=0)
            acc = d if acc is None else acc + d
            late.append(fill(d[0:8, 0:T]) if k // T in slots else None)
            if small and k // T in (SLOTS3 if s == 3 else SLOTS2[i]):
                next(small[0], None)
        yield 5 * G
        while deferred:
            deferred.pop(0)()
            yield G + 8
        return acc

    def project_q(s, g):
        q = yield from proj(0, s, g, SLOTS[0])
        r8 = _iota((8, L), 0)
        qs = q * QSCALE
        for h in range(4):
            lo = 16 * h
            a0, a1, a2 = qs[lo:lo + 8], qs[lo + 8:lo + 16], qs[lo + 16:lo + 24]
            if h > 0:
                a0 = jnp.where(r8 >= 2 * h, a0, 0.0)
            if h < 3:
                a2 = jnp.where(r8 < 2 * h + 2, a2, 0.0)
            qm[s, 4 * g + h, :, :] = jnp.concatenate(
                [a0, a1, a2, jnp.zeros((8, L), f32)], axis=0).astype(bf16)
        if s > 0:
            pq = jnp.concatenate([_phi(q), jnp.zeros((T - G, L), f32)], axis=0).astype(bf16)
            deferred.append(functools.partial(memory_read, s, g, pq))

    def memory_read(s, g, pq):
        r8 = _iota((8, L), 0)
        mrow = _iota((G + 8, T), 0)
        mkeep = jnp.where(mrow < G, _head_of(mrow), mrow - G) == _head_of(_iota((G + 8, T), 1))
        nd = _dot(jnp.where(mkeep, mst[g], 0.0).astype(bf16), pq)
        inv = _rcp(nd[G:] + 1e-6)
        ib = [jnp.broadcast_to(inv[h:h + 1], (8, L)) for h in range(4)]
        iv = jnp.concatenate(
            [ib[0], ib[0], jnp.where(r8 < 2, ib[0], ib[1]), ib[1],
             jnp.where(r8 < 4, ib[1], ib[2]), ib[2],
             jnp.where(r8 < 6, ib[2], ib[3]), ib[3], ib[3]], axis=0)
        gg = gcol[g * G:(g + 1) * G, :]
        ot[s, g * G:(g + 1) * G, :] = nd[:G] * iv * jnp.concatenate([gg] * NT, axis=1)

    def memory_update(s, g, v80, pk):
        upd = _dot_nt(v80, pk)
        mst[g] = upd if s == 0 else mst[g] + upd

    def project_k(s, g):
        k = yield from proj(1, s, g, SLOTS[1] if s else SLOTS[2])
        zpad = jnp.zeros((T - G, L), f32)
        kn[s, g, :, :] = jnp.concatenate([k, zpad], axis=0).astype(bf16).T
        if s < NSEG - 1:
            return jnp.concatenate([_phi(k), zpad], axis=0).astype(bf16)

    def project_v(s, g, pk):
        v = yield from proj(2, s, g, SLOTS[2] if s else SLOTS[0])
        for h in range(4):
            a = [v[16 * h + c:16 * h + c + 8] for c in (0, 8, 16)]
            c, r = divmod(ONES_ROW[h], 8)
            a[c] = jnp.where(_iota((8, L), 0) == r, 1.0, a[c])
            vl[s, 4 * g + h] = jnp.concatenate(a, axis=0)
        if pk is not None:
            v80 = jnp.concatenate([v, jnp.ones((8, L), f32)], axis=0)
            deferred.append(functools.partial(memory_update, s, g, v80, pk))
        if g % PIN_G == PIN_G - 1:
            for ref in (qm, kn, vl):
                pin(ref, (s, 0), PIN_P)
            if s:
                pin(ot, (s,), PIN_P)

    def attention(segs):
        r8 = _iota((8, T), 0)
        units = [(s, g, i, j) for s in segs for g in range(NG) for i, j in ORDER]
        run, accs = {}, {}

        lane32 = _iota((32, T), 1)
        carry = {}

        def own_queries(s, g, i):
            w = []
            for h in range(4):
                parts = [qm[s, 4 * g + h, :, i * T:(i + 1) * T]]
                if h > 0:
                    parts.insert(0, jnp.zeros((16 * h, T), bf16))
                parts.append(jnp.zeros((T - 32 - 16 * h, T), bf16))
                w.append(jnp.concatenate(parts, axis=0))
            return jnp.concatenate(w, axis=1)

        def shared_queries(qw, *parts):
            slots = [None] * 8
            for h, shift, lo, hi in parts:
                q = pltpu.roll(qw[h], shift, 1) if shift else qw[h]
                for e in range(2):
                    t = q[8 * e:8 * e + 8] & lanes[RANGES.index((lo, hi))]
                    slots[h + e] = t if slots[h + e] is None else t | slots[h + e]
            slots = [jnp.zeros((8, T), u32) if t is None else t for t in slots]
            return pltpu.bitcast(jnp.concatenate(slots, axis=0), bf16)

        def diagonal_scores(s, g, i):
            k0 = i * T
            own = carry.pop("own") if i else _dot(kn[s, g, 0:32, :], own_queries(s, g, 0))
            qw = [qm.words[s, 4 * g + h, :, k0:k0 + T] for h in range(4)]
            x = _dot(kn[s, g, k0 + 32:k0 + 64, :], jnp.concatenate(
                [shared_queries(qw, (h, 0, 32, T), (3, 96 - 32 * h, 0, 32)) for h in range(3)],
                axis=1))
            y = _dot(kn[s, g, k0 + 64:k0 + 96, :], jnp.concatenate(
                [shared_queries(qw, (h, 0, 64, T), (h + 1, 64, 0, 64)) for h in (0, 2)], axis=1))
            z = _dot(kn[s, g, k0 + 96:k0 + T, :], shared_queries(
                qw, *[(h, (32 * h + 32) % T, 32 * h, 32 * h + 32) for h in range(4)]))
            xs = [x[:, h * T:(h + 1) * T] for h in range(3)]
            xr = [pltpu.roll(xs[h], 32 * h + 32, 1) for h in range(3)]
            xs.append(jnp.where(lane32 < 64, xr[0], jnp.where(lane32 < 96, xr[1], xr[2])))
            ys = [y[:, :T], pltpu.roll(y[:, :T], 64, 1), y[:, T:], pltpu.roll(y[:, T:], 64, 1)]
            zs = [pltpu.roll(z, 96 - 32 * h, 1) for h in range(3)] + [z]
            return [jnp.concatenate([own[:, h * T:(h + 1) * T], xs[h], ys[h], zs[h]], axis=0)
                    for h in range(4)]

        def scores(s, g, i, j):
            if DIAG and i == j:
                shs = diagonal_scores(s, g, i)
            else:
                more = 32 if DIAG and j == i - 1 else 0
                st = _dot(pinned_operand(kn[s, g, j * T:(j + 1) * T + more, :]),
                          own_queries(s, g, i))
                if more:
                    carry["own"] = st[T:]
                shs = [st[:T, h * T:(h + 1) * T] for h in range(4)]
            ps, alphas = [], []
            later = any(a == i for a, _ in ORDER[:ORDER.index((i, j))])
            for h in range(4):
                sh = shs[h]
                if i == j:
                    sh = sh + causal[...]
                m = jnp.max(sh, axis=0, keepdims=True)
                if later:
                    m = jnp.maximum(m, run[i, h])
                    alphas.append(jnp.exp2(run[i, h] - m))
                run[i, h] = m
                ps.append(jnp.exp2(sh - m).astype(bf16))
            return ps, alphas

        def values(s, g, i, j, ps, alphas):
            new = [_dot(vl[s, 4 * g + h, :, j * T:(j + 1) * T], ps[h]) for h in range(4)]
            if alphas:
                new = [a * al + b for a, al, b in zip(accs.pop(i), alphas, new)]
            if any(a == i for a, _ in ORDER[ORDER.index((i, j)) + 1:]):
                accs[i] = new
                return
            o = []
            for h in range(4):
                inv = _rcp(jnp.broadcast_to(new[h][ONES_ROW[h]:ONES_ROW[h] + 1], (8, T)))
                o.append([new[h][8 * c:8 * c + 8] * inv for c in range(3)])
            a_dot = jnp.concatenate(
                [o[0][0], o[0][1], jnp.where(r8 < 2, o[0][2], o[1][0]), o[1][1],
                 jnp.where(r8 < 4, o[1][2], o[2][0]), o[2][1],
                 jnp.where(r8 < 6, o[2][2], o[3][0]), o[3][1], o[3][2]], axis=0)
            dst = (s, slice(g * G, (g + 1) * G), slice(i * T, (i + 1) * T))
            mix = (1.0 - gcol[g * G:(g + 1) * G, :]) * a_dot
            ot[dst] = ot[dst] + mix if s > 0 else mix
            if (i, j) == ORDER[-1] and g % PIN_G == PIN_G - 1:
                pin(ot, (s,), PIN_A)

        pend = {}
        for t in range(len(units) + LAG):
            if t < len(units):
                pend[t] = scores(*units[t])
            if t >= LAG:
                values(*units[t - LAG], *pend.pop(t - LAG))
            yield t < len(units) and units[t][2] != units[t][3]

    def out_proj(s):
        o = jnp.concatenate(
            [ot[s], hot[:, s * L:(s + 1) * L], jnp.zeros((DP - D - 8, L), f32)], axis=0).astype(bf16)
        for p in range(NP):
            rows = slice(p * 2 * G, (p + 1) * 2 * G)
            halves = []
            for g in (2 * p, 2 * p + 1):
                a = None
                for k in range(0, DP, T):
                    d = _dot(pinned_operand(wt[3, g * G:(g + 1) * G, k:k + T]), o[k:k + T])
                    a = d if a is None else a + d
                halves.append(a)
                yield 5 * G
            a = jnp.concatenate(halves, axis=0)
            for c in range(NT):
                b = s * NT + c
                res = x_v[rows, b * T:(b + 1) * T].astype(f32) + xn_v[b, rows, :].astype(f32)
                o_v[s, rows, c * T:(c + 1) * T] = (res + a[:, c * T:(c + 1) * T]).astype(bf16)
            o_cp[s][p].start()
            spare = (NSEG, slice(0, 16), slice(0, T))
            o_v[opaque(o_v, spare)] = jnp.zeros((16, T), bf16)
            pin(o_v, (NSEG,), PIN_P)

    routed = {}

    def row_block(ref, k, cols):
        w = ref[k:min(k + T, D), cols]
        if k + T > D:
            w = jnp.concatenate([w, jnp.zeros((DP - D, w.shape[1]), bf16)], axis=0)
        return w

    def route():
        def both(op, a):
            return op(op(a, axis=0, keepdims=True), axis=1, keepdims=True)

        r = r_v[...]
        idx = (_iota(r.shape, 0) * T + _iota(r.shape, 1)).astype(f32)
        m1 = both(jnp.max, r)
        i1 = both(jnp.min, jnp.where(r == m1, idx, S))
        r = jnp.where(idx == i1, -jnp.inf, r)
        m2 = both(jnp.max, r)
        i2 = both(jnp.min, jnp.where((r == m2) & (idx != i1), idx, S))
        row = _iota((8, T), 0)
        routed["w"] = jax.nn.sigmoid(jnp.where(row == 0, m1, m2))
        pick = jnp.where(row == 0, i1, jnp.where(row == 1, i2, -1.0))
        for b in range(S // T):
            hot[:, b * T:(b + 1) * T] = (pick == (lane8 + b * T).astype(f32)).astype(f32)
        for _ in range(ROUTE_WAIT):
            yield True
        blocks = [jnp.broadcast_to(i.astype(jnp.int32) >> 7, (32, T)) for i in (i1, i2)]
        tiles = [[], []]
        for r0 in range(0, DP // 2, 32):
            acc = [xn_v.words[0, r0:r0 + 32, :]] * 2
            for b in range(1, S // T):
                w = xn_v.words[b, r0:r0 + 32, :]
                acc = [jnp.where(blocks[n] == b, w, acc[n]) for n in range(2)]
            for n in range(2):
                tiles[n].append(acc[n])
            if r0 % 64:
                yield True
        x = None
        for n, i in enumerate((i1, i2)):
            pick = (row == n) & (lane8 == (i.astype(jnp.int32) & (T - 1)))
            d = _dot_nt(pick.astype(f32), pltpu.bitcast(jnp.concatenate(tiles[n], axis=0), bf16))
            x = d if x is None else x + d
        routed["x"] = [x[:, k:k + T] for k in range(0, DP, T)]

    def ffn_hidden():
        routed["h"] = []
        for n in range(0, F, L):
            gu = []
            for w_ref in (wg_v, wu_v):
                acc = None
                for c, k in enumerate(range(0, D, T)):
                    d = _dot(routed["x"][c], row_block(w_ref, k, slice(n, n + L)))
                    acc = d if acc is None else acc + d
                    yield True
                gu.append(acc)
            routed["h"].append(gu[0] * jax.nn.sigmoid(gu[0]) * gu[1])

    def ffn_down():
        for k in range(0, D, T):
            acc = None
            for c, n in enumerate(range(0, F, L)):
                d = _dot_nt(routed["h"][c], row_block(wd_v, k, slice(n, n + L)))
                acc = d if acc is None else acc + d
                yield
            y = jnp.concatenate([jnp.zeros((D - 4 * T, T), f32), acc * routed["w"],
                                 jnp.zeros((DP - D - 8, T), f32)], axis=0).T
            dst = (3, slice(k, min(k + T, D)), slice(4 * T, DP))
            wt[dst] = wt[dst] + y[0:min(T, D - k)]
            pin(wt, (3,), PIN_A)

    for c in (*c_cp, *x_cp[:2], *wq_cp, *w_cp[1:3]):
        c.start()
    causal[...] = jnp.where(_iota((T, T), 0) <= _iota((T, T), 1), 0.0, NEG)
    for n, (lo, hi) in enumerate(RANGES):
        lanes[n] = pltpu.bitcast(jnp.where((lane8 >= lo) & (lane8 < hi), -1, 0), u32)
    for c in c_cp:
        c.wait()
    router_column()
    for _ in gate_column():
        pass
    for b in range(NT):
        if b % 2 == 0:
            x_cp[b // 2].wait()
        fillers.append(layernorm(b, LNROWS0))
        prev = [None, None]
        while fillers:
            prev.append(fill(prev.pop(0)))
    x_cp[2].start()
    wq_cp[0].wait()
    fillers.append(transpose_w(0, 0, 2 * T))
    drain()
    for p in range(NG):
        if p == 2:
            wq_cp[1].wait()
            fillers.append(transpose_w(0, 2 * T))
            drain()
        if p == NG - 1:
            for c in (x_cp[3], w_cp[3]):
                c.start()
            w_cp[1].wait()
            fillers.append(transpose_w(1))
            drain()
        run(project_q(0, p))
    pks = []
    for p in range(NG):
        if p == NG - 1:
            for ref in (wg_v, wu_v, wd_v):
                ref[0:16, 0:T] = kn[0, 0, 0:16, :]
            for c in f_cp:
                c.start()
            for c in (w_cp[2], x_cp[2]):
                c.wait()
            fillers.append(transpose_w(2))
            drain()
            fillers.extend(layernorm(b, LNROWS1) for b in range(NT, 2 * NT))
        pks.append(run(project_k(0, p)))
    for p in range(NG):
        run(project_v(0, p, pks[p]))
    drain()
    def dense(s):
        while normed[0] < (s + 1) * NT:
            fill()
        for p in range(NG):
            yield from project_q(s, p)
            if s == 1 and p == 0:
                for c in (x_cp[3], w_cp[3]):
                    c.wait()
                fillers.extend(layernorm(b, LNROWS) for b in range(2 * NT, S // T))
                fillers.append(route())
                small.append(transpose_w(3))
            yield from project_v(s, p, (yield from project_k(s, p)))
            if s == NSEG - 1 and p == FWAIT:
                for c in f_cp:
                    c.wait()
                run(small.pop())
                small.append(ffn_hidden())

    def weave(main, steps, other, rows, extra=iter(())):
        done = 0
        for t in range(steps):
            if next(main):
                next(extra, None)
            while done < (t + 1) * rows // steps:
                done += next(other, rows)

    def finish(main, other):
        for _ in range(LAG):
            next(other)
            next(main)
        run(main)
        run(other)

    per_seg = NG * len(ORDER)
    seg_rows = NP * (15 * 2 * G + 4 * (G + 8))
    run(dense(1))
    run(dense(2))
    drain()
    att, steps = attention([0]), dense(3)
    weave(att, per_seg, iter(()), 0)
    finish(att, steps)
    run(small[0])
    drain()
    att = attention(range(1, NSEG))
    steps = ffn_down()
    weave(att, per_seg, iter(()), 0, steps)
    run(steps)
    outs = (n for s in range(NSEG - 1) for n in out_proj(s))
    weave(att, 2 * per_seg, outs, 3 * NP * 5 * 2 * G - TAIL * G)
    finish(att, outs)
    run(out_proj(NSEG - 1))
    for cs in o_cp:
        for c in cs:
            c.wait()


@jax.jit
def pallas_parallel_sum__memory_aug_infini_attn__moe_arch_mod__prompt_kernel(
    A_x: jax.Array,
    A_wq: jax.Array,
    A_wk: jax.Array,
    A_wv: jax.Array,
    A_wo: jax.Array,
    A_beta: jax.Array,
    B_x: jax.Array,
    B_w_r: jax.Array,
    B_w_gate: jax.Array,
    B_w_up: jax.Array,
    B_w_down: jax.Array,
):
    del B_x
    hbm = pl.BlockSpec(memory_space=pltpu.HBM)
    out = pl.pallas_call(
        _kernel,
        out_shape=jax.ShapeDtypeStruct((D, S), A_x.dtype),
        in_specs=[hbm] * 10,
        out_specs=hbm,
        scratch_shapes=[
            pltpu.VMEM((D, S), bf16),
            pltpu.VMEM((4, D, D), bf16),
            pltpu.VMEM((1, H), bf16),
            pltpu.VMEM((D,), bf16),
            pltpu.VMEM((D, F), bf16),
            pltpu.VMEM((D, F), bf16),
            pltpu.VMEM((D, F), bf16),
            pltpu.VMEM((4, D, DP), f32),
            pltpu.VMEM((D, T), f32),
            pltpu.VMEM((S // T, DP // 2, T), u32),
            pltpu.VMEM((NSEG, H, 16, L), u32),
            pltpu.VMEM((NSEG, H, 24, L), f32),
            pltpu.VMEM((NSEG, NG, L // 2, T), u32),
            pltpu.VMEM((NSEG, D, L), f32),
            pltpu.VMEM((NG, G + 8, T), f32),
            pltpu.VMEM((D, T), f32),
            pltpu.VMEM((S // T, T), f32),
            pltpu.VMEM((8, S), f32),
            pltpu.VMEM((NSEG + 1, D, L), bf16),
            pltpu.VMEM((T, T), f32),
            pltpu.VMEM((len(RANGES), 8, T), u32),
            pltpu.SemaphoreType.DMA((8 + len(XPARTS),)),
        ],
        compiler_params=pltpu.CompilerParams(vmem_limit_bytes=100 * 2**20),
    )(A_x.reshape(S, D).T, A_wq, A_wk, A_wv, A_wo, A_beta.reshape(1, H), B_w_r,
      B_w_gate, B_w_up, B_w_down.T)
    return out.T.reshape(A_x.shape)
```

```python
import functools

import jax
import jax.numpy as jnp
import jax.experimental.pallas as pl
import jax.experimental.pallas.tpu as pltpu

S, D, H, DH, NSEG, L, F = 2048, 576, 32, 18, 4, 512, 4608
DP = 640
G = 4 * DH
NG = H // 4
T = 128
NT = L // T
NP = NG // 2
LATE = 2
ROUTE_AT = 55
WO_READY = (0, 2, 6, 0)
FWAIT = (2, 3, 0)
WAIT_K = 4
SLOTS2 = ((),(0,1,2),(0,1))
TAIL = 30
SLOTS3 = (0, 1, 2, 3)
ROUTE_WAIT = 5
LNROWS0 = 144
LNROWS1 = 144
LAG = 2
ORDER = ((3, 2), (3, 3), (3, 0), (0, 0), (3, 1), (2, 1), (2, 2), (2, 0), (1, 0), (1, 1))
SLOTS = ((0, 1, 2, 3, 4), (3, 4,), (2, 3, 4))
LNROWS = 96
LOG2E = 1.4426950408889634
QSCALE = DH ** -0.5 * LOG2E
NEG = -1e30
ONES_ROW = (23, 23, 0, 0)
XPARTS = ((0, 256), (256, 256), (512, 512), (1024, 1024))
ROT = (32, 64, 96, 0)
RANGES = ((0b0001, 0b0010, 0b0100, 0b1000, 0b1101, 0b1011, 0b0111, 0b1001, 0b0110, 0b0011, 0b1100))

f32, bf16, u32 = jnp.float32, jnp.bfloat16, jnp.uint32


def _dot(a, b):
    return jnp.dot(a, b, preferred_element_type=f32)


def _dot_nt(a, b):
    return jax.lax.dot_general(a, b, (((1,), (1,)), ((), ())), preferred_element_type=f32)


def _rnd(a):
    return a.astype(bf16).astype(f32)


def _rcp(a):
    return pltpu.reciprocal(a, full_range=False)


def _iota(shape, axis):
    return jax.lax.broadcasted_iota(jnp.int32, shape, axis)


def _pad_to_tile(a):
    if a.shape[1] < T:
        a = jnp.concatenate([a, jnp.zeros((a.shape[0], T - a.shape[1]), a.dtype)], axis=1)
    if a.shape[0] < T:
        a = jnp.concatenate([a, jnp.zeros((T - a.shape[0], T), a.dtype)], axis=0)
    return a


def _roll(a, shift):
    return pltpu.roll(a, shift % T, 1) if shift % T else a


def _phi(t):
    return jnp.where(t > 0, t + 1.0, jnp.exp(t))


def _head_of(i):
    return ((i >= DH).astype(jnp.int32) + (i >= 2 * DH).astype(jnp.int32)
            + (i >= 3 * DH).astype(jnp.int32) + (i >= 4 * DH).astype(jnp.int32))


class _Packed:
    def __init__(self, ref):
        self.words = ref

    def _index(self, idx):
        *lead, rows, cols = idx
        start, stop, _ = rows.indices(2 * self.words.shape[-2])
        return (*lead, slice(start // 2, stop // 2), cols)

    def __getitem__(self, idx):
        return pltpu.bitcast(self.words[self._index(idx)], bf16)

    def __setitem__(self, idx, value):
        self.words[self._index(idx)] = pltpu.bitcast(value, u32)


def run(gen):
    try:
        while True:
            next(gen)
    except StopIteration as stop:
        return stop.value


def _kernel(x_hbm, wq_hbm, wk_hbm, wv_hbm, wo_hbm, beta_hbm, wr_hbm, wg_hbm, wu_hbm,
            wd_hbm, o_hbm,
            x_v, w_v, beta_v, wr_v, wg_v, wu_v, wd_v, wt, wrc, xn_v, qm, vl, kn, ot, mst,
            gcol, r_v, hot, o_v, causal, lanes, sem):
    xn_v, qm, kn = (_Packed(r) for r in (xn_v, qm, kn))
    x_cp = [pltpu.make_async_copy(x_hbm.at[:, pl.ds(t, n)], x_v.at[:, pl.ds(t, n)], sem.at[7 + i])
            for i, (t, n) in enumerate(XPARTS)]
    w_cp = [pltpu.make_async_copy(w, w_v.at[i], sem.at[i]) if i else None
            for i, w in enumerate((wq_hbm, wk_hbm, wv_hbm, wo_hbm))]
    wq_cp = [pltpu.make_async_copy(wq_hbm.at[:, pl.ds(c, n)], w_v.at[0, :, pl.ds(c, n)], sm)
             for c, n, sm in ((0, 2 * T, sem.at[0]), (2 * T, D - 2 * T, sem.at[7 + len(XPARTS)]))]
    f_cp = [pltpu.make_async_copy(a, b, sem.at[4])
            for i, (a, b) in enumerate(((wg_hbm, wg_v), (wu_hbm, wu_v), (wd_hbm, wd_v)))]
    c_cp = [pltpu.make_async_copy(a, b, sem.at[5])
            for i, (a, b) in enumerate(((wr_hbm, wr_v), (beta_hbm, beta_v)))]
    o_cp = [[pltpu.make_async_copy(o_v.at[s, pl.ds(p * 2 * G, 2 * G)],
                                   o_hbm.at[pl.ds(p * 2 * G, 2 * G), pl.ds(s * L, L)],
                                   sem.at[6]) for p in range(NP)] for s in range(NSEG)]

    fillers = []

    lane8 = _iota((8, T), 1)
    never = lane8 < jnp.min(lane8, axis=1, keepdims=True)
    zero = jnp.min(lane8)
    link = [None, None]

    def tie(a, b):
        return a if b is None else jnp.where(never, b, a)

    def fill(after=None):
        link[0], link[1] = after, None
        while fillers:
            if next(fillers[0], False):
                break
            fillers.pop(0)
        return link[1]

    def drain():
        while fillers:
            fill()

    def gate_column():
        gate = jax.nn.sigmoid(beta_v[...].astype(f32))
        gate = jnp.concatenate([gate, jnp.zeros((1, T - H), f32)], axis=1)
        gate = jnp.broadcast_to(gate, (T, T)).T
        r8 = _iota((8, T), 0)
        for v in range(D // 8):
            h0, h1 = (8 * v) // DH, (8 * v + 7) // DH
            gv = jnp.broadcast_to(gate[h0:h0 + 1], (8, T))
            if h1 != h0:
                gv = jnp.where(r8 < h1 * DH - 8 * v, gv, jnp.broadcast_to(gate[h1:h1 + 1], (8, T)))
            gcol[8 * v:8 * v + 8, :] = gv
            if v % 9 == 8:
                yield True

    def router_column():
        wr = wr_v[...].astype(f32).reshape(1, D)
        wr = jnp.concatenate([wr, jnp.zeros((1, DP - D), f32)], axis=1)
        wrc[...] = jnp.broadcast_to(wr, (T, DP)).T[0:D]

    def transpose_w(i, lo=0, hi=D):
        for c in range(lo, hi, T):
            n = min(T, D - c)
            for k in range(0, D, T):
                w = _pad_to_tile(w_v[i, k:min(k + T, D), c:c + n].astype(f32))
                w = jnp.concatenate([tie(w[r:r + 8], link[0]) for r in range(0, T, 8)], axis=0).T
                wt[i, c:c + n, k:k + T] = w[0:n]
                yield True

    normed = [0]

    def layernorm(b, step):

        def chain(acc, v):
            h = v.shape[0] // 16 * 8
            a, c = v[0:8], v[h:h + 8]
            for k in range(8, h, 8):
                a, c = a + v[k:k + 8], c + v[h + k:h + k + 8]
            return a + c if acc is None else acc + (a + c)

        def rows(v):
            return jnp.concatenate([tie(v, link[0])] * (step // 8), axis=0)

        def bcast(v):
            return jnp.broadcast_to(v, (8, T))

        def load(r, n):
            return x_v[r:r + step, pl.ds(pl.multiple_of((b + n * zero) * T, T), T)].astype(f32)

        acc = jnp.zeros((8, T), f32)
        for r in range(0, D, step):
            x = load(r, 0)
            link[1] = acc = chain(tie(acc, link[0]), x)
            yield True
        mean = bcast(jnp.sum(acc, axis=0, keepdims=True) * (1.0 / D))
        acc = None
        for r in range(0, D, step):
            xc = load(r, 1) - rows(mean)
            link[1] = acc = chain(acc, xc * xc)
            yield True
        var = bcast(jnp.sum(acc, axis=0, keepdims=True) * (1.0 / D))
        sd = _rnd(jnp.sqrt(_rnd(_rnd(var) + _rnd(jnp.full((8, T), 1e-5, f32)))))
        inv, mean = jnp.concatenate([1.0 / sd] * (step // 8), axis=0), _rnd(mean)
        acc = None
        for r in range(0, D, step):
            x = load(r, 2)
            xn = (_rnd(x - rows(mean)) * inv).astype(bf16)
            xn_v[b, r:r + step, :] = xn
            link[1] = acc = chain(acc, xn.astype(f32) * wrc[r:r + step, :])
            if r + step == D:
                xn_v[b, D:DP, :] = jnp.zeros((DP - D, T), bf16)
                r_v[b:b + 1, :] = _rnd(jnp.sum(acc, axis=0, keepdims=True))
                normed[0] += 1
            yield True

    late = [None] * LATE
    deferred = []
    arrivals = {}
    small = []

    def proj(i, s, g, slots):
        acc = None
        for k in range(0, DP, T):
            xs = jnp.concatenate([xn_v[s * NT + c, k:k + T, :] for c in range(NT)], axis=1)
            w = wt[i, g * G:(g + 1) * G, k:k + T]
            if (i, s, g, k) == WO_READY:
                done = wt[zero, pl.ds(pl.multiple_of(zero * 8, 8), 8),
                          pl.ds(pl.multiple_of(zero * T, T), T)]
                w = jnp.concatenate([w[:-8], tie(w[-8:], done)], axis=0)
            if (i, s, g) in arrivals and k == WAIT_K * T:
                arrivals.pop((i, s, g))()
            d = _dot(w, xs)
            done = late.pop(0)
            top = tie(d[-8:, :T], done)
            d = jnp.concatenate([d[:-8], jnp.concatenate([top, d[-8:, T:]], axis=1)], axis=0)
            acc = d if acc is None else acc + d
            late.append(fill(d[0:8, 0:T]) if k // T in slots else None)
            if small and k // T in (SLOTS3 if s == 3 else SLOTS2[i]):
                next(small[0], None)
        yield 5 * G
        while deferred:
            deferred.pop(0)()
            yield G + 8
        return acc

    def project_q(s, g):
        q = yield from proj(0, s, g, SLOTS[0])
        r8 = _iota((8, L), 0)
        qs = q * QSCALE
        for h in range(4):
            lo = 16 * h
            a0, a1, a2 = qs[lo:lo + 8], qs[lo + 8:lo + 16], qs[lo + 16:lo + 24]
            if h > 0:
                a0 = jnp.where(r8 >= 2 * h, a0, 0.0)
            if h < 3:
                a2 = jnp.where(r8 < 2 * h + 2, a2, 0.0)
            w = pltpu.bitcast(jnp.concatenate(
                [a0, a1, a2, jnp.zeros((8, L), f32)], axis=0).astype(bf16), u32)
            for c in range(0, L, T):
                qm.words[s, 4 * g + h, :, c:c + T] = _roll(w[:, c:c + T], ROT[h])
        if s > 0:
            pq = jnp.concatenate([_phi(q), jnp.zeros((T - G, L), f32)], axis=0).astype(bf16)
            deferred.append(functools.partial(memory_read, s, g, pq))

    def memory_read(s, g, pq):
        r8 = _iota((8, L), 0)
        mrow = _iota((G + 8, T), 0)
        mkeep = jnp.where(mrow < G, _head_of(mrow), mrow - G) == _head_of(_iota((G + 8, T), 1))
        nd = _dot(jnp.where(mkeep, mst[g], 0.0).astype(bf16), pq)
        inv = _rcp(nd[G:] + 1e-6)
        ib = [jnp.broadcast_to(inv[h:h + 1], (8, L)) for h in range(4)]
        iv = jnp.concatenate(
            [ib[0], ib[0], jnp.where(r8 < 2, ib[0], ib[1]), ib[1],
             jnp.where(r8 < 4, ib[1], ib[2]), ib[2],
             jnp.where(r8 < 6, ib[2], ib[3]), ib[3], ib[3]], axis=0)
        gg = gcol[g * G:(g + 1) * G, :]
        ot[s, g * G:(g + 1) * G, :] = nd[:G] * iv * jnp.concatenate([gg] * NT, axis=1)

    def memory_update(s, g, v80, pk):
        upd = _dot_nt(v80, pk)
        mst[g] = upd if s == 0 else mst[g] + upd

    def project_k(s, g):
        k = yield from proj(1, s, g, SLOTS[1] if s else SLOTS[2])
        zpad = jnp.zeros((T - G, L), f32)
        kn[s, g, :, :] = jnp.concatenate([k, zpad], axis=0).astype(bf16).T
        if s < NSEG - 1:
            return jnp.concatenate([_phi(k), zpad], axis=0).astype(bf16)

    def project_v(s, g, pk):
        v = yield from proj(2, s, g, SLOTS[2] if s else SLOTS[0])
        for h in range(4):
            a = [v[16 * h + c:16 * h + c + 8] for c in (0, 8, 16)]
            c, r = divmod(ONES_ROW[h], 8)
            a[c] = jnp.where(_iota((8, L), 0) == r, 1.0, a[c])
            vl[s, 4 * g + h] = jnp.concatenate(a, axis=0)
        if pk is not None:
            v80 = jnp.concatenate([v, jnp.ones((8, L), f32)], axis=0)
            deferred.append(functools.partial(memory_update, s, g, v80, pk))

    def attention(segs):
        r8 = _iota((8, T), 0)
        units = [(s, g, i, j) for s in segs for g in range(NG) for i, j in ORDER]
        run, accs = {}, {}

        lane32 = _iota((32, T), 1)
        carry = {}

        def own_queries(s, g, i):
            w = []
            for h in range(4):
                parts = [qm[s, 4 * g + h, :, i * T:(i + 1) * T]]
                if h > 0:
                    parts.insert(0, jnp.zeros((16 * h, T), bf16))
                parts.append(jnp.zeros((T - 32 - 16 * h, T), bf16))
                w.append(jnp.concatenate(parts, axis=0))
            return jnp.concatenate(w, axis=1)

        def shared_queries(qw, *parts):
            slots = [None] * 8
            for h, quarters in parts:
                for e in range(2):
                    t = qw[h][8 * e:8 * e + 8] & lanes[RANGES.index(quarters)]
                    slots[h + e] = t if slots[h + e] is None else t | slots[h + e]
            slots = [jnp.zeros((8, T), u32) if t is None else t for t in slots]
            return pltpu.bitcast(jnp.concatenate(slots, axis=0), bf16)

        def diagonal_scores(s, g, i):
            k0 = i * T
            own = carry.pop("own") if i else _dot(kn[s, g, 0:32, :], own_queries(s, g, 0))
            qw = [qm.words[s, 4 * g + h, :, k0:k0 + T] for h in range(4)]
            x = _dot(kn[s, g, k0 + 32:k0 + 64, :], jnp.concatenate(
                [shared_queries(qw, (h, 15 - (2 << h)), (3, 2 << h)) for h in range(3)], axis=1))
            y = _dot(kn[s, g, k0 + 64:k0 + 96, :], jnp.concatenate(
                [shared_queries(qw, (0, 0b1001), (2, 0b0110)),
                 shared_queries(qw, (1, 0b0011), (3, 0b1100))], axis=1))
            z = _dot(kn[s, g, k0 + 96:k0 + T, :],
                     shared_queries(qw, *[(h, 1 << h) for h in range(4)]))
            xs = [x[:, h * T:(h + 1) * T] for h in range(3)]
            xs.append(jnp.where(lane32 < 64, xs[0], jnp.where(lane32 < 96, xs[1], xs[2])))
            ys = [y[:, :T], y[:, T:]] * 2
            zs = [z] * 4
            return [jnp.concatenate([own[:, h * T:(h + 1) * T], xs[h], ys[h], zs[h]], axis=0)
                    for h in range(4)]

        def scores(s, g, i, j):
            if i == j:
                shs = diagonal_scores(s, g, i)
            else:
                more = 32 if j == i - 1 else 0
                st = _dot(kn[s, g, j * T:(j + 1) * T + more, :],
                          own_queries(s, g, i))
                if more:
                    carry["own"] = st[T:]
                shs = [st[:T, h * T:(h + 1) * T] for h in range(4)]
            ps, alphas = [], []
            later = any(a == i for a, _ in ORDER[:ORDER.index((i, j))])
            for h in range(4):
                sh = shs[h]
                if i == j:
                    sh = sh + causal[h]
                m = jnp.max(sh, axis=0, keepdims=True)
                if later:
                    m = jnp.maximum(m, run[i, h])
                    alphas.append(jnp.exp2(run[i, h] - m))
                run[i, h] = m
                ps.append(jnp.exp2(sh - m).astype(bf16))
            return ps, alphas

        def values(s, g, i, j, ps, alphas):
            new = [_dot(vl[s, 4 * g + h, :, j * T:(j + 1) * T], ps[h]) for h in range(4)]
            if alphas:
                new = [a * al + b for a, al, b in zip(accs.pop(i), alphas, new)]
            if any(a == i for a, _ in ORDER[ORDER.index((i, j)) + 1:]):
                accs[i] = new
                return
            o = []
            for h in range(4):
                inv = _rcp(jnp.broadcast_to(new[h][ONES_ROW[h]:ONES_ROW[h] + 1], (8, T)))
                o.append([_roll(new[h][8 * c:8 * c + 8] * inv, -ROT[h]) for c in range(3)])
            a_dot = jnp.concatenate(
                [o[0][0], o[0][1], jnp.where(r8 < 2, o[0][2], o[1][0]), o[1][1],
                 jnp.where(r8 < 4, o[1][2], o[2][0]), o[2][1],
                 jnp.where(r8 < 6, o[2][2], o[3][0]), o[3][1], o[3][2]], axis=0)
            dst = (s, slice(g * G, (g + 1) * G), slice(i * T, (i + 1) * T))
            mix = (1.0 - gcol[g * G:(g + 1) * G, :]) * a_dot
            ot[dst] = ot[dst] + mix if s > 0 else mix

        pend = {}
        for t in range(len(units) + LAG):
            if t < len(units):
                pend[t] = scores(*units[t])
            if t >= LAG:
                values(*units[t - LAG], *pend.pop(t - LAG))
            yield t < len(units) and units[t][2] != units[t][3]

    def out_proj(s):
        o = jnp.concatenate(
            [ot[s], hot[:, s * L:(s + 1) * L], jnp.zeros((DP - D - 8, L), f32)], axis=0).astype(bf16)
        for p in range(NP):
            rows = slice(p * 2 * G, (p + 1) * 2 * G)
            halves = []
            for g in (2 * p, 2 * p + 1):
                a = None
                for k in range(0, DP, T):
                    d = _dot(wt[3, g * G:(g + 1) * G, k:k + T], o[k:k + T])
                    a = d if a is None else a + d
                halves.append(a)
                yield 5 * G
            a = jnp.concatenate(halves, axis=0)
            for c in range(NT):
                b = s * NT + c
                res = x_v[rows, b * T:(b + 1) * T].astype(f32) + xn_v[b, rows, :].astype(f32)
                o_v[s, rows, c * T:(c + 1) * T] = (res + a[:, c * T:(c + 1) * T]).astype(bf16)
            o_cp[s][p].start()

    routed = {}

    def row_block(ref, k, cols):
        w = ref[k:min(k + T, D), cols]
        if k + T > D:
            w = jnp.concatenate([w, jnp.zeros((DP - D, w.shape[1]), bf16)], axis=0)
        return w

    def route():
        def both(op, a):
            return op(op(a, axis=0, keepdims=True), axis=1, keepdims=True)

        r = r_v[...]
        idx = (_iota(r.shape, 0) * T + _iota(r.shape, 1)).astype(f32)
        m1 = both(jnp.max, r)
        i1 = both(jnp.min, jnp.where(r == m1, idx, S))
        r = jnp.where(idx == i1, -jnp.inf, r)
        m2 = both(jnp.max, r)
        i2 = both(jnp.min, jnp.where((r == m2) & (idx != i1), idx, S))
        row = _iota((8, T), 0)
        routed["w"] = jax.nn.sigmoid(jnp.where(row == 0, m1, m2))
        pick = jnp.where(row == 0, i1, jnp.where(row == 1, i2, -1.0))
        for b in range(S // T):
            hot[:, b * T:(b + 1) * T] = (pick == (lane8 + b * T).astype(f32)).astype(f32)
        for _ in range(ROUTE_WAIT):
            yield True
        blocks = [jnp.broadcast_to(i.astype(jnp.int32) >> 7, (32, T)) for i in (i1, i2)]
        tiles = [[], []]
        for r0 in range(0, DP // 2, 32):
            acc = [xn_v.words[0, r0:r0 + 32, :]] * 2
            for b in range(1, S // T):
                w = xn_v.words[b, r0:r0 + 32, :]
                acc = [jnp.where(blocks[n] == b, w, acc[n]) for n in range(2)]
            for n in range(2):
                tiles[n].append(acc[n])
            if r0 % 64:
                yield True
        x = None
        for n, i in enumerate((i1, i2)):
            pick = (row == n) & (lane8 == (i.astype(jnp.int32) & (T - 1)))
            d = _dot_nt(pick.astype(f32), pltpu.bitcast(jnp.concatenate(tiles[n], axis=0), bf16))
            x = d if x is None else x + d
        routed["x"] = [x[:, k:k + T] for k in range(0, DP, T)]

    def ffn_hidden():
        routed["h"] = []
        for n in range(0, F, L):
            gu = []
            for w_ref in (wg_v, wu_v):
                acc = None
                for c, k in enumerate(range(0, D, T)):
                    d = _dot(routed["x"][c], row_block(w_ref, k, slice(n, n + L)))
                    acc = d if acc is None else acc + d
                    yield True
                gu.append(acc)
            routed["h"].append(gu[0] * jax.nn.sigmoid(gu[0]) * gu[1])

    def ffn_down():
        for k in range(0, D, T):
            acc = None
            for c, n in enumerate(range(0, F, L)):
                d = _dot_nt(routed["h"][c], row_block(wd_v, k, slice(n, n + L)))
                acc = d if acc is None else acc + d
                yield
            y = jnp.concatenate([jnp.zeros((D - 4 * T, T), f32), acc * routed["w"],
                                 jnp.zeros((DP - D - 8, T), f32)], axis=0).T
            dst = (3, slice(k, min(k + T, D)), slice(4 * T, DP))
            wt[dst] = wt[dst] + y[0:min(T, D - k)]

    for c in (*c_cp, *x_cp[:2], *wq_cp, *w_cp[1:3]):
        c.start()
    for h in range(4):
        query = (_iota((T, T), 1) - ROT[h]) & (T - 1)
        causal[h] = jnp.where(_iota((T, T), 0) <= query, 0.0, NEG)
    for n, quarters in enumerate(RANGES):
        lanes[n] = pltpu.bitcast(-((quarters >> (lane8 >> 5)) & 1), u32)
    for c in c_cp:
        c.wait()
    router_column()
    for _ in gate_column():
        pass
    for b in range(NT):
        if b % 2 == 0:
            x_cp[b // 2].wait()
        fillers.append(layernorm(b, LNROWS0))
        prev = [None, None]
        while fillers:
            prev.append(fill(prev.pop(0)))
    x_cp[2].start()
    wq_cp[0].wait()
    fillers.append(transpose_w(0, 0, 2 * T))
    drain()

    def rest_of_wq():
        wq_cp[1].wait()
        run(transpose_w(0, 2 * T))

    def wk_arrives():
        for c in (x_cp[3], w_cp[3]):
            c.start()
        w_cp[1].wait()
        run(transpose_w(1))

    def wv_arrives():
        for ref in (wg_v, wu_v, wd_v):
            ref[0:16, 0:T] = kn[0, 0, 0:16, :]
        for c in f_cp:
            c.start()
        for c in (w_cp[2], x_cp[2]):
            c.wait()
        run(transpose_w(2))
        fillers.extend(layernorm(b, LNROWS1) for b in range(NT, 2 * NT))

    def wo_arrives():
        for c in (x_cp[3], w_cp[3]):
            c.wait()
        fillers.extend(layernorm(b, LNROWS) for b in range(2 * NT, S // T))
        small.append(transpose_w(3))

    def ffn_arrives():
        for c in f_cp:
            c.wait()
        run(small.pop())
        small.append(ffn_hidden())

    arrivals.update({(0, 0, 2): rest_of_wq, (0, 0, NG - 1): wk_arrives, (1, 0, NG - 1): wv_arrives,
                     (0, 1, 0): wo_arrives, FWAIT: ffn_arrives})
    for g in range(NG):
        run(project_q(0, g))
    pks = [run(project_k(0, g)) for g in range(NG)]
    for g in range(NG):
        run(project_v(0, g, pks[g]))

    def dense(s):
        while normed[0] < (s + 1) * NT:
            fill()
        for g in range(NG):
            yield from project_q(s, g)
            yield from project_v(s, g, (yield from project_k(s, g)))

    def weave(main, steps, other, rows, extra=iter(())):
        done = 0
        for t in range(steps):
            if next(main):
                next(extra, None)
            while done < (t + 1) * rows // steps:
                done += next(other, rows)

    def finish(main, other):
        for _ in range(LAG):
            next(other)
            next(main)
        run(main)
        run(other)

    per_seg = NG * len(ORDER)
    seg_rows = NP * (15 * 2 * G + 4 * (G + 8))
    run(dense(1))
    run(dense(2))
    drain()
    att, steps = attention([0]), dense(3)
    weave(att, ROUTE_AT, iter(()), 0)
    routing = route()
    weave(att, per_seg - ROUTE_AT, iter(()), 0, routing)
    run(routing)
    finish(att, steps)
    run(small[0])
    drain()
    att = attention(range(1, NSEG))
    steps = ffn_down()
    weave(att, per_seg, iter(()), 0, steps)
    run(steps)
    outs = (n for s in range(NSEG - 1) for n in out_proj(s))
    weave(att, 2 * per_seg, outs, 3 * NP * 5 * 2 * G - TAIL * G)
    finish(att, outs)
    run(out_proj(NSEG - 1))
    for cs in o_cp:
        for c in cs:
            c.wait()


@jax.jit
def pallas_parallel_sum__memory_aug_infini_attn__moe_arch_mod__prompt_kernel(
    A_x: jax.Array,
    A_wq: jax.Array,
    A_wk: jax.Array,
    A_wv: jax.Array,
    A_wo: jax.Array,
    A_beta: jax.Array,
    B_x: jax.Array,
    B_w_r: jax.Array,
    B_w_gate: jax.Array,
    B_w_up: jax.Array,
    B_w_down: jax.Array,
):
    del B_x
    hbm = pl.BlockSpec(memory_space=pltpu.HBM)
    out = pl.pallas_call(
        _kernel,
        out_shape=jax.ShapeDtypeStruct((D, S), A_x.dtype),
        in_specs=[hbm] * 10,
        out_specs=hbm,
        scratch_shapes=[
            pltpu.VMEM((D, S), bf16),
            pltpu.VMEM((4, D, D), bf16),
            pltpu.VMEM((1, H), bf16),
            pltpu.VMEM((D,), bf16),
            pltpu.VMEM((D, F), bf16),
            pltpu.VMEM((D, F), bf16),
            pltpu.VMEM((D, F), bf16),
            pltpu.VMEM((4, D, DP), f32),
            pltpu.VMEM((D, T), f32),
            pltpu.VMEM((S // T, DP // 2, T), u32),
            pltpu.VMEM((NSEG, H, 16, L), u32),
            pltpu.VMEM((NSEG, H, 24, L), f32),
            pltpu.VMEM((NSEG, NG, L // 2, T), u32),
            pltpu.VMEM((NSEG, D, L), f32),
            pltpu.VMEM((NG, G + 8, T), f32),
            pltpu.VMEM((D, T), f32),
            pltpu.VMEM((S // T, T), f32),
            pltpu.VMEM((8, S), f32),
            pltpu.VMEM((NSEG, D, L), bf16),
            pltpu.VMEM((4, T, T), f32),
            pltpu.VMEM((len(RANGES), 8, T), u32),
            pltpu.SemaphoreType.DMA((8 + len(XPARTS),)),
        ],
        compiler_params=pltpu.CompilerParams(vmem_limit_bytes=100 * 2**20),
    )(A_x.reshape(S, D).T, A_wq, A_wk, A_wv, A_wo, A_beta.reshape(1, H), B_w_r,
      B_w_gate, B_w_up, B_w_down.T)
    return out.T.reshape(A_x.shape)
```

```python
import functools

import jax
import jax.numpy as jnp
import jax.experimental.pallas as pl
import jax.experimental.pallas.tpu as pltpu

S, D, H, DH, NSEG, L, F = 2048, 576, 32, 18, 4, 512, 4608
DP = 640
G = 4 * DH
NG = H // 4
T = 128
NT = L // T
NP = NG // 2
LATE = 2
ROUTE_AT = 55
WO_READY = (0, 2, 6, 0)
FWAIT = (0, 3, 1)
WAIT_K = 4
SLOTS2 = ((),(0,1,2),(0,1))
TAIL = 30
SLOTS3 = (0, 1, 2, 3)
ROUTE_WAIT = 5
LNROWS0 = 144
LNROWS1 = 144
LAG = 3
ORDER = ((3, 2), (3, 3), (3, 0), (0, 0), (3, 1), (2, 1), (2, 2), (2, 0), (1, 0), (1, 1))
SLOTS = ((0, 1, 2, 3, 4), (3, 4,), (2, 3, 4))
LNROWS = 96
LOG2E = 1.4426950408889634
QSCALE = DH ** -0.5 * LOG2E
NEG = -1e30
ONES_ROW = (23, 23, 0, 0)
XPARTS = ((0, 128), (128, 384), (512, 512), (1024, 1024))
ROT = (32, 64, 96, 0)
RANGES = ((0b0001, 0b0010, 0b0100, 0b1000, 0b1101, 0b1011, 0b0111, 0b1001, 0b0110, 0b0011, 0b1100))

f32, bf16, u32 = jnp.float32, jnp.bfloat16, jnp.uint32


def _dot(a, b):
    return jnp.dot(a, b, preferred_element_type=f32)


def _dot_nt(a, b):
    return jax.lax.dot_general(a, b, (((1,), (1,)), ((), ())), preferred_element_type=f32)


def _rnd(a):
    return a.astype(bf16).astype(f32)


def _rcp(a):
    return pltpu.reciprocal(a, full_range=False)


def _iota(shape, axis):
    return jax.lax.broadcasted_iota(jnp.int32, shape, axis)


def _pad_to_tile(a):
    if a.shape[1] < T:
        a = jnp.concatenate([a, jnp.zeros((a.shape[0], T - a.shape[1]), a.dtype)], axis=1)
    if a.shape[0] < T:
        a = jnp.concatenate([a, jnp.zeros((T - a.shape[0], T), a.dtype)], axis=0)
    return a


def _roll(a, shift):
    return pltpu.roll(a, shift % T, 1) if shift % T else a


def _phi(t):
    return jnp.where(t > 0, t + 1.0, jnp.exp(t))


def _head_of(i):
    return ((i >= DH).astype(jnp.int32) + (i >= 2 * DH).astype(jnp.int32)
            + (i >= 3 * DH).astype(jnp.int32) + (i >= 4 * DH).astype(jnp.int32))


class _Packed:
    def __init__(self, ref):
        self.words = ref

    def _index(self, idx):
        *lead, rows, cols = idx
        start, stop, _ = rows.indices(2 * self.words.shape[-2])
        return (*lead, slice(start // 2, stop // 2), cols)

    def __getitem__(self, idx):
        return pltpu.bitcast(self.words[self._index(idx)], bf16)

    def __setitem__(self, idx, value):
        self.words[self._index(idx)] = pltpu.bitcast(value, u32)


def run(gen):
    try:
        while True:
            next(gen)
    except StopIteration as stop:
        return stop.value


def _kernel(x_hbm, wq_hbm, wk_hbm, wv_hbm, wo_hbm, beta_hbm, wr_hbm, wg_hbm, wu_hbm,
            wd_hbm, o_hbm,
            x_v, w_v, beta_v, wr_v, wg_v, wu_v, wd_v, wt, wrc, xn_v, qm, vl, kn, ot, mst, zst,
            gcol, r_v, hot, o_v, causal, lanes, sem):
    xn_v, qm, kn = (_Packed(r) for r in (xn_v, qm, kn))
    x_cp = [pltpu.make_async_copy(x_hbm.at[:, pl.ds(t, n)], x_v.at[:, pl.ds(t, n)], sem.at[7 + i])
            for i, (t, n) in enumerate(XPARTS)]
    w_cp = [pltpu.make_async_copy(w, w_v.at[i], sem.at[i]) if i else None
            for i, w in enumerate((wq_hbm, wk_hbm, wv_hbm, wo_hbm))]
    wq_cp = [pltpu.make_async_copy(wq_hbm.at[:, pl.ds(c, n)], w_v.at[0, :, pl.ds(c, n)], sm)
             for c, n, sm in ((0, 2 * T, sem.at[0]), (2 * T, D - 2 * T, sem.at[7 + len(XPARTS)]))]
    f_cp = [pltpu.make_async_copy(a, b, sem.at[4])
            for i, (a, b) in enumerate(((wg_hbm, wg_v), (wu_hbm, wu_v), (wd_hbm, wd_v)))]
    c_cp = [pltpu.make_async_copy(a, b, sem.at[5])
            for i, (a, b) in enumerate(((wr_hbm, wr_v), (beta_hbm, beta_v)))]
    o_cp = [[pltpu.make_async_copy(o_v.at[s, pl.ds(p * 2 * G, 2 * G)],
                                   o_hbm.at[pl.ds(p * 2 * G, 2 * G), pl.ds(s * L, L)],
                                   sem.at[6]) for p in range(NP)] for s in range(NSEG)]

    fillers = []

    lane8 = _iota((8, T), 1)
    never = lane8 < jnp.min(lane8, axis=1, keepdims=True)
    zero = jnp.min(lane8)
    link = [None, None]

    def tie(a, b):
        return a if b is None else jnp.where(never, b, a)

    def fill(after=None):
        link[0], link[1] = after, None
        while fillers:
            if next(fillers[0], False):
                break
            fillers.pop(0)
        return link[1]

    def drain():
        while fillers:
            fill()

    def gate_column():
        gate = jax.nn.sigmoid(beta_v[...].astype(f32))
        gate = jnp.concatenate([gate, jnp.zeros((1, T - H), f32)], axis=1)
        gate = jnp.broadcast_to(gate, (T, T)).T
        r8 = _iota((8, T), 0)
        for v in range(D // 8):
            h0, h1 = (8 * v) // DH, (8 * v + 7) // DH
            gv = jnp.broadcast_to(gate[h0:h0 + 1], (8, T))
            if h1 != h0:
                gv = jnp.where(r8 < h1 * DH - 8 * v, gv, jnp.broadcast_to(gate[h1:h1 + 1], (8, T)))
            gcol[8 * v:8 * v + 8, :] = gv
            if v % 9 == 8:
                yield True

    def router_column():
        wr = wr_v[...].astype(f32).reshape(1, D)
        wr = jnp.concatenate([wr, jnp.zeros((1, DP - D), f32)], axis=1)
        wrc[...] = jnp.broadcast_to(wr, (T, DP)).T[0:D]

    def transpose_w(i, lo=0, hi=D):
        for c in range(lo, hi, T):
            n = min(T, D - c)
            for k in range(0, D, T):
                w = _pad_to_tile(w_v[i, k:min(k + T, D), c:c + n].astype(f32))
                w = jnp.concatenate([tie(w[r:r + 8], link[0]) for r in range(0, T, 8)], axis=0).T
                wt[i, c:c + n, k:k + T] = w[0:n]
                yield True

    normed = [0]

    def layernorm(b, step):

        def chain(acc, v):
            h = v.shape[0] // 16 * 8
            a, c = v[0:8], v[h:h + 8]
            for k in range(8, h, 8):
                a, c = a + v[k:k + 8], c + v[h + k:h + k + 8]
            return a + c if acc is None else acc + (a + c)

        def rows(v):
            return jnp.concatenate([tie(v, link[0])] * (step // 8), axis=0)

        def bcast(v):
            return jnp.broadcast_to(v, (8, T))

        def load(r, n):
            return x_v[r:r + step, pl.ds(pl.multiple_of((b + n * zero) * T, T), T)].astype(f32)

        acc = jnp.zeros((8, T), f32)
        for r in range(0, D, step):
            x = load(r, 0)
            link[1] = acc = chain(tie(acc, link[0]), x)
            yield True
        mean = bcast(jnp.sum(acc, axis=0, keepdims=True) * (1.0 / D))
        acc = None
        for r in range(0, D, step):
            xc = load(r, 1) - rows(mean)
            link[1] = acc = chain(acc, xc * xc)
            yield True
        var = bcast(jnp.sum(acc, axis=0, keepdims=True) * (1.0 / D))
        sd = _rnd(jnp.sqrt(_rnd(_rnd(var) + _rnd(jnp.full((8, T), 1e-5, f32)))))
        inv, mean = jnp.concatenate([1.0 / sd] * (step // 8), axis=0), _rnd(mean)
        acc = None
        for r in range(0, D, step):
            x = load(r, 2)
            xn = (_rnd(x - rows(mean)) * inv).astype(bf16)
            xn_v[b, r:r + step, :] = xn
            link[1] = acc = chain(acc, xn.astype(f32) * wrc[r:r + step, :])
            if r + step == D:
                xn_v[b, D:DP, :] = jnp.zeros((DP - D, T), bf16)
                r_v[b:b + 1, :] = _rnd(jnp.sum(acc, axis=0, keepdims=True))
                normed[0] += 1
            yield True

    late = [None] * LATE
    deferred = []
    arrivals = {}
    small = []

    def proj(i, s, g, slots):
        acc = None
        for k in range(0, DP, T):
            xs = jnp.concatenate([xn_v[s * NT + c, k:k + T, :] for c in range(NT)], axis=1)
            w = wt[i, g * G:(g + 1) * G, k:k + T]
            if (i, s, g, k) == WO_READY:
                done = wt[zero, pl.ds(pl.multiple_of(zero * 8, 8), 8),
                          pl.ds(pl.multiple_of(zero * T, T), T)]
                w = jnp.concatenate([w[:-8], tie(w[-8:], done)], axis=0)
            if (i, s, g) in arrivals and k == WAIT_K * T:
                arrivals.pop((i, s, g))()
            d = _dot(w, xs)
            done = late.pop(0)
            top = tie(d[-8:, :T], done)
            d = jnp.concatenate([d[:-8], jnp.concatenate([top, d[-8:, T:]], axis=1)], axis=0)
            acc = d if acc is None else acc + d
            late.append(fill(d[0:8, 0:T]) if k // T in slots else None)
            if small and k // T in (SLOTS3 if s == 3 else SLOTS2[i]):
                next(small[0], None)
        yield 5 * G
        while deferred:
            deferred.pop(0)()
            yield G
        return acc

    def project_q(s, g):
        q = yield from proj(0, s, g, SLOTS[0])
        r8 = _iota((8, L), 0)
        qs = q * QSCALE
        for h in range(4):
            lo = 16 * h
            a0, a1, a2 = qs[lo:lo + 8], qs[lo + 8:lo + 16], qs[lo + 16:lo + 24]
            if h > 0:
                a0 = jnp.where(r8 >= 2 * h, a0, 0.0)
            if h < 3:
                a2 = jnp.where(r8 < 2 * h + 2, a2, 0.0)
            w = pltpu.bitcast(jnp.concatenate(
                [a0, a1, a2, jnp.zeros((8, L), f32)], axis=0).astype(bf16), u32)
            for c in range(0, L, T):
                qm.words[s, 4 * g + h, :, c:c + T] = _roll(w[:, c:c + T], ROT[h])
        if s > 0:
            deferred.append(functools.partial(memory_read, s, g, _phi(q)))

    def memory_read(s, g, pq):
        r8 = _iota((8, L), 0)
        same_head = _head_of(_iota((G, T), 0)) == _head_of(_iota((G, T), 1))
        num = _dot(jnp.where(same_head, mst[g], 0.0),
                   jnp.concatenate([pq, jnp.zeros((T - G, L), f32)], axis=0).astype(bf16))
        t = pq * jnp.concatenate([zst[g]] * NT, axis=1)
        t = [t[r:r + 8] for r in range(0, G, 8)]
        ib = []
        for h in range(4):
            a, b, c = t[2 * h:2 * h + 3]
            if h > 0:
                a = jnp.where(r8 >= 2 * h, a, 0.0)
            if h < 3:
                c = jnp.where(r8 < 2 * h + 2, c, 0.0)
            den = jnp.sum(a + b + c, axis=0, keepdims=True)
            ib.append(_rcp(jnp.broadcast_to(den, (8, L)) + 1e-6))
        iv = jnp.concatenate(
            [ib[0], ib[0], jnp.where(r8 < 2, ib[0], ib[1]), ib[1],
             jnp.where(r8 < 4, ib[1], ib[2]), ib[2],
             jnp.where(r8 < 6, ib[2], ib[3]), ib[3], ib[3]], axis=0)
        gg = gcol[g * G:(g + 1) * G, :]
        ot[s, g * G:(g + 1) * G, :] = num * iv * jnp.concatenate([gg] * NT, axis=1)

    def memory_update(s, g, v, pk, z):
        upd = _dot_nt(v, pk)
        mst[g] = upd if s == 0 else mst[g] + upd
        zst[g] = z if s == 0 else zst[g] + z

    def project_k(s, g):
        k = yield from proj(1, s, g, SLOTS[1] if s else SLOTS[2])
        zpad = jnp.zeros((T - G, L), f32)
        kn[s, g, :, :] = jnp.concatenate([k, zpad], axis=0).astype(bf16).T
        if s < NSEG - 1:
            pk = _phi(k)
            z = sum(pk[:, c:c + T] for c in range(T, L, T)) + pk[:, :T]
            z = jnp.broadcast_to(jnp.sum(z, axis=1, keepdims=True), (G, T))
            return jnp.concatenate([pk, zpad], axis=0).astype(bf16), z

    def project_v(s, g, pk):
        v = yield from proj(2, s, g, SLOTS[2] if s else SLOTS[0])
        for h in range(4):
            a = [v[16 * h + c:16 * h + c + 8] for c in (0, 8, 16)]
            c, r = divmod(ONES_ROW[h], 8)
            a[c] = jnp.where(_iota((8, L), 0) == r, 1.0, a[c])
            vl[s, 4 * g + h] = jnp.concatenate(a, axis=0)
        if pk is not None:
            deferred.append(functools.partial(memory_update, s, g, v, *pk))

    def attention(segs):
        r8 = _iota((8, T), 0)
        units = [(s, g, i, j) for s in segs for g in range(NG) for i, j in ORDER]
        run, accs = {}, {}

        lane32 = _iota((32, T), 1)
        carry = {}

        def own_queries(s, g, i):
            w = []
            for h in range(4):
                parts = [qm[s, 4 * g + h, :, i * T:(i + 1) * T]]
                if h > 0:
                    parts.insert(0, jnp.zeros((16 * h, T), bf16))
                parts.append(jnp.zeros((T - 32 - 16 * h, T), bf16))
                w.append(jnp.concatenate(parts, axis=0))
            return jnp.concatenate(w, axis=1)

        def shared_queries(qw, *parts):
            slots = [None] * 8
            for h, quarters in parts:
                for e in range(2):
                    t = qw[h][8 * e:8 * e + 8] & lanes[RANGES.index(quarters)]
                    slots[h + e] = t if slots[h + e] is None else t | slots[h + e]
            slots = [jnp.zeros((8, T), u32) if t is None else t for t in slots]
            return pltpu.bitcast(jnp.concatenate(slots, axis=0), bf16)

        def diagonal_scores(s, g, i):
            k0 = i * T
            own = carry.pop("own") if i else _dot(kn[s, g, 0:32, :], own_queries(s, g, 0))
            qw = [qm.words[s, 4 * g + h, :, k0:k0 + T] for h in range(4)]
            x = _dot(kn[s, g, k0 + 32:k0 + 64, :], jnp.concatenate(
                [shared_queries(qw, (h, 15 - (2 << h)), (3, 2 << h)) for h in range(3)], axis=1))
            y = _dot(kn[s, g, k0 + 64:k0 + 96, :], jnp.concatenate(
                [shared_queries(qw, (0, 0b1001), (2, 0b0110)),
                 shared_queries(qw, (1, 0b0011), (3, 0b1100))], axis=1))
            z = _dot(kn[s, g, k0 + 96:k0 + T, :],
                     shared_queries(qw, *[(h, 1 << h) for h in range(4)]))
            xs = [x[:, h * T:(h + 1) * T] for h in range(3)]
            xs.append(jnp.where(lane32 < 64, xs[0], jnp.where(lane32 < 96, xs[1], xs[2])))
            ys = [y[:, :T], y[:, T:]] * 2
            zs = [z] * 4
            return [jnp.concatenate([own[:, h * T:(h + 1) * T], xs[h], ys[h], zs[h]], axis=0)
                    for h in range(4)]

        def scores(s, g, i, j):
            if i == j:
                shs = diagonal_scores(s, g, i)
            else:
                more = 32 if j == i - 1 else 0
                st = _dot(kn[s, g, j * T:(j + 1) * T + more, :],
                          own_queries(s, g, i))
                if more:
                    carry["own"] = st[T:]
                shs = [st[:T, h * T:(h + 1) * T] for h in range(4)]
            ps, alphas = [], []
            later = any(a == i for a, _ in ORDER[:ORDER.index((i, j))])
            for h in range(4):
                sh = shs[h]
                if i == j:
                    sh = sh + causal[h]
                m = jnp.max(sh, axis=0, keepdims=True)
                if later:
                    m = jnp.maximum(m, run[i, h])
                    alphas.append(jnp.exp2(run[i, h] - m))
                run[i, h] = m
                ps.append(jnp.exp2(sh - m).astype(bf16))
            return ps, alphas

        def values(s, g, i, j, ps, alphas):
            new = [_dot(vl[s, 4 * g + h, :, j * T:(j + 1) * T], ps[h]) for h in range(4)]
            if alphas:
                new = [a * al + b for a, al, b in zip(accs.pop(i), alphas, new)]
            if any(a == i for a, _ in ORDER[ORDER.index((i, j)) + 1:]):
                accs[i] = new
                return
            o = []
            for h in range(4):
                inv = _rcp(jnp.broadcast_to(new[h][ONES_ROW[h]:ONES_ROW[h] + 1], (8, T)))
                o.append([_roll(new[h][8 * c:8 * c + 8] * inv, -ROT[h]) for c in range(3)])
            a_dot = jnp.concatenate(
                [o[0][0], o[0][1], jnp.where(r8 < 2, o[0][2], o[1][0]), o[1][1],
                 jnp.where(r8 < 4, o[1][2], o[2][0]), o[2][1],
                 jnp.where(r8 < 6, o[2][2], o[3][0]), o[3][1], o[3][2]], axis=0)
            dst = (s, slice(g * G, (g + 1) * G), slice(i * T, (i + 1) * T))
            mix = (1.0 - gcol[g * G:(g + 1) * G, :]) * a_dot
            ot[dst] = ot[dst] + mix if s > 0 else mix

        pend = {}
        for t in range(len(units) + LAG):
            if t < len(units):
                pend[t] = scores(*units[t])
            if t >= LAG:
                values(*units[t - LAG], *pend.pop(t - LAG))
            yield t < len(units) and units[t][2] != units[t][3]

    def out_proj(s):
        o = jnp.concatenate(
            [ot[s], hot[:, s * L:(s + 1) * L], jnp.zeros((DP - D - 8, L), f32)], axis=0).astype(bf16)
        for p in range(NP):
            rows = slice(p * 2 * G, (p + 1) * 2 * G)
            halves = []
            for g in (2 * p, 2 * p + 1):
                a = None
                for k in range(0, DP, T):
                    d = _dot(wt[3, g * G:(g + 1) * G, k:k + T], o[k:k + T])
                    a = d if a is None else a + d
                halves.append(a)
                yield 5 * G
            a = jnp.concatenate(halves, axis=0)
            for c in range(NT):
                b = s * NT + c
                res = x_v[rows, b * T:(b + 1) * T].astype(f32) + xn_v[b, rows, :].astype(f32)
                o_v[s, rows, c * T:(c + 1) * T] = (res + a[:, c * T:(c + 1) * T]).astype(bf16)
            o_cp[s][p].start()

    routed = {}

    def row_block(ref, k, cols):
        w = ref[k:min(k + T, D), cols]
        if k + T > D:
            w = jnp.concatenate([w, jnp.zeros((DP - D, w.shape[1]), bf16)], axis=0)
        return w

    def route():
        def both(op, a):
            return op(op(a, axis=0, keepdims=True), axis=1, keepdims=True)

        r = r_v[...]
        idx = (_iota(r.shape, 0) * T + _iota(r.shape, 1)).astype(f32)
        m1 = both(jnp.max, r)
        i1 = both(jnp.min, jnp.where(r == m1, idx, S))
        r = jnp.where(idx == i1, -jnp.inf, r)
        m2 = both(jnp.max, r)
        i2 = both(jnp.min, jnp.where((r == m2) & (idx != i1), idx, S))
        row = _iota((8, T), 0)
        routed["w"] = jax.nn.sigmoid(jnp.where(row == 0, m1, m2))
        pick = jnp.where(row == 0, i1, jnp.where(row == 1, i2, -1.0))
        for b in range(S // T):
            hot[:, b * T:(b + 1) * T] = (pick == (lane8 + b * T).astype(f32)).astype(f32)
        for _ in range(ROUTE_WAIT):
            yield True
        blocks = [jnp.broadcast_to(i.astype(jnp.int32) >> 7, (32, T)) for i in (i1, i2)]
        tiles = [[], []]
        for r0 in range(0, DP // 2, 32):
            acc = [xn_v.words[0, r0:r0 + 32, :]] * 2
            for b in range(1, S // T):
                w = xn_v.words[b, r0:r0 + 32, :]
                acc = [jnp.where(blocks[n] == b, w, acc[n]) for n in range(2)]
            for n in range(2):
                tiles[n].append(acc[n])
            if r0 % 64:
                yield True
        x = None
        for n, i in enumerate((i1, i2)):
            pick = (row == n) & (lane8 == (i.astype(jnp.int32) & (T - 1)))
            d = _dot_nt(pick.astype(f32), pltpu.bitcast(jnp.concatenate(tiles[n], axis=0), bf16))
            x = d if x is None else x + d
        routed["x"] = [x[:, k:k + T] for k in range(0, DP, T)]

    def ffn_hidden():
        routed["h"] = []
        for n in range(0, F, L):
            gu = []
            for w_ref in (wg_v, wu_v):
                acc = None
                for c, k in enumerate(range(0, D, T)):
                    d = _dot(routed["x"][c], row_block(w_ref, k, slice(n, n + L)))
                    acc = d if acc is None else acc + d
                    yield True
                gu.append(acc)
            routed["h"].append(gu[0] * jax.nn.sigmoid(gu[0]) * gu[1])

    def ffn_down():
        for k in range(0, D, T):
            acc = None
            for c, n in enumerate(range(0, F, L)):
                d = _dot_nt(routed["h"][c], row_block(wd_v, k, slice(n, n + L)))
                acc = d if acc is None else acc + d
                yield
            y = jnp.concatenate([jnp.zeros((D - 4 * T, T), f32), acc * routed["w"],
                                 jnp.zeros((DP - D - 8, T), f32)], axis=0).T
            dst = (3, slice(k, min(k + T, D)), slice(4 * T, DP))
            wt[dst] = wt[dst] + y[0:min(T, D - k)]

    for c in (*c_cp, *x_cp[:2], *wq_cp, *w_cp[1:3]):
        c.start()
    for h in range(4):
        query = (_iota((T, T), 1) - ROT[h]) & (T - 1)
        causal[h] = jnp.where(_iota((T, T), 0) <= query, 0.0, NEG)
    for n, quarters in enumerate(RANGES):
        lanes[n] = pltpu.bitcast(-((quarters >> (lane8 >> 5)) & 1), u32)
    for c in c_cp:
        c.wait()
    router_column()
    for _ in gate_column():
        pass
    for b in range(NT):
        if b < 2:
            x_cp[b].wait()
        fillers.append(layernorm(b, LNROWS0))
        prev = [None, None]
        while fillers:
            prev.append(fill(prev.pop(0)))
    x_cp[2].start()
    wq_cp[0].wait()
    fillers.append(transpose_w(0, 0, 2 * T))
    drain()

    def rest_of_wq():
        wq_cp[1].wait()
        run(transpose_w(0, 2 * T))

    def wk_arrives():
        for c in (x_cp[3], w_cp[3]):
            c.start()
        w_cp[1].wait()
        run(transpose_w(1))

    def wv_arrives():
        for ref in (wg_v, wu_v, wd_v):
            ref[0:16, 0:T] = kn[0, 0, 0:16, :]
        for c in f_cp:
            c.start()
        for c in (w_cp[2], x_cp[2]):
            c.wait()
        run(transpose_w(2))
        fillers.extend(layernorm(b, LNROWS1) for b in range(NT, 2 * NT))

    def wo_arrives():
        for c in (x_cp[3], w_cp[3]):
            c.wait()
        fillers.extend(layernorm(b, LNROWS) for b in range(2 * NT, S // T))
        small.append(transpose_w(3))

    def ffn_arrives():
        for c in f_cp:
            c.wait()
        run(small.pop())
        small.append(ffn_hidden())

    arrivals.update({(0, 0, 2): rest_of_wq, (0, 0, NG - 1): wk_arrives, (1, 0, NG - 1): wv_arrives,
                     (0, 1, 0): wo_arrives, FWAIT: ffn_arrives})
    for g in range(NG):
        run(project_q(0, g))
    pks = [run(project_k(0, g)) for g in range(NG)]
    for g in range(NG):
        run(project_v(0, g, pks[g]))

    def dense(s):
        while normed[0] < (s + 1) * NT:
            fill()
        for g in range(NG):
            yield from project_q(s, g)
            yield from project_v(s, g, (yield from project_k(s, g)))

    def weave(main, steps, other, rows, extra=iter(())):
        done = 0
        for t in range(steps):
            if next(main):
                next(extra, None)
            while done < (t + 1) * rows // steps:
                done += next(other, rows)

    def finish(main, other):
        for _ in range(LAG):
            next(other)
            next(main)
        run(main)
        run(other)

    per_seg = NG * len(ORDER)
    seg_rows = NP * (15 * 2 * G + 4 * (G + 8))
    run(dense(1))
    run(dense(2))
    drain()
    att, steps = attention([0]), dense(3)
    weave(att, ROUTE_AT, iter(()), 0)
    routing = route()
    weave(att, per_seg - ROUTE_AT, iter(()), 0, routing)
    run(routing)
    finish(att, steps)
    run(small[0])
    drain()
    att = attention(range(1, NSEG))
    steps = ffn_down()
    weave(att, per_seg, iter(()), 0, steps)
    run(steps)
    outs = (n for s in range(NSEG - 1) for n in out_proj(s))
    weave(att, 2 * per_seg, outs, 3 * NP * 5 * 2 * G - TAIL * G)
    finish(att, outs)
    run(out_proj(NSEG - 1))
    for cs in o_cp:
        for c in cs:
            c.wait()


@jax.jit
def pallas_parallel_sum__memory_aug_infini_attn__moe_arch_mod__prompt_kernel(
    A_x: jax.Array,
    A_wq: jax.Array,
    A_wk: jax.Array,
    A_wv: jax.Array,
    A_wo: jax.Array,
    A_beta: jax.Array,
    B_x: jax.Array,
    B_w_r: jax.Array,
    B_w_gate: jax.Array,
    B_w_up: jax.Array,
    B_w_down: jax.Array,
):
    del B_x
    hbm = pl.BlockSpec(memory_space=pltpu.HBM)
    out = pl.pallas_call(
        _kernel,
        out_shape=jax.ShapeDtypeStruct((D, S), A_x.dtype),
        in_specs=[hbm] * 10,
        out_specs=hbm,
        scratch_shapes=[
            pltpu.VMEM((D, S), bf16),
            pltpu.VMEM((4, D, D), bf16),
            pltpu.VMEM((1, H), bf16),
            pltpu.VMEM((D,), bf16),
            pltpu.VMEM((D, F), bf16),
            pltpu.VMEM((D, F), bf16),
            pltpu.VMEM((D, F), bf16),
            pltpu.VMEM((4, D, DP), f32),
            pltpu.VMEM((D, T), f32),
            pltpu.VMEM((S // T, DP // 2, T), u32),
            pltpu.VMEM((NSEG, H, 16, L), u32),
            pltpu.VMEM((NSEG, H, 24, L), f32),
            pltpu.VMEM((NSEG, NG, L // 2, T), u32),
            pltpu.VMEM((NSEG, D, L), f32),
            pltpu.VMEM((NG, G, T), f32),
            pltpu.VMEM((NG, G, T), f32),
            pltpu.VMEM((D, T), f32),
            pltpu.VMEM((S // T, T), f32),
            pltpu.VMEM((8, S), f32),
            pltpu.VMEM((NSEG, D, L), bf16),
            pltpu.VMEM((4, T, T), f32),
            pltpu.VMEM((len(RANGES), 8, T), u32),
            pltpu.SemaphoreType.DMA((8 + len(XPARTS),)),
        ],
        compiler_params=pltpu.CompilerParams(vmem_limit_bytes=100 * 2**20),
    )(A_x.reshape(S, D).T, A_wq, A_wk, A_wv, A_wo, A_beta.reshape(1, H), B_w_r,
      B_w_gate, B_w_up, B_w_down.T)
    return out.T.reshape(A_x.shape)
```

```python
import functools

import jax
import jax.numpy as jnp
import jax.experimental.pallas as pl
import jax.experimental.pallas.tpu as pltpu

S, D, H, DH, NSEG, L, F = 2048, 576, 32, 18, 4, 512, 4608
DP = 640
G = 4 * DH
NG = H // 4
T = 128
NT = L // T
NP = NG // 2
LATE = 2
SOONM = 9
SOONR = (0, 24, 40, 64)
SOON = 9
HK = 256
DEFER = 4
OSTEPS = (2, 5, 8)
WAIT_Q = (0, 0, 0, 9)
WAIT_V = (1, 0, 3, 4)
WAIT_O = (0, 1, 0, 4)
SLOTS0 = ((0, 1, 2, 3, 4, 7, 8, 9), (5, 8), (0, 1, 2, 3, 4, 5, 6, 7, 8))
ROUTE_AT = 30
WO_READY = (0, 2, 1, 2)
FWAIT = (0, 3, 1, 0)
WAIT_K = (0, 0, 3, 4)
SLOTS2 = ((), (7,), (1, 7))
TAIL = 27
SLOTS3 = (0, 1, 2, 3, 4, 5, 6, 7, 8)
ROUTE_WAIT = 5
LNROWS0 = (144, 144, 144)
LNROWS1 = (576, 288, 96, 128)
LAG = 2
ORDER = ((3, 2), (3, 3), (3, 0), (0, 0), (3, 1), (2, 1), (2, 2), (2, 0), (1, 0), (1, 1))
SLOTS = ((0,1,2,3,4,5,6,7,8),(0,1,2,3,4,5,6,7,8),(0,1,2,3,4,5,6,7,8))
LNROWS = (192, 96, 48, 32)
LOG2E = 1.4426950408889634
QSCALE = DH ** -0.5 * LOG2E
NEG = -1e30
ONES_ROW = (23, 23, 0, 0)
XPARTS = ((0, 128), (128, 384), (512, 512), (1024, 1024))
ROT = (32, 64, 96, 0)
RANGES = ((0b0001, 0b0010, 0b0100, 0b1000, 0b1101, 0b1011, 0b0111, 0b1001, 0b0110, 0b0011, 0b1100))

f32, bf16, u32 = jnp.float32, jnp.bfloat16, jnp.uint32


def _dot(a, b):
    return jnp.dot(a, b, preferred_element_type=f32)


def _dot_nt(a, b):
    return jax.lax.dot_general(a, b, (((1,), (1,)), ((), ())), preferred_element_type=f32)


def _rnd(a):
    return a.astype(bf16).astype(f32)


def _rcp(a):
    return pltpu.reciprocal(a, full_range=False)


def _iota(shape, axis):
    return jax.lax.broadcasted_iota(jnp.int32, shape, axis)


def _pad_to_tile(a):
    if a.shape[1] < T:
        a = jnp.concatenate([a, jnp.zeros((a.shape[0], T - a.shape[1]), a.dtype)], axis=1)
    if a.shape[0] < T:
        a = jnp.concatenate([a, jnp.zeros((T - a.shape[0], T), a.dtype)], axis=0)
    return a


def _roll(a, shift):
    return pltpu.roll(a, shift % T, 1) if shift % T else a


def _phi(t):
    return jnp.where(t > 0, t + 1.0, jnp.exp(t))


def _head_of(i):
    return ((i >= DH).astype(jnp.int32) + (i >= 2 * DH).astype(jnp.int32)
            + (i >= 3 * DH).astype(jnp.int32) + (i >= 4 * DH).astype(jnp.int32))


class _Packed:
    def __init__(self, ref):
        self.words = ref

    def _index(self, idx):
        *lead, rows, cols = idx
        start, stop, _ = rows.indices(2 * self.words.shape[-2])
        return (*lead, slice(start // 2, stop // 2), cols)

    def __getitem__(self, idx):
        return pltpu.bitcast(self.words[self._index(idx)], bf16)

    def __setitem__(self, idx, value):
        self.words[self._index(idx)] = pltpu.bitcast(value, u32)


def run(gen):
    try:
        while True:
            next(gen)
    except StopIteration as stop:
        return stop.value


def _kernel(x_hbm, wq_hbm, wk_hbm, wv_hbm, wo_hbm, beta_hbm, wr_hbm, wg_hbm, wu_hbm,
            wd_hbm, o_hbm,
            x_v, w_v, beta_v, wr_v, wg_v, wu_v, wd_v, wt, wrc, xn_v, bsum, qm, vl, kn, ot, mst, zst,
            gcol, r_v, hot, o_v, causal, lanes, sem):
    xn_v, bsum, qm, kn = (_Packed(r) for r in (xn_v, bsum, qm, kn))
    x_cp = [pltpu.make_async_copy(x_hbm.at[:, pl.ds(t, n)], x_v.at[:, pl.ds(t, n)], sem.at[7 + i])
            for i, (t, n) in enumerate(XPARTS)]
    w_cp = [pltpu.make_async_copy(w, w_v.at[i], sem.at[i]) if i else None
            for i, w in enumerate((wq_hbm, wk_hbm, wv_hbm, wo_hbm))]
    wq_cp = [pltpu.make_async_copy(wq_hbm.at[:, pl.ds(c, n)], w_v.at[0, :, pl.ds(c, n)], sm)
             for c, n, sm in ((0, 2 * T, sem.at[0]), (2 * T, D - 2 * T, sem.at[7 + len(XPARTS)]))]
    f_cp = [pltpu.make_async_copy(a, b, sem.at[4])
            for i, (a, b) in enumerate(((wg_hbm, wg_v), (wu_hbm, wu_v), (wd_hbm, wd_v)))]
    c_cp = [pltpu.make_async_copy(a, b, sem.at[5])
            for i, (a, b) in enumerate(((wr_hbm, wr_v), (beta_hbm, beta_v)))]
    o_cp = [[pltpu.make_async_copy(o_v.at[s, pl.ds(p * 2 * G, 2 * G)],
                                   o_hbm.at[pl.ds(p * 2 * G, 2 * G), pl.ds(s * L, L)],
                                   sem.at[6]) for p in range(NP)] for s in range(NSEG)]

    fillers = []

    lane8 = _iota((8, T), 1)
    never = lane8 < jnp.min(lane8, axis=1, keepdims=True)
    zero = jnp.min(lane8)
    link = [None, None]

    def tie(a, b):
        return a if b is None else jnp.where(never, b, a)

    def fill(after=None):
        link[0], link[1] = after, None
        while fillers:
            if next(fillers[0], False):
                break
            fillers.pop(0)
        return link[1]

    def drain():
        while fillers:
            fill()

    def gate_column():
        gate = jax.nn.sigmoid(beta_v[...].astype(f32))
        gate = jnp.concatenate([gate, jnp.zeros((1, T - H), f32)], axis=1)
        gate = jnp.broadcast_to(gate, (T, T)).T
        r8 = _iota((8, T), 0)
        for v in range(D // 8):
            h0, h1 = (8 * v) // DH, (8 * v + 7) // DH
            gv = jnp.broadcast_to(gate[h0:h0 + 1], (8, T))
            if h1 != h0:
                gv = jnp.where(r8 < h1 * DH - 8 * v, gv, jnp.broadcast_to(gate[h1:h1 + 1], (8, T)))
            gcol[8 * v:8 * v + 8, :] = gv
            if v % 9 == 8:
                yield True

    def router_column():
        wr = wr_v[...].astype(f32).reshape(1, D)
        wr = jnp.concatenate([wr, jnp.zeros((1, DP - D), f32)], axis=1)
        wrc[...] = jnp.broadcast_to(wr, (T, DP)).T[0:D]

    def transpose_w(i, lo=0, hi=D):
        for c in range(lo, hi, T):
            n = min(T, D - c)
            for k in range(0, D, T):
                w = _pad_to_tile(w_v[i, k:min(k + T, D), c:c + n].astype(f32))
                w = jnp.concatenate([tie(w[r:r + 8], link[0]) for r in range(0, T, 8)], axis=0).T
                wt[i, c:c + n, k:k + T] = w[0:n]
                yield True

    normed = [0]

    def layernorm(b, steps):

        def chain(acc, v):
            h = v.shape[0] // 16 * 8
            a, c = v[0:8], v[h:h + 8]
            for k in range(8, h, 8):
                a, c = a + v[k:k + 8], c + v[h + k:h + k + 8]
            return a + c if acc is None else acc + (a + c)

        def rows(v):
            return jnp.concatenate([tie(v, link[0])] * (step // 8), axis=0)

        def bcast(v):
            return jnp.broadcast_to(v, (8, T))

        def load(r, n):
            return x_v[r:r + step, pl.ds(pl.multiple_of((b + n * zero) * T, T), T)].astype(f32)

        acc, step = jnp.zeros((8, T), f32), steps[0]
        for r in range(0, D, step):
            x = load(r, 0)
            link[1] = acc = chain(tie(acc, link[0]), x)
            yield True
        mean = bcast(jnp.sum(acc, axis=0, keepdims=True) * (1.0 / D))
        acc, step = None, steps[1]
        for r in range(0, D, step):
            xc = load(r, 1) - rows(mean)
            link[1] = acc = chain(acc, xc * xc)
            yield True
        var = bcast(jnp.sum(acc, axis=0, keepdims=True) * (1.0 / D))
        sd = _rnd(jnp.sqrt(_rnd(_rnd(var) + _rnd(jnp.full((8, T), 1e-5, f32)))))
        step = steps[2]
        inv, mean = jnp.concatenate([1.0 / sd] * (step // 8), axis=0), _rnd(mean)
        acc = None
        for r in range(0, D, step):
            x = load(r, 2)
            xn = (_rnd(x - rows(mean)) * inv).astype(bf16)
            xn_v[b, r:r + step, :] = xn
            link[1] = acc = chain(acc, xn.astype(f32) * wrc[r:r + step, :])
            if r + step == D:
                xn_v[b, D:DP, :] = jnp.zeros((DP - D, T), bf16)
                r_v[b:b + 1, :] = _rnd(jnp.sum(acc, axis=0, keepdims=True))
            yield True

    late = [None] * LATE
    deferred = []
    soon = []
    arrivals = {}
    small = []

    def combine(s, rows):
        for c in range(NT // 2):
            for r in range(0, HK, rows):
                b11, b12, b21, b22 = (
                    xn_v[s * NT + c + n + zero, k + r:k + r + rows, :].astype(f32)
                    for k in (0, HK) for n in (0, NT // 2))
                b11 = jnp.concatenate(
                    [tie(b11[k:k + 8], link[0]) for k in range(0, rows, 8)], axis=0)
                for n, t in enumerate((b11 + b22, b12 - b22, b21 - b11, b11 + b12, b21 + b22)):
                    bsum[s, n, r:r + rows, c * T:(c + 1) * T] = t.astype(bf16)
                    link[1] = tie(t[-8:], link[1])
                normed[0] += c == NT // 2 - 1 and r + rows == HK
                yield True

    def strassen(i, p, part, sums, rest, step, top, bottom):
        r0, r1 = slice(2 * p * G, (2 * p + 1) * G), slice((2 * p + 1) * G, (2 * p + 2) * G)
        a11, a12 = (lambda: wt[i, r0, 0:HK]), (lambda: wt[i, r0, HK:2 * HK])
        a21, a22 = (lambda: wt[i, r1, 0:HK]), (lambda: wt[i, r1, HK:2 * HK])
        c11 = yield from step(0, a12() - a22(), sums(4))
        m = yield from step(1, a11() + a12(), part(1, 1))
        c11, c12 = c11 - m, m
        m = yield from step(2, wt[i, r0, 2 * HK:DP], rest())
        c11, c12 = c11 + m[:, :HK], c12 + m[:, HK:]
        m = yield from step(3, a11() + a22(), sums(0))
        c11, c22 = c11 + m, m
        m = yield from step(4, a11(), sums(1))
        c12, c22 = c12 + m, c22 + m
        c21 = yield from step(5, a22(), sums(2))
        top(jnp.concatenate([c11 + c21, c12], axis=1))
        m = yield from step(6, a21() + a22(), part(0, 0))
        c21, c22 = c21 + m, c22 - m
        c22 = c22 + (yield from step(7, a21() - a11(), sums(3)))
        m = yield from step(8, wt[i, r1, 2 * HK:DP], rest())
        bottom(jnp.concatenate([c21, c22], axis=1) + m)

    def proj(i, s, p, slots, finish):
        def block(k, n, cs):
            return jnp.concatenate([xn_v[s * NT + c, k:k + n, :] for c in cs], axis=1)

        def step(n, w, xs):
            if (i, s, p, n) == WO_READY:
                done = wt[zero, pl.ds(pl.multiple_of(zero * 8, 8), 8),
                          pl.ds(pl.multiple_of(zero * T, T), T)]
                w = jnp.concatenate([w[:-8], tie(w[-8:], done)], axis=0)
            if (i, s, p, n) in arrivals:
                arrivals.pop((i, s, p, n))()
            d = _dot(w, xs)
            top = tie(d[-8:, :T], late.pop(0))
            for job in soon:
                job[0] -= 1
                if job[0] == -1:
                    top = tie(top, job[1])
            d = jnp.concatenate([d[:-8], jnp.concatenate([top, d[-8:, T:]], axis=1)], axis=0)
            late.append(fill(d[0:8, 0:T]) if n in slots else None)
            if small and n in (SLOTS3 if s == 3 else SLOTS2[i]):
                next(small[0], None)
            for job in deferred:
                job[0] -= 1
            while deferred and deferred[0][0] < 0:
                deferred.pop(0)[1]()
            yield G
            return d

        if (i, s, p) == (0, 0, 0):
            for e in range(2):
                acc = None
                for n, k in enumerate(range(0, DP, T)):
                    d = yield from step(5 * e + n, wt[i, e * G:(e + 1) * G, k:k + T],
                                        block(k, T, range(NT)))
                    acc = d if acc is None else acc + d
                finish(s, e, acc)
            drain()
            return
        yield from strassen(
            i, p, lambda k, n: block(k * HK, HK, (2 * n, 2 * n + 1)),
            lambda n: bsum[s, n, :, :], lambda: block(2 * HK, T, range(NT)), step,
            functools.partial(finish, s, 2 * p), functools.partial(finish, s, 2 * p + 1))

    def finish_q(s, g, q):
        r8 = _iota((8, L), 0)
        qs = q * QSCALE
        for h in range(4):
            lo = 16 * h
            a0, a1, a2 = qs[lo:lo + 8], qs[lo + 8:lo + 16], qs[lo + 16:lo + 24]
            if h > 0:
                a0 = jnp.where(r8 >= 2 * h, a0, 0.0)
            if h < 3:
                a2 = jnp.where(r8 < 2 * h + 2, a2, 0.0)
            w = pltpu.bitcast(jnp.concatenate(
                [a0, a1, a2, jnp.zeros((8, L), f32)], axis=0).astype(bf16), u32)
            for c in range(0, L, T):
                qm.words[s, 4 * g + h, :, c:c + T] = _roll(w[:, c:c + T], ROT[h])
        if s > 0:
            deferred.append([DEFER, functools.partial(memory_read, s, g, _phi(q))])

    def memory_read(s, g, pq):
        r8 = _iota((8, L), 0)
        same_head = _head_of(_iota((G, T), 0)) == _head_of(_iota((G, T), 1))
        num = _dot(jnp.where(same_head, mst[g], 0.0),
                   jnp.concatenate([pq, jnp.zeros((T - G, L), f32)], axis=0).astype(bf16))
        t = pq * jnp.concatenate([zst[g]] * NT, axis=1)
        t = [t[r:r + 8] for r in range(0, G, 8)]
        ib = []
        for h in range(4):
            a, b, c = t[2 * h:2 * h + 3]
            if h > 0:
                a = jnp.where(r8 >= 2 * h, a, 0.0)
            if h < 3:
                c = jnp.where(r8 < 2 * h + 2, c, 0.0)
            den = jnp.sum(a + b + c, axis=0, keepdims=True)
            ib.append(_rcp(jnp.broadcast_to(den, (8, L)) + 1e-6))
        iv = jnp.concatenate(
            [ib[0], ib[0], jnp.where(r8 < 2, ib[0], ib[1]), ib[1],
             jnp.where(r8 < 4, ib[1], ib[2]), ib[2],
             jnp.where(r8 < 6, ib[2], ib[3]), ib[3], ib[3]], axis=0)
        gg = gcol[g * G:(g + 1) * G, :]
        res = num * iv * jnp.concatenate([gg] * NT, axis=1)
        ot[s, g * G:(g + 1) * G, :] = res
        if SOONM:
            t = None
            for c in range(0, L, T):
                for r in SOONR:
                    t = tie(res[r:r + 8, c:c + T], t)
            soon.append([SOONM, t])

    def memory_update(s, g, v, pk, z):
        upd = _dot_nt(v, pk)
        mst[g] = upd if s == 0 else mst[g] + upd
        zst[g] = z if s == 0 else zst[g] + z

    keys = {}

    def finish_k(s, g, k):
        zpad = jnp.zeros((T - G, L), f32)
        kt = jnp.concatenate([k, zpad], axis=0).astype(bf16).T
        kn[s, g, :, :] = kt
        if SOON:
            soon.append([SOON, pltpu.bitcast(kt[-16:], f32)])
        if s < NSEG - 1:
            pk = _phi(k)
            z = sum(pk[:, c:c + T] for c in range(T, L, T)) + pk[:, :T]
            z = jnp.broadcast_to(jnp.sum(z, axis=1, keepdims=True), (G, T))
            keys[g] = jnp.concatenate([pk, zpad], axis=0).astype(bf16), z

    def finish_v(s, g, v):
        for h in range(4):
            a = [v[16 * h + c:16 * h + c + 8] for c in (0, 8, 16)]
            c, r = divmod(ONES_ROW[h], 8)
            a[c] = jnp.where(_iota((8, L), 0) == r, 1.0, a[c])
            vl[s, 4 * g + h] = jnp.concatenate(a, axis=0)
        if s < NSEG - 1:
            deferred.append([DEFER, functools.partial(memory_update, s, g, v, *keys.pop(g))])

    def attention(segs):
        r8 = _iota((8, T), 0)
        units = [(s, g, i, j) for s in segs for g in range(NG) for i, j in ORDER]
        run, accs = {}, {}

        lane32 = _iota((32, T), 1)
        carry = {}

        def own_queries(s, g, i):
            w = []
            for h in range(4):
                parts = [qm[s, 4 * g + h, :, i * T:(i + 1) * T]]
                if h > 0:
                    parts.insert(0, jnp.zeros((16 * h, T), bf16))
                parts.append(jnp.zeros((T - 32 - 16 * h, T), bf16))
                w.append(jnp.concatenate(parts, axis=0))
            return jnp.concatenate(w, axis=1)

        def shared_queries(qw, *parts):
            slots = [None] * 8
            for h, quarters in parts:
                for e in range(2):
                    t = qw[h][8 * e:8 * e + 8] & lanes[RANGES.index(quarters)]
                    slots[h + e] = t if slots[h + e] is None else t | slots[h + e]
            slots = [jnp.zeros((8, T), u32) if t is None else t for t in slots]
            return pltpu.bitcast(jnp.concatenate(slots, axis=0), bf16)

        def diagonal_scores(s, g, i):
            k0 = i * T
            own = carry.pop("own") if i else _dot(kn[s, g, 0:32, :], own_queries(s, g, 0))
            qw = [qm.words[s, 4 * g + h, :, k0:k0 + T] for h in range(4)]
            x = _dot(kn[s, g, k0 + 32:k0 + 64, :], jnp.concatenate(
                [shared_queries(qw, (h, 15 - (2 << h)), (3, 2 << h)) for h in range(3)], axis=1))
            y = _dot(kn[s, g, k0 + 64:k0 + 96, :], jnp.concatenate(
                [shared_queries(qw, (0, 0b1001), (2, 0b0110)),
                 shared_queries(qw, (1, 0b0011), (3, 0b1100))], axis=1))
            z = _dot(kn[s, g, k0 + 96:k0 + T, :],
                     shared_queries(qw, *[(h, 1 << h) for h in range(4)]))
            xs = [x[:, h * T:(h + 1) * T] for h in range(3)]
            xs.append(jnp.where(lane32 < 64, xs[0], jnp.where(lane32 < 96, xs[1], xs[2])))
            ys = [y[:, :T], y[:, T:]] * 2
            zs = [z] * 4
            return [jnp.concatenate([own[:, h * T:(h + 1) * T], xs[h], ys[h], zs[h]], axis=0)
                    for h in range(4)]

        def scores(s, g, i, j):
            if i == j:
                shs = diagonal_scores(s, g, i)
            else:
                more = 32 if j == i - 1 else 0
                st = _dot(kn[s, g, j * T:(j + 1) * T + more, :],
                          own_queries(s, g, i))
                if more:
                    carry["own"] = st[T:]
                shs = [st[:T, h * T:(h + 1) * T] for h in range(4)]
            ps, alphas = [], []
            later = any(a == i for a, _ in ORDER[:ORDER.index((i, j))])
            for h in range(4):
                sh = shs[h]
                if i == j:
                    sh = sh + causal[h]
                m = jnp.max(sh, axis=0, keepdims=True)
                if later:
                    m = jnp.maximum(m, run[i, h])
                    alphas.append(jnp.exp2(run[i, h] - m))
                run[i, h] = m
                ps.append(jnp.exp2(sh - m).astype(bf16))
            return ps, alphas

        def values(s, g, i, j, ps, alphas):
            new = [_dot(vl[s, 4 * g + h, :, j * T:(j + 1) * T], ps[h]) for h in range(4)]
            if alphas:
                new = [a * al + b for a, al, b in zip(accs.pop(i), alphas, new)]
            if any(a == i for a, _ in ORDER[ORDER.index((i, j)) + 1:]):
                accs[i] = new
                return
            o = []
            for h in range(4):
                inv = _rcp(jnp.broadcast_to(new[h][ONES_ROW[h]:ONES_ROW[h] + 1], (8, T)))
                o.append([_roll(new[h][8 * c:8 * c + 8] * inv, -ROT[h]) for c in range(3)])
            a_dot = jnp.concatenate(
                [o[0][0], o[0][1], jnp.where(r8 < 2, o[0][2], o[1][0]), o[1][1],
                 jnp.where(r8 < 4, o[1][2], o[2][0]), o[2][1],
                 jnp.where(r8 < 6, o[2][2], o[3][0]), o[3][1], o[3][2]], axis=0)
            dst = (s, slice(g * G, (g + 1) * G), slice(i * T, (i + 1) * T))
            mix = (1.0 - gcol[g * G:(g + 1) * G, :]) * a_dot
            ot[dst] = ot[dst] + mix if s > 0 else mix

        pend = {}
        for t in range(len(units) + LAG):
            if t < len(units):
                pend[t] = scores(*units[t])
            if t >= LAG:
                values(*units[t - LAG], *pend.pop(t - LAG))
            yield t < len(units) and units[t][2] != units[t][3]

    def out_proj(s):
        b11, b12, b21, b22 = (ot[s, k:k + HK, n:n + HK] for k in (0, HK) for n in (0, HK))
        sums = [t.astype(bf16) for t in (b11 + b22, b12 - b22, b21 - b11, b11 + b12, b21 + b22)]
        parts = [b11.astype(bf16), b22.astype(bf16)]
        rest = jnp.concatenate([ot[s, 2 * HK:D, :], hot[:, s * L:(s + 1) * L],
                                jnp.zeros((DP - D - 8, L), f32)], axis=0).astype(bf16)

        def step(n, w, o):
            d = _dot(w, o)
            if n in OSTEPS:
                yield 9 * G // len(OSTEPS)
            return d

        for p in range(NP):
            halves = []
            yield from strassen(3, p, lambda k, n: parts[k], lambda n: sums[n], lambda: rest,
                                step, halves.append, halves.append)
            a = jnp.concatenate(halves, axis=0)
            rows = slice(p * 2 * G, (p + 1) * 2 * G)
            for c in range(NT):
                b = s * NT + c
                res = x_v[rows, b * T:(b + 1) * T].astype(f32) + xn_v[b, rows, :].astype(f32)
                o_v[s, rows, c * T:(c + 1) * T] = (res + a[:, c * T:(c + 1) * T]).astype(bf16)
            o_cp[s][p].start()

    routed = {}

    def row_block(ref, k, cols):
        w = ref[k:min(k + T, D), cols]
        if k + T > D:
            w = jnp.concatenate([w, jnp.zeros((DP - D, w.shape[1]), bf16)], axis=0)
        return w

    def route():
        def both(op, a):
            return op(op(a, axis=0, keepdims=True), axis=1, keepdims=True)

        r = r_v[...]
        idx = (_iota(r.shape, 0) * T + _iota(r.shape, 1)).astype(f32)
        m1 = both(jnp.max, r)
        i1 = both(jnp.min, jnp.where(r == m1, idx, S))
        r = jnp.where(idx == i1, -jnp.inf, r)
        m2 = both(jnp.max, r)
        i2 = both(jnp.min, jnp.where((r == m2) & (idx != i1), idx, S))
        row = _iota((8, T), 0)
        routed["w"] = jnp.where(row < 2, jax.nn.sigmoid(jnp.where(row == 0, m1, m2)), 0.0)
        pick = jnp.where(row == 0, i1, jnp.where(row == 1, i2, -1.0))
        for b in range(S // T):
            hot[:, b * T:(b + 1) * T] = (pick == (lane8 + b * T).astype(f32)).astype(f32)
        for _ in range(ROUTE_WAIT):
            yield True
        blocks = [jnp.broadcast_to(i.astype(jnp.int32) >> 7, (32, T)) for i in (i1, i2)]
        tiles = [[], []]
        for r0 in range(0, DP // 2, 32):
            acc = [xn_v.words[0, r0:r0 + 32, :]] * 2
            for b in range(1, S // T):
                w = xn_v.words[b, r0:r0 + 32, :]
                acc = [jnp.where(blocks[n] == b, w, acc[n]) for n in range(2)]
            for n in range(2):
                tiles[n].append(acc[n])
            if r0 % 64:
                yield True
        x = None
        for n, i in enumerate((i1, i2)):
            pick = (row == n) & (lane8 == (i.astype(jnp.int32) & (T - 1)))
            d = _dot_nt(pick.astype(f32), pltpu.bitcast(jnp.concatenate(tiles[n], axis=0), bf16))
            x = d if x is None else x + d
        routed["x"] = [x[:, k:k + T] for k in range(0, DP, T)]

    def ffn_hidden():
        routed["h"] = []
        tail = routed["x"][D // T]
        tail = tail + pltpu.roll(_roll(tail, 64), 2, 0)
        for n in range(0, F, L):
            gu = []
            for w_ref in (wg_v, wu_v):
                acc = None
                for c in range(D // T):
                    d = _dot(routed["x"][c], w_ref[c * T:(c + 1) * T, n:n + L])
                    acc = d if acc is None else acc + d
                    yield True
                gu.append(acc)
            d = _dot(tail, jnp.concatenate(
                [w_ref[D // T * T:D, n:n + L] for w_ref in (wg_v, wu_v)], axis=0))
            yield True
            gt, up = gu[0] + d, gu[1] + pltpu.roll(d, 6, 0)
            routed["h"].append(gt * jax.nn.sigmoid(gt) * up)

    def ffn_down():
        for k in range(0, D, T):
            acc = None
            for c, n in enumerate(range(0, F, L)):
                d = _dot_nt(routed["h"][c], row_block(wd_v, k, slice(n, n + L)))
                acc = d if acc is None else acc + d
                yield
            y = jnp.concatenate([jnp.zeros((D - 4 * T, T), f32), acc * routed["w"],
                                 jnp.zeros((DP - D - 8, T), f32)], axis=0).T
            dst = (3, slice(k, min(k + T, D)), slice(4 * T, DP))
            wt[dst] = wt[dst] + y[0:min(T, D - k)]

    for c in (*c_cp, *x_cp[:2], *wq_cp, *w_cp[1:3]):
        c.start()
    for h in range(4):
        query = (_iota((T, T), 1) - ROT[h]) & (T - 1)
        causal[h] = jnp.where(_iota((T, T), 0) <= query, 0.0, NEG)
    for n, quarters in enumerate(RANGES):
        lanes[n] = pltpu.bitcast(-((quarters >> (lane8 >> 5)) & 1), u32)
    for c in c_cp:
        c.wait()
    router_column()
    for _ in gate_column():
        pass
    for b in range(NT):
        if b < 2:
            x_cp[b].wait()
        fillers.append(layernorm(b, LNROWS0))
        prev = [None, None]
        while fillers:
            prev.append(fill(prev.pop(0)))
    x_cp[2].start()
    wq_cp[0].wait()
    fillers.append(transpose_w(0, 0, 2 * T))
    drain()

    def prepare(s, step):
        fillers.extend(layernorm(b, step) for b in range(s * NT, (s + 1) * NT))
        fillers.append(combine(s, step[3]))

    def rest_of_wq():
        wq_cp[1].wait()
        run(transpose_w(0, 2 * T))

    def wk_arrives():
        for c in (x_cp[3], w_cp[3]):
            c.start()
        w_cp[1].wait()
        run(transpose_w(1))

    def wv_arrives():
        for ref in (wg_v, wu_v, wd_v):
            ref[0:16, 0:T] = kn[0, 0, 0:16, :]
        for c in f_cp:
            c.start()
        for c in (w_cp[2], x_cp[2]):
            c.wait()
        run(transpose_w(2))
        prepare(1, LNROWS1)

    def wo_arrives():
        for c in (x_cp[3], w_cp[3]):
            c.wait()
        prepare(2, LNROWS)
        prepare(3, LNROWS)
        small.append(transpose_w(3))

    def ffn_arrives():
        for c in f_cp:
            c.wait()
        run(small.pop())
        small.append(ffn_hidden())

    arrivals.update({WAIT_Q: rest_of_wq, WAIT_K: wk_arrives, WAIT_V: wv_arrives,
                     WAIT_O: wo_arrives, FWAIT: ffn_arrives})
    fillers.append(combine(0, 64))
    for i, finish in enumerate((finish_q, finish_k, finish_v)):
        for p in range(NP):
            run(proj(i, 0, p, SLOTS0[i], finish))

    def dense(s):
        while normed[0] <= s:
            fill()
        for p in range(NP):
            for i, finish in enumerate((finish_q, finish_k, finish_v)):
                yield from proj(i, s, p, SLOTS[i], finish)

    def weave(main, steps, other, rows, extra=iter(())):
        done = 0
        for t in range(steps):
            if next(main):
                next(extra, None)
            while done < (t + 1) * rows // steps:
                done += next(other, rows)

    def finish(main, other):
        for _ in range(LAG):
            done = 0
            while done < 4 * G:
                done += next(other)
            next(main)
        run(main)
        run(other)

    per_seg = NG * len(ORDER)
    run(dense(1))
    run(dense(2))
    drain()
    att, steps = attention([0]), dense(3)
    weave(att, ROUTE_AT, iter(()), 0)
    routing = route()
    weave(att, per_seg - ROUTE_AT, iter(()), 0, routing)
    run(routing)
    finish(att, steps)
    run(small[0])
    drain()
    att = attention(range(1, NSEG))
    steps = ffn_down()
    weave(att, per_seg, iter(()), 0, steps)
    run(steps)
    outs = (n for s in range(NSEG - 1) for n in out_proj(s))
    weave(att, 2 * per_seg, outs, 3 * NP * 9 * G - TAIL * G)
    finish(att, outs)
    run(out_proj(NSEG - 1))
    assert not deferred and not arrivals
    for cs in o_cp:
        for c in cs:
            c.wait()


@jax.jit
def pallas_parallel_sum__memory_aug_infini_attn__moe_arch_mod__prompt_kernel(
    A_x: jax.Array,
    A_wq: jax.Array,
    A_wk: jax.Array,
    A_wv: jax.Array,
    A_wo: jax.Array,
    A_beta: jax.Array,
    B_x: jax.Array,
    B_w_r: jax.Array,
    B_w_gate: jax.Array,
    B_w_up: jax.Array,
    B_w_down: jax.Array,
):
    del B_x
    hbm = pl.BlockSpec(memory_space=pltpu.HBM)
    out = pl.pallas_call(
        _kernel,
        out_shape=jax.ShapeDtypeStruct((D, S), A_x.dtype),
        in_specs=[hbm] * 10,
        out_specs=hbm,
        scratch_shapes=[
            pltpu.VMEM((D, S), bf16),
            pltpu.VMEM((4, D, D), bf16),
            pltpu.VMEM((1, H), bf16),
            pltpu.VMEM((D,), bf16),
            pltpu.VMEM((D, F), bf16),
            pltpu.VMEM((D, F), bf16),
            pltpu.VMEM((D, F), bf16),
            pltpu.VMEM((4, D, DP), f32),
            pltpu.VMEM((D, T), f32),
            pltpu.VMEM((S // T, DP // 2, T), u32),
            pltpu.VMEM((NSEG, 5, HK // 2, HK), u32),
            pltpu.VMEM((NSEG, H, 16, L), u32),
            pltpu.VMEM((NSEG, H, 24, L), f32),
            pltpu.VMEM((NSEG, NG, L // 2, T), u32),
            pltpu.VMEM((NSEG, D, L), f32),
            pltpu.VMEM((NG, G, T), f32),
            pltpu.VMEM((NG, G, T), f32),
            pltpu.VMEM((D, T), f32),
            pltpu.VMEM((S // T, T), f32),
            pltpu.VMEM((8, S), f32),
            pltpu.VMEM((NSEG, D, L), bf16),
            pltpu.VMEM((4, T, T), f32),
            pltpu.VMEM((len(RANGES), 8, T), u32),
            pltpu.SemaphoreType.DMA((8 + len(XPARTS),)),
        ],
        compiler_params=pltpu.CompilerParams(vmem_limit_bytes=100 * 2**20),
    )(A_x.reshape(S, D).T, A_wq, A_wk, A_wv, A_wo, A_beta.reshape(1, H), B_w_r,
      B_w_gate, B_w_up, B_w_down.T)
    return out.T.reshape(A_x.shape)
```

```python
import functools

import jax
import jax.numpy as jnp
import jax.experimental.pallas as pl
import jax.experimental.pallas.tpu as pltpu

S, D, H, DH, NSEG, L, F = 2048, 576, 32, 18, 4, 512, 4608
T = 128
HK = 2 * T
DP = 640
G = 4 * DH
NG = H // 4
NP = NG // 2
NT = L // T
QSCALE = DH ** -0.5 * 1.4426950408889634
NEG = -1e30
ONES_ROW = (23, 23, 0, 0)
ROT = (32, 64, 96, 0)
QUARTERS = (0b0001, 0b0010, 0b0100, 0b1000, 0b1101, 0b1011, 0b0111,
            0b1001, 0b0110, 0b0011, 0b1100)
XPARTS = ((0, 128), (128, 384), (512, 512), (1024, 1024))

ORDER = ((3, 2), (3, 3), (3, 0), (0, 0), (3, 1), (2, 1), (2, 2), (2, 0), (1, 0), (1, 1))
LAG = 2
WAIT_Q, WAIT_K, WAIT_V = (0, 0, 0, 9), (0, 0, 3, 4), (1, 0, 3, 4)
WAIT_O, WAIT_F, WO_READY = (0, 1, 0, 4), (0, 3, 1, 0), (0, 2, 1, 2)
FILL_FIRST = ((0, 1, 2, 3, 4, 7, 8, 9), (5, 8), range(9))
FILL_WO = ((), (7,), (1, 7))
LN_ROWS = ((144, 144, 144, 64), (576, 288, 96, 128), (192, 96, 48, 32))
LATE, DEFER, SOON = 2, 4, 9
ROUTE_AT, ROUTE_WAIT, TAIL = 30, 5, 27

f32, bf16, u32 = jnp.float32, jnp.bfloat16, jnp.uint32


def _dot(a, b):
    return jnp.dot(a, b, preferred_element_type=f32)


def _dot_nt(a, b):
    return jax.lax.dot_general(a, b, (((1,), (1,)), ((), ())), preferred_element_type=f32)


def _rnd(a):
    return a.astype(bf16).astype(f32)


def _rcp(a):
    return pltpu.reciprocal(a, full_range=False)


def _iota(shape, axis):
    return jax.lax.broadcasted_iota(jnp.int32, shape, axis)


def _pad_to_tile(a):
    if a.shape[1] < T:
        a = jnp.concatenate([a, jnp.zeros((a.shape[0], T - a.shape[1]), a.dtype)], axis=1)
    if a.shape[0] < T:
        a = jnp.concatenate([a, jnp.zeros((T - a.shape[0], T), a.dtype)], axis=0)
    return a


def _roll(a, shift):
    return pltpu.roll(a, shift % T, 1) if shift % T else a


def _phi(t):
    return jnp.where(t > 0, t + 1.0, jnp.exp(t))


def _head_of(i):
    return ((i >= DH).astype(jnp.int32) + (i >= 2 * DH).astype(jnp.int32)
            + (i >= 3 * DH).astype(jnp.int32) + (i >= 4 * DH).astype(jnp.int32))


class _Packed:
    def __init__(self, ref):
        self.words = ref

    def _index(self, idx):
        *lead, rows, cols = idx
        start, stop, _ = rows.indices(2 * self.words.shape[-2])
        return (*lead, slice(start // 2, stop // 2), cols)

    def __getitem__(self, idx):
        return pltpu.bitcast(self.words[self._index(idx)], bf16)

    def __setitem__(self, idx, value):
        self.words[self._index(idx)] = pltpu.bitcast(value, u32)


def _run(steps):
    for _ in steps:
        pass


def _kernel(x_hbm, wq_hbm, wk_hbm, wv_hbm, wo_hbm, beta_hbm, wr_hbm, wg_hbm, wu_hbm,
            wd_hbm, o_hbm,
            x_v, w_v, beta_v, wr_v, wg_v, wu_v, wd_v, wt, wrc, xn_v, bsum, qm, vl, kn, ot,
            mst, zst, gcol, r_v, hot, o_v, causal, lanes, sem):
    xn_v, bsum, qm, kn = (_Packed(r) for r in (xn_v, bsum, qm, kn))
    copy = pltpu.make_async_copy
    wq_cp = [copy(wq_hbm.at[:, pl.ds(c, n)], w_v.at[0, :, pl.ds(c, n)], sem.at[i])
             for c, n, i in ((0, 2 * T, 0), (2 * T, D - 2 * T, 7 + len(XPARTS)))]
    wk_cp, wv_cp, wo_cp = (copy(w, w_v.at[i], sem.at[i])
                           for i, w in ((1, wk_hbm), (2, wv_hbm), (3, wo_hbm)))
    f_cp = [copy(a, b, sem.at[4]) for a, b in ((wg_hbm, wg_v), (wu_hbm, wu_v), (wd_hbm, wd_v))]
    c_cp = [copy(a, b, sem.at[5]) for a, b in ((wr_hbm, wr_v), (beta_hbm, beta_v))]
    o_cp = [[copy(o_v.at[s, pl.ds(p * 2 * G, 2 * G)],
                  o_hbm.at[pl.ds(p * 2 * G, 2 * G), pl.ds(s * L, L)], sem.at[6])
             for p in range(NP)] for s in range(NSEG)]
    x_cp = [copy(x_hbm.at[:, pl.ds(t, n)], x_v.at[:, pl.ds(t, n)], sem.at[7 + i])
            for i, (t, n) in enumerate(XPARTS)]

    lane8 = _iota((8, T), 1)
    never = lane8 < jnp.min(lane8, axis=1, keepdims=True)
    zero = jnp.min(lane8)
    fillers = []
    link = [None, None]

    def tie(a, b):
        return a if b is None else jnp.where(never, b, a)

    def fill(after=None):
        link[0], link[1] = after, None
        while fillers:
            if next(fillers[0], False):
                break
            fillers.pop(0)
        return link[1]

    def drain():
        while fillers:
            fill()

    def gate_column():
        gate = jax.nn.sigmoid(beta_v[...].astype(f32))
        gate = jnp.concatenate([gate, jnp.zeros((1, T - H), f32)], axis=1)
        gate = jnp.broadcast_to(gate, (T, T)).T
        r8 = _iota((8, T), 0)
        for v in range(D // 8):
            h0, h1 = (8 * v) // DH, (8 * v + 7) // DH
            gv = jnp.broadcast_to(gate[h0:h0 + 1], (8, T))
            if h1 != h0:
                gv = jnp.where(r8 < h1 * DH - 8 * v, gv, jnp.broadcast_to(gate[h1:h1 + 1], (8, T)))
            gcol[8 * v:8 * v + 8, :] = gv

    def router_column():
        wr = wr_v[...].astype(f32).reshape(1, D)
        wr = jnp.concatenate([wr, jnp.zeros((1, DP - D), f32)], axis=1)
        wrc[...] = jnp.broadcast_to(wr, (T, DP)).T[0:D]

    def transpose_w(i, lo=0, hi=D):
        for c in range(lo, hi, T):
            n = min(T, D - c)
            for k in range(0, D, T):
                w = _pad_to_tile(w_v[i, k:min(k + T, D), c:c + n].astype(f32))
                w = jnp.concatenate([tie(w[r:r + 8], link[0]) for r in range(0, T, 8)], axis=0).T
                wt[i, c:c + n, k:k + T] = w[0:n]
                yield True

    def layernorm(b, steps):
        def total(acc, v):
            h = v.shape[0] // 16 * 8
            a, c = v[0:8], v[h:h + 8]
            for k in range(8, h, 8):
                a, c = a + v[k:k + 8], c + v[h + k:h + k + 8]
            return a + c if acc is None else acc + (a + c)

        def rows(v):
            return jnp.concatenate([tie(v, link[0])] * (step // 8), axis=0)

        def bcast(v):
            return jnp.broadcast_to(v, (8, T))

        def load(r, n):
            return x_v[r:r + step, pl.ds(pl.multiple_of((b + n * zero) * T, T), T)].astype(f32)

        acc, step = jnp.zeros((8, T), f32), steps[0]
        for r in range(0, D, step):
            x = load(r, 0)
            link[1] = acc = total(tie(acc, link[0]), x)
            yield True
        mean = bcast(jnp.sum(acc, axis=0, keepdims=True) * (1.0 / D))
        acc, step = None, steps[1]
        for r in range(0, D, step):
            xc = load(r, 1) - rows(mean)
            link[1] = acc = total(acc, xc * xc)
            yield True
        var = bcast(jnp.sum(acc, axis=0, keepdims=True) * (1.0 / D))
        sd = _rnd(jnp.sqrt(_rnd(_rnd(var) + _rnd(jnp.full((8, T), 1e-5, f32)))))
        step = steps[2]
        inv, mean = jnp.concatenate([1.0 / sd] * (step // 8), axis=0), _rnd(mean)
        acc = None
        for r in range(0, D, step):
            x = load(r, 2)
            xn = (_rnd(x - rows(mean)) * inv).astype(bf16)
            xn_v[b, r:r + step, :] = xn
            link[1] = acc = total(acc, xn.astype(f32) * wrc[r:r + step, :])
            if r + step == D:
                xn_v[b, D:DP, :] = jnp.zeros((DP - D, T), bf16)
                r_v[b:b + 1, :] = _rnd(jnp.sum(acc, axis=0, keepdims=True))
            yield True

    prepared = [0]

    def block_sums(s, rows):
        for c in range(NT // 2):
            for r in range(0, HK, rows):
                b11, b12, b21, b22 = (
                    xn_v[s * NT + c + n + zero, k + r:k + r + rows, :].astype(f32)
                    for k in (0, HK) for n in (0, NT // 2))
                b11 = jnp.concatenate(
                    [tie(b11[k:k + 8], link[0]) for k in range(0, rows, 8)], axis=0)
                for n, t in enumerate((b11 + b22, b12 - b22, b21 - b11, b11 + b12, b21 + b22)):
                    bsum[s, n, r:r + rows, c * T:(c + 1) * T] = t.astype(bf16)
                    link[1] = tie(t[-8:], link[1])
                prepared[0] += c == NT // 2 - 1 and r + rows == HK
                yield True

    def strassen(i, p, part, sums, rest, step, top, bottom):
        r0, r1 = slice(2 * p * G, (2 * p + 1) * G), slice((2 * p + 1) * G, (2 * p + 2) * G)
        a11, a12 = (lambda: wt[i, r0, 0:HK]), (lambda: wt[i, r0, HK:2 * HK])
        a21, a22 = (lambda: wt[i, r1, 0:HK]), (lambda: wt[i, r1, HK:2 * HK])
        c11 = yield from step(0, a12() - a22(), sums(4))
        m = yield from step(1, a11() + a12(), part(1))
        c11, c12 = c11 - m, m
        m = yield from step(2, wt[i, r0, 2 * HK:DP], rest())
        c11, c12 = c11 + m[:, :HK], c12 + m[:, HK:]
        m = yield from step(3, a11() + a22(), sums(0))
        c11, c22 = c11 + m, m
        m = yield from step(4, a11(), sums(1))
        c12, c22 = c12 + m, c22 + m
        c21 = yield from step(5, a22(), sums(2))
        top(jnp.concatenate([c11 + c21, c12], axis=1))
        m = yield from step(6, a21() + a22(), part(0))
        c21, c22 = c21 + m, c22 - m
        c22 = c22 + (yield from step(7, a21() - a11(), sums(3)))
        m = yield from step(8, wt[i, r1, 2 * HK:DP], rest())
        bottom(jnp.concatenate([c21, c22], axis=1) + m)

    late = [None] * LATE
    soon = []
    deferred = []
    arrivals = {}
    other = []

    def project(i, s, p, slots, finish):
        def block(k, n, cs):
            return jnp.concatenate([xn_v[s * NT + c, k:k + n, :] for c in cs], axis=1)

        def step(n, w, xs):
            if (i, s, p, n) == WO_READY:
                done = wt[zero, pl.ds(pl.multiple_of(zero * 8, 8), 8),
                          pl.ds(pl.multiple_of(zero * T, T), T)]
                w = jnp.concatenate([w[:-8], tie(w[-8:], done)], axis=0)
            if (i, s, p, n) in arrivals:
                arrivals.pop((i, s, p, n))()
            d = _dot(w, xs)
            top = tie(d[-8:, :T], late.pop(0))
            for job in soon:
                job[0] -= 1
                if job[0] == -1:
                    top = tie(top, job[1])
            d = jnp.concatenate([d[:-8], jnp.concatenate([top, d[-8:, T:]], axis=1)], axis=0)
            late.append(fill(d[0:8, 0:T]) if n in slots else None)
            if other and (s == NSEG - 1 or n in FILL_WO[i]):
                next(other[0], None)
            for job in deferred:
                job[0] -= 1
            while deferred and deferred[0][0] < 0:
                deferred.pop(0)[1]()
            yield G
            return d

        if (i, s, p) == (0, 0, 0):
            for e in range(2):
                acc = None
                for n, k in enumerate(range(0, DP, T)):
                    d = yield from step(5 * e + n, wt[i, e * G:(e + 1) * G, k:k + T],
                                        block(k, T, range(NT)))
                    acc = d if acc is None else acc + d
                finish(s, e, acc)
            drain()
            return
        yield from strassen(
            i, p, lambda k: block(k * HK, HK, (2 * k, 2 * k + 1)),
            lambda n: bsum[s, n, :, :], lambda: block(2 * HK, T, range(NT)), step,
            functools.partial(finish, s, 2 * p), functools.partial(finish, s, 2 * p + 1))

    def finish_q(s, g, q):
        r8 = _iota((8, L), 0)
        qs = q * QSCALE
        for h in range(4):
            lo = 16 * h
            a0, a1, a2 = qs[lo:lo + 8], qs[lo + 8:lo + 16], qs[lo + 16:lo + 24]
            if h > 0:
                a0 = jnp.where(r8 >= 2 * h, a0, 0.0)
            if h < 3:
                a2 = jnp.where(r8 < 2 * h + 2, a2, 0.0)
            w = pltpu.bitcast(jnp.concatenate(
                [a0, a1, a2, jnp.zeros((8, L), f32)], axis=0).astype(bf16), u32)
            for c in range(0, L, T):
                qm.words[s, 4 * g + h, :, c:c + T] = _roll(w[:, c:c + T], ROT[h])
        if s > 0:
            deferred.append([DEFER, functools.partial(memory_read, s, g, _phi(q))])

    def memory_read(s, g, pq):
        r8 = _iota((8, L), 0)
        same_head = _head_of(_iota((G, T), 0)) == _head_of(_iota((G, T), 1))
        num = _dot(jnp.where(same_head, mst[g], 0.0),
                   jnp.concatenate([pq, jnp.zeros((T - G, L), f32)], axis=0).astype(bf16))
        t = pq * jnp.concatenate([zst[g]] * NT, axis=1)
        t = [t[r:r + 8] for r in range(0, G, 8)]
        ib = []
        for h in range(4):
            a, b, c = t[2 * h:2 * h + 3]
            if h > 0:
                a = jnp.where(r8 >= 2 * h, a, 0.0)
            if h < 3:
                c = jnp.where(r8 < 2 * h + 2, c, 0.0)
            den = jnp.sum(a + b + c, axis=0, keepdims=True)
            ib.append(_rcp(jnp.broadcast_to(den, (8, L)) + 1e-6))
        iv = jnp.concatenate(
            [ib[0], ib[0], jnp.where(r8 < 2, ib[0], ib[1]), ib[1],
             jnp.where(r8 < 4, ib[1], ib[2]), ib[2],
             jnp.where(r8 < 6, ib[2], ib[3]), ib[3], ib[3]], axis=0)
        gg = gcol[g * G:(g + 1) * G, :]
        res = num * iv * jnp.concatenate([gg] * NT, axis=1)
        ot[s, g * G:(g + 1) * G, :] = res
        t = None
        for c in range(0, L, T):
            for r in (0, 24, 40, 64):
                t = tie(res[r:r + 8, c:c + T], t)
        soon.append([SOON, t])

    def memory_update(s, g, v, pk, z):
        upd = _dot_nt(v, pk)
        mst[g] = upd if s == 0 else mst[g] + upd
        zst[g] = z if s == 0 else zst[g] + z

    keys = {}

    def finish_k(s, g, k):
        zpad = jnp.zeros((T - G, L), f32)
        kt = jnp.concatenate([k, zpad], axis=0).astype(bf16).T
        kn[s, g, :, :] = kt
        soon.append([SOON, pltpu.bitcast(kt[-16:], f32)])
        if s < NSEG - 1:
            pk = _phi(k)
            z = sum(pk[:, c:c + T] for c in range(T, L, T)) + pk[:, :T]
            z = jnp.broadcast_to(jnp.sum(z, axis=1, keepdims=True), (G, T))
            keys[g] = jnp.concatenate([pk, zpad], axis=0).astype(bf16), z

    def finish_v(s, g, v):
        for h in range(4):
            a = [v[16 * h + c:16 * h + c + 8] for c in (0, 8, 16)]
            c, r = divmod(ONES_ROW[h], 8)
            a[c] = jnp.where(_iota((8, L), 0) == r, 1.0, a[c])
            vl[s, 4 * g + h] = jnp.concatenate(a, axis=0)
        if s < NSEG - 1:
            deferred.append([DEFER, functools.partial(memory_update, s, g, v, *keys.pop(g))])

    attended = [0] * NSEG

    def attention(segs):
        r8 = _iota((8, T), 0)
        lane32 = _iota((32, T), 1)
        units = [(s, g, i, j) for s in segs for g in range(NG) for i, j in ORDER]
        maxes, accs, carry = {}, {}, {}

        def own_queries(s, g, i):
            w = []
            for h in range(4):
                parts = [qm[s, 4 * g + h, :, i * T:(i + 1) * T]]
                if h > 0:
                    parts.insert(0, jnp.zeros((16 * h, T), bf16))
                parts.append(jnp.zeros((T - 32 - 16 * h, T), bf16))
                w.append(jnp.concatenate(parts, axis=0))
            return jnp.concatenate(w, axis=1)

        def shared_queries(qw, *parts):
            slots = [None] * 8
            for h, quarters in parts:
                for e in range(2):
                    t = qw[h][8 * e:8 * e + 8] & lanes[QUARTERS.index(quarters)]
                    slots[h + e] = t if slots[h + e] is None else t | slots[h + e]
            slots = [jnp.zeros((8, T), u32) if t is None else t for t in slots]
            return pltpu.bitcast(jnp.concatenate(slots, axis=0), bf16)

        def diagonal_scores(s, g, i):
            k0 = i * T
            own = carry.pop("own") if i else _dot(kn[s, g, 0:32, :], own_queries(s, g, 0))
            qw = [qm.words[s, 4 * g + h, :, k0:k0 + T] for h in range(4)]
            x = _dot(kn[s, g, k0 + 32:k0 + 64, :], jnp.concatenate(
                [shared_queries(qw, (h, 15 - (2 << h)), (3, 2 << h)) for h in range(3)], axis=1))
            y = _dot(kn[s, g, k0 + 64:k0 + 96, :], jnp.concatenate(
                [shared_queries(qw, (0, 0b1001), (2, 0b0110)),
                 shared_queries(qw, (1, 0b0011), (3, 0b1100))], axis=1))
            z = _dot(kn[s, g, k0 + 96:k0 + T, :],
                     shared_queries(qw, *[(h, 1 << h) for h in range(4)]))
            xs = [x[:, h * T:(h + 1) * T] for h in range(3)]
            xs.append(jnp.where(lane32 < 64, xs[0], jnp.where(lane32 < 96, xs[1], xs[2])))
            ys = [y[:, :T], y[:, T:]] * 2
            return [jnp.concatenate([own[:, h * T:(h + 1) * T], xs[h], ys[h], z], axis=0)
                    for h in range(4)]

        def scores(s, g, i, j):
            if i == j:
                shs = diagonal_scores(s, g, i)
            else:
                more = 32 if j == i - 1 else 0
                st = _dot(kn[s, g, j * T:(j + 1) * T + more, :], own_queries(s, g, i))
                if more:
                    carry["own"] = st[T:]
                shs = [st[:T, h * T:(h + 1) * T] for h in range(4)]
            ps, alphas = [], []
            later = any(a == i for a, _ in ORDER[:ORDER.index((i, j))])
            for h in range(4):
                sh = shs[h]
                if i == j:
                    sh = sh + causal[h]
                m = jnp.max(sh, axis=0, keepdims=True)
                if later:
                    m = jnp.maximum(m, maxes[i, h])
                    alphas.append(jnp.exp2(maxes[i, h] - m))
                maxes[i, h] = m
                ps.append(jnp.exp2(sh - m).astype(bf16))
            return ps, alphas

        def values(s, g, i, j, ps, alphas):
            new = [_dot(vl[s, 4 * g + h, :, j * T:(j + 1) * T], ps[h]) for h in range(4)]
            if alphas:
                new = [a * al + b for a, al, b in zip(accs.pop(i), alphas, new)]
            if any(a == i for a, _ in ORDER[ORDER.index((i, j)) + 1:]):
                accs[i] = new
                return
            o = []
            for h in range(4):
                inv = _rcp(jnp.broadcast_to(new[h][ONES_ROW[h]:ONES_ROW[h] + 1], (8, T)))
                o.append([_roll(new[h][8 * c:8 * c + 8] * inv, -ROT[h]) for c in range(3)])
            a_dot = jnp.concatenate(
                [o[0][0], o[0][1], jnp.where(r8 < 2, o[0][2], o[1][0]), o[1][1],
                 jnp.where(r8 < 4, o[1][2], o[2][0]), o[2][1],
                 jnp.where(r8 < 6, o[2][2], o[3][0]), o[3][1], o[3][2]], axis=0)
            dst = (s, slice(g * G, (g + 1) * G), slice(i * T, (i + 1) * T))
            mix = (1.0 - gcol[g * G:(g + 1) * G, :]) * a_dot
            ot[dst] = ot[dst] + mix if s > 0 else mix
            attended[s] += 1

        pend = {}
        for t in range(len(units) + LAG):
            if t < len(units):
                pend[t] = scores(*units[t])
            if t >= LAG:
                values(*units[t - LAG], *pend.pop(t - LAG))
            yield t < len(units) and units[t][2] != units[t][3]

    def out_proj(s):
        assert attended[s] == NG * NT
        b11, b12, b21, b22 = (ot[s, k:k + HK, n:n + HK] for k in (0, HK) for n in (0, HK))
        sums = [t.astype(bf16) for t in (b11 + b22, b12 - b22, b21 - b11, b11 + b12, b21 + b22)]
        parts = [b11.astype(bf16), b22.astype(bf16)]
        rest = jnp.concatenate([ot[s, 2 * HK:D, :], hot[:, s * L:(s + 1) * L],
                                jnp.zeros((DP - D - 8, L), f32)], axis=0).astype(bf16)

        def step(n, w, o):
            d = _dot(w, o)
            if n % 3 == 2:
                yield 3 * G
            return d

        for p in range(NP):
            halves = []
            yield from strassen(3, p, parts.__getitem__, sums.__getitem__, lambda: rest,
                                step, halves.append, halves.append)
            a = jnp.concatenate(halves, axis=0)
            rows = slice(p * 2 * G, (p + 1) * 2 * G)
            for c in range(NT):
                b = s * NT + c
                res = x_v[rows, b * T:(b + 1) * T].astype(f32) + xn_v[b, rows, :].astype(f32)
                o_v[s, rows, c * T:(c + 1) * T] = (res + a[:, c * T:(c + 1) * T]).astype(bf16)
            o_cp[s][p].start()

    routed = {}

    def route():
        def both(op, a):
            return op(op(a, axis=0, keepdims=True), axis=1, keepdims=True)

        r = r_v[...]
        idx = (_iota(r.shape, 0) * T + _iota(r.shape, 1)).astype(f32)
        m1 = both(jnp.max, r)
        i1 = both(jnp.min, jnp.where(r == m1, idx, S))
        r = jnp.where(idx == i1, -jnp.inf, r)
        m2 = both(jnp.max, r)
        i2 = both(jnp.min, jnp.where((r == m2) & (idx != i1), idx, S))
        row = _iota((8, T), 0)
        routed["w"] = jnp.where(row < 2, jax.nn.sigmoid(jnp.where(row == 0, m1, m2)), 0.0)
        pick = jnp.where(row == 0, i1, jnp.where(row == 1, i2, -1.0))
        for b in range(S // T):
            hot[:, b * T:(b + 1) * T] = (pick == (lane8 + b * T).astype(f32)).astype(f32)
        for _ in range(ROUTE_WAIT):
            yield
        blocks = [jnp.broadcast_to(i.astype(jnp.int32) >> 7, (32, T)) for i in (i1, i2)]
        tiles = [[], []]
        for r0 in range(0, DP // 2, 32):
            acc = [xn_v.words[0, r0:r0 + 32, :]] * 2
            for b in range(1, S // T):
                w = xn_v.words[b, r0:r0 + 32, :]
                acc = [jnp.where(blocks[n] == b, w, acc[n]) for n in range(2)]
            for n in range(2):
                tiles[n].append(acc[n])
            if r0 % 64:
                yield
        x = None
        for n, i in enumerate((i1, i2)):
            pick = (row == n) & (lane8 == (i.astype(jnp.int32) & (T - 1)))
            d = _dot_nt(pick.astype(f32), pltpu.bitcast(jnp.concatenate(tiles[n], axis=0), bf16))
            x = d if x is None else x + d
        routed["x"] = [x[:, k:k + T] for k in range(0, DP, T)]

    def ffn_hidden():
        routed["h"] = []
        tail = routed["x"][D // T]
        tail = tail + pltpu.roll(_roll(tail, 64), 2, 0)
        for n in range(0, F, L):
            gu = []
            for w_ref in (wg_v, wu_v):
                acc = None
                for c in range(D // T):
                    d = _dot(routed["x"][c], w_ref[c * T:(c + 1) * T, n:n + L])
                    acc = d if acc is None else acc + d
                    yield
                gu.append(acc)
            d = _dot(tail, jnp.concatenate(
                [w_ref[D // T * T:D, n:n + L] for w_ref in (wg_v, wu_v)], axis=0))
            yield
            gt, up = gu[0] + d, gu[1] + pltpu.roll(d, 6, 0)
            routed["h"].append(gt * jax.nn.sigmoid(gt) * up)

    def ffn_down():
        for k in range(0, D, T):
            acc = None
            for c, n in enumerate(range(0, F, L)):
                w = wd_v[k:min(k + T, D), n:n + L]
                if k + T > D:
                    w = jnp.concatenate([w, jnp.zeros((DP - D, L), bf16)], axis=0)
                d = _dot_nt(routed["h"][c], w)
                acc = d if acc is None else acc + d
                yield
            y = jnp.concatenate([jnp.zeros((D - 4 * T, T), f32), acc * routed["w"],
                                 jnp.zeros((DP - D - 8, T), f32)], axis=0).T
            dst = (3, slice(k, min(k + T, D)), slice(4 * T, DP))
            wt[dst] = wt[dst] + y[0:min(T, D - k)]

    for c in (*c_cp, *x_cp[:2], *wq_cp, wk_cp, wv_cp):
        c.start()
    for h in range(4):
        query = (_iota((T, T), 1) - ROT[h]) & (T - 1)
        causal[h] = jnp.where(_iota((T, T), 0) <= query, 0.0, NEG)
    for n, quarters in enumerate(QUARTERS):
        lanes[n] = pltpu.bitcast(-((quarters >> (lane8 >> 5)) & 1), u32)
    for c in c_cp:
        c.wait()
    router_column()
    gate_column()
    for b in range(NT):
        if b < 2:
            x_cp[b].wait()
        fillers.append(layernorm(b, LN_ROWS[0]))
        prev = [None, None]
        while fillers:
            prev.append(fill(prev.pop(0)))
    x_cp[2].start()
    wq_cp[0].wait()
    fillers.append(transpose_w(0, 0, 2 * T))
    drain()

    def prepare(s, rows):
        fillers.extend(layernorm(b, rows) for b in range(s * NT, (s + 1) * NT))
        fillers.append(block_sums(s, rows[3]))

    def wq_arrives():
        wq_cp[1].wait()
        _run(transpose_w(0, 2 * T))

    def wk_arrives():
        for c in (x_cp[3], wo_cp):
            c.start()
        wk_cp.wait()
        _run(transpose_w(1))

    def wv_arrives():
        for ref in (wg_v, wu_v, wd_v):
            ref[0:16, 0:T] = kn[0, 0, 0:16, :]
        for c in f_cp:
            c.start()
        for c in (wv_cp, x_cp[2]):
            c.wait()
        _run(transpose_w(2))
        prepare(1, LN_ROWS[1])

    def wo_arrives():
        for c in (x_cp[3], wo_cp):
            c.wait()
        prepare(2, LN_ROWS[2])
        prepare(3, LN_ROWS[2])
        other.append(transpose_w(3))

    def ffn_arrives():
        for c in f_cp:
            c.wait()
        _run(other.pop())
        other.append(ffn_hidden())

    arrivals.update({WAIT_Q: wq_arrives, WAIT_K: wk_arrives, WAIT_V: wv_arrives,
                     WAIT_O: wo_arrives, WAIT_F: ffn_arrives})
    finishers = tuple(enumerate((finish_q, finish_k, finish_v)))
    fillers.append(block_sums(0, LN_ROWS[0][3]))
    for i, finish in finishers:
        for p in range(NP):
            _run(project(i, 0, p, FILL_FIRST[i], finish))

    def project_segment(s):
        while prepared[0] <= s:
            assert fillers
            fill()
        for p in range(NP):
            for i, finish in finishers:
                yield from project(i, s, p, range(9), finish)

    def attend(att, steps, extra=iter(()), dense=iter(()), rows=0):
        done = 0
        for t in range(steps):
            if next(att):
                next(extra, None)
            while done < (t + 1) * rows // steps:
                done += next(dense)

    def wind_down(att, dense):
        for _ in range(LAG):
            done = 0
            while done < 4 * G:
                done += next(dense)
            next(att)
        _run(att)
        _run(dense)

    per_seg = NG * len(ORDER)
    _run(project_segment(1))
    _run(project_segment(2))
    drain()
    att, steps = attention([0]), route()
    attend(att, ROUTE_AT)
    attend(att, per_seg - ROUTE_AT, steps)
    _run(steps)
    wind_down(att, project_segment(3))
    _run(other[0])
    att, steps = attention(range(1, NSEG)), ffn_down()
    attend(att, per_seg, steps)
    _run(steps)
    outs = (n for s in range(NSEG - 1) for n in out_proj(s))
    attend(att, 2 * per_seg, dense=outs, rows=((NSEG - 1) * NP * 9 - TAIL) * G)
    wind_down(att, outs)
    _run(out_proj(NSEG - 1))
    assert not deferred and not arrivals
    for cs in o_cp:
        for c in cs:
            c.wait()


@jax.jit
def pallas_parallel_sum__memory_aug_infini_attn__moe_arch_mod__prompt_kernel(
    A_x: jax.Array,
    A_wq: jax.Array,
    A_wk: jax.Array,
    A_wv: jax.Array,
    A_wo: jax.Array,
    A_beta: jax.Array,
    B_x: jax.Array,
    B_w_r: jax.Array,
    B_w_gate: jax.Array,
    B_w_up: jax.Array,
    B_w_down: jax.Array,
):
    del B_x
    hbm = pl.BlockSpec(memory_space=pltpu.HBM)
    out = pl.pallas_call(
        _kernel,
        out_shape=jax.ShapeDtypeStruct((D, S), A_x.dtype),
        in_specs=[hbm] * 10,
        out_specs=hbm,
        scratch_shapes=[
            pltpu.VMEM((D, S), bf16),
            pltpu.VMEM((4, D, D), bf16),
            pltpu.VMEM((1, H), bf16),
            pltpu.VMEM((D,), bf16),
            pltpu.VMEM((D, F), bf16),
            pltpu.VMEM((D, F), bf16),
            pltpu.VMEM((D, F), bf16),
            pltpu.VMEM((4, D, DP), f32),
            pltpu.VMEM((D, T), f32),
            pltpu.VMEM((S // T, DP // 2, T), u32),
            pltpu.VMEM((NSEG, 5, HK // 2, HK), u32),
            pltpu.VMEM((NSEG, H, 16, L), u32),
            pltpu.VMEM((NSEG, H, 24, L), f32),
            pltpu.VMEM((NSEG, NG, L // 2, T), u32),
            pltpu.VMEM((NSEG, D, L), f32),
            pltpu.VMEM((NG, G, T), f32),
            pltpu.VMEM((NG, G, T), f32),
            pltpu.VMEM((D, T), f32),
            pltpu.VMEM((S // T, T), f32),
            pltpu.VMEM((8, S), f32),
            pltpu.VMEM((NSEG, D, L), bf16),
            pltpu.VMEM((4, T, T), f32),
            pltpu.VMEM((len(QUARTERS), 8, T), u32),
            pltpu.SemaphoreType.DMA((8 + len(XPARTS),)),
        ],
        compiler_params=pltpu.CompilerParams(vmem_limit_bytes=100 * 2**20),
    )(A_x.reshape(S, D).T, A_wq, A_wk, A_wv, A_wo, A_beta.reshape(1, H), B_w_r,
      B_w_gate, B_w_up, B_w_down.T)
    return out.T.reshape(A_x.shape)
```

```python
import functools

import jax
import jax.numpy as jnp
import jax.experimental.pallas as pl
import jax.experimental.pallas.tpu as pltpu

S, D, H, DH, NSEG, L, F = 2048, 576, 32, 18, 4, 512, 4608
T = 128
HK = 2 * T
DP = 640
G = 4 * DH
NG = H // 4
NP = NG // 2
NT = L // T
QSCALE = DH ** -0.5 * 1.4426950408889634
NEG = -1e30
ONES_ROW = (23, 23, 0, 0)
ROT = (32, 64, 96, 0)
QUARTERS = (0b0001, 0b0010, 0b0100, 0b1000, 0b1101, 0b1011, 0b0111,
            0b1001, 0b0110, 0b0011, 0b1100)
XPARTS = ((0, 128), (128, 384), (512, 512), (1024, 1024))

ORDER = ((3, 2), (3, 3), (3, 0), (2, 1), (2, 2), (3, 1), (0, 0), (2, 0), (1, 0), (1, 1))
LAG = 2
WAIT_Q, WAIT_K, WAIT_V = (0, 0, 0, 9), (0, 0, 3, 4), (1, 0, 3, 4)
WAIT_O, WAIT_F, WO_READY = (0, 1, 0, 4), (0, 3, 1, 0), (0, 2, 1, 2)
FILL_FIRST = ((0, 1, 2, 3, 4, 7, 8, 9), (5, 8), range(9))
FILL_WO = ((), (7,), (1, 7))
LN_ROWS = ((144, 144, 144, 64), (576, 288, 96, 128), (192, 96, 48, 32))
LATE, DEFER, SOON = 2, 4, 9
ROUTE_AT, ROUTE_WAIT, TAIL = 30, 5, 27

f32, bf16, u32 = jnp.float32, jnp.bfloat16, jnp.uint32


def _dot(a, b):
    return jnp.dot(a, b, preferred_element_type=f32)


def _dot_nt(a, b):
    return jax.lax.dot_general(a, b, (((1,), (1,)), ((), ())), preferred_element_type=f32)


def _rnd(a):
    return a.astype(bf16).astype(f32)


def _rcp(a):
    return pltpu.reciprocal(a, full_range=False)


def _iota(shape, axis):
    return jax.lax.broadcasted_iota(jnp.int32, shape, axis)


def _pad_to_tile(a):
    if a.shape[1] < T:
        a = jnp.concatenate([a, jnp.zeros((a.shape[0], T - a.shape[1]), a.dtype)], axis=1)
    if a.shape[0] < T:
        a = jnp.concatenate([a, jnp.zeros((T - a.shape[0], T), a.dtype)], axis=0)
    return a


def _roll(a, shift):
    return pltpu.roll(a, shift % T, 1) if shift % T else a


def _phi(t):
    return jnp.where(t > 0, t + 1.0, jnp.exp(t))


def _head_of(i):
    return ((i >= DH).astype(jnp.int32) + (i >= 2 * DH).astype(jnp.int32)
            + (i >= 3 * DH).astype(jnp.int32) + (i >= 4 * DH).astype(jnp.int32))


class _Packed:
    def __init__(self, ref):
        self.words = ref

    def _index(self, idx):
        *lead, rows, cols = idx
        start, stop, _ = rows.indices(2 * self.words.shape[-2])
        return (*lead, slice(start // 2, stop // 2), cols)

    def __getitem__(self, idx):
        return pltpu.bitcast(self.words[self._index(idx)], bf16)

    def __setitem__(self, idx, value):
        self.words[self._index(idx)] = pltpu.bitcast(value, u32)


def _run(steps):
    for _ in steps:
        pass


def _kernel(x_hbm, wq_hbm, wk_hbm, wv_hbm, wo_hbm, beta_hbm, wr_hbm, wg_hbm, wu_hbm,
            wd_hbm, o_hbm,
            x_v, w_v, beta_v, wr_v, wg_v, wu_v, wd_v, wt, wrc, xn_v, bsum, qm, vl, kn, ot,
            mst, zst, gcol, r_v, hot, o_v, causal, lanes, sem):
    xn_v, bsum, qm, kn = (_Packed(r) for r in (xn_v, bsum, qm, kn))
    copy = pltpu.make_async_copy
    wq_cp = [copy(wq_hbm.at[:, pl.ds(c, n)], w_v.at[0, :, pl.ds(c, n)], sem.at[i])
             for c, n, i in ((0, 2 * T, 0), (2 * T, D - 2 * T, 7 + len(XPARTS)))]
    wk_cp, wv_cp, wo_cp = (copy(w, w_v.at[i], sem.at[i])
                           for i, w in ((1, wk_hbm), (2, wv_hbm), (3, wo_hbm)))
    f_cp = [copy(a, b, sem.at[4]) for a, b in ((wg_hbm, wg_v), (wu_hbm, wu_v), (wd_hbm, wd_v))]
    c_cp = [copy(a, b, sem.at[5]) for a, b in ((wr_hbm, wr_v), (beta_hbm, beta_v))]
    o_cp = [[copy(o_v.at[s, pl.ds(p * 2 * G, 2 * G)],
                  o_hbm.at[pl.ds(p * 2 * G, 2 * G), pl.ds(s * L, L)], sem.at[6])
             for p in range(NP)] for s in range(NSEG)]
    x_cp = [copy(x_hbm.at[:, pl.ds(t, n)], x_v.at[:, pl.ds(t, n)], sem.at[7 + i])
            for i, (t, n) in enumerate(XPARTS)]

    lane8 = _iota((8, T), 1)
    never = lane8 < jnp.min(lane8, axis=1, keepdims=True)
    zero = jnp.min(lane8)
    fillers = []
    link = [None, None]

    def tie(a, b):
        return a if b is None else jnp.where(never, b, a)

    def fill(after=None):
        link[0], link[1] = after, None
        while fillers:
            if next(fillers[0], False):
                break
            fillers.pop(0)
        return link[1]

    def drain():
        while fillers:
            fill()

    def gate_column():
        gate = jax.nn.sigmoid(beta_v[...].astype(f32))
        gate = jnp.concatenate([gate, jnp.zeros((1, T - H), f32)], axis=1)
        gate = jnp.broadcast_to(gate, (T, T)).T
        r8 = _iota((8, T), 0)
        for v in range(D // 8):
            h0, h1 = (8 * v) // DH, (8 * v + 7) // DH
            gv = jnp.broadcast_to(gate[h0:h0 + 1], (8, T))
            if h1 != h0:
                gv = jnp.where(r8 < h1 * DH - 8 * v, gv, jnp.broadcast_to(gate[h1:h1 + 1], (8, T)))
            gcol[8 * v:8 * v + 8, :] = gv

    def router_column():
        wr = wr_v[...].astype(f32).reshape(1, D)
        wr = jnp.concatenate([wr, jnp.zeros((1, DP - D), f32)], axis=1)
        wrc[...] = jnp.broadcast_to(wr, (T, DP)).T[0:D]

    def transpose_w(i, lo=0, hi=D):
        for c in range(lo, hi, T):
            n = min(T, D - c)
            for k in range(0, D, T):
                w = _pad_to_tile(w_v[i, k:min(k + T, D), c:c + n].astype(f32))
                w = jnp.concatenate([tie(w[r:r + 8], link[0]) for r in range(0, T, 8)], axis=0).T
                wt[i, c:c + n, k:k + T] = w[0:n]
                yield True

    def layernorm(b, steps):
        def total(acc, v):
            h = v.shape[0] // 16 * 8
            a, c = v[0:8], v[h:h + 8]
            for k in range(8, h, 8):
                a, c = a + v[k:k + 8], c + v[h + k:h + k + 8]
            return a + c if acc is None else acc + (a + c)

        def rows(v):
            return jnp.concatenate([tie(v, link[0])] * (step // 8), axis=0)

        def bcast(v):
            return jnp.broadcast_to(v, (8, T))

        def load(r, n):
            return x_v[r:r + step, pl.ds(pl.multiple_of((b + n * zero) * T, T), T)].astype(f32)

        acc, step = jnp.zeros((8, T), f32), steps[0]
        for r in range(0, D, step):
            x = load(r, 0)
            link[1] = acc = total(tie(acc, link[0]), x)
            yield True
        mean = bcast(jnp.sum(acc, axis=0, keepdims=True) * (1.0 / D))
        acc, step = None, steps[1]
        for r in range(0, D, step):
            xc = load(r, 1) - rows(mean)
            link[1] = acc = total(acc, xc * xc)
            yield True
        var = bcast(jnp.sum(acc, axis=0, keepdims=True) * (1.0 / D))
        sd = _rnd(jnp.sqrt(_rnd(_rnd(var) + _rnd(jnp.full((8, T), 1e-5, f32)))))
        step = steps[2]
        inv, mean = jnp.concatenate([1.0 / sd] * (step // 8), axis=0), _rnd(mean)
        acc = None
        for r in range(0, D, step):
            x = load(r, 2)
            xn = (_rnd(x - rows(mean)) * inv).astype(bf16)
            xn_v[b, r:r + step, :] = xn
            link[1] = acc = total(acc, xn.astype(f32) * wrc[r:r + step, :])
            if r + step == D:
                xn_v[b, D:DP, :] = jnp.zeros((DP - D, T), bf16)
                r_v[b:b + 1, :] = _rnd(jnp.sum(acc, axis=0, keepdims=True))
            yield True

    prepared = [0]

    def block_sums(s, rows):
        for c in range(NT // 2):
            for r in range(0, HK, rows):
                b11, b12, b21, b22 = (
                    xn_v[s * NT + c + n + zero, k + r:k + r + rows, :].astype(f32)
                    for k in (0, HK) for n in (0, NT // 2))
                b11 = jnp.concatenate(
                    [tie(b11[k:k + 8], link[0]) for k in range(0, rows, 8)], axis=0)
                for n, t in enumerate((b11 + b22, b12 - b22, b21 - b11, b11 + b12, b21 + b22)):
                    bsum[s, n, r:r + rows, c * T:(c + 1) * T] = t.astype(bf16)
                    link[1] = tie(t[-8:], link[1])
                prepared[0] += c == NT // 2 - 1 and r + rows == HK
                yield True

    def strassen(i, p, part, sums, rest, step, top, bottom):
        r0, r1 = slice(2 * p * G, (2 * p + 1) * G), slice((2 * p + 1) * G, (2 * p + 2) * G)
        a11, a12 = (lambda: wt[i, r0, 0:HK]), (lambda: wt[i, r0, HK:2 * HK])
        a21, a22 = (lambda: wt[i, r1, 0:HK]), (lambda: wt[i, r1, HK:2 * HK])
        c11 = yield from step(0, a12() - a22(), sums(4))
        m = yield from step(1, a11() + a12(), part(1))
        c11, c12 = c11 - m, m
        m = yield from step(2, wt[i, r0, 2 * HK:DP], rest())
        c11, c12 = c11 + m[:, :HK], c12 + m[:, HK:]
        m = yield from step(3, a11() + a22(), sums(0))
        c11, c22 = c11 + m, m
        m = yield from step(4, a11(), sums(1))
        c12, c22 = c12 + m, c22 + m
        c21 = yield from step(5, a22(), sums(2))
        top(jnp.concatenate([c11 + c21, c12], axis=1))
        m = yield from step(6, a21() + a22(), part(0))
        c21, c22 = c21 + m, c22 - m
        c22 = c22 + (yield from step(7, a21() - a11(), sums(3)))
        m = yield from step(8, wt[i, r1, 2 * HK:DP], rest())
        bottom(jnp.concatenate([c21, c22], axis=1) + m)

    late = [None] * LATE
    soon = []
    deferred = []
    arrivals = {}
    other = []

    def project(i, s, p, slots, finish):
        def block(k, n, cs):
            return jnp.concatenate([xn_v[s * NT + c, k:k + n, :] for c in cs], axis=1)

        def step(n, w, xs):
            if (i, s, p, n) == WO_READY:
                done = wt[zero, pl.ds(pl.multiple_of(zero * 8, 8), 8),
                          pl.ds(pl.multiple_of(zero * T, T), T)]
                w = jnp.concatenate([w[:-8], tie(w[-8:], done)], axis=0)
            if (i, s, p, n) in arrivals:
                arrivals.pop((i, s, p, n))()
            d = _dot(w, xs)
            top = tie(d[-8:, :T], late.pop(0))
            for job in soon:
                job[0] -= 1
                if job[0] == -1:
                    top = tie(top, job[1])
            d = jnp.concatenate([d[:-8], jnp.concatenate([top, d[-8:, T:]], axis=1)], axis=0)
            late.append(fill(d[0:8, 0:T]) if n in slots else None)
            if other and (s == NSEG - 1 or n in FILL_WO[i]):
                next(other[0], None)
            for job in deferred:
                job[0] -= 1
            while deferred and deferred[0][0] < 0:
                deferred.pop(0)[1]()
            yield G
            return d

        if (i, s, p) == (0, 0, 0):
            for e in range(2):
                acc = None
                for n, k in enumerate(range(0, DP, T)):
                    d = yield from step(5 * e + n, wt[i, e * G:(e + 1) * G, k:k + T],
                                        block(k, T, range(NT)))
                    acc = d if acc is None else acc + d
                finish(s, e, acc)
            drain()
            return
        yield from strassen(
            i, p, lambda k: block(k * HK, HK, (2 * k, 2 * k + 1)),
            lambda n: bsum[s, n, :, :], lambda: block(2 * HK, T, range(NT)), step,
            functools.partial(finish, s, 2 * p), functools.partial(finish, s, 2 * p + 1))

    def finish_q(s, g, q):
        r8 = _iota((8, L), 0)
        qs = q * QSCALE
        for h in range(4):
            lo = 16 * h
            a0, a1, a2 = qs[lo:lo + 8], qs[lo + 8:lo + 16], qs[lo + 16:lo + 24]
            if h > 0:
                a0 = jnp.where(r8 >= 2 * h, a0, 0.0)
            if h < 3:
                a2 = jnp.where(r8 < 2 * h + 2, a2, 0.0)
            w = pltpu.bitcast(jnp.concatenate(
                [a0, a1, a2, jnp.zeros((8, L), f32)], axis=0).astype(bf16), u32)
            for c in range(0, L, T):
                qm.words[s, 4 * g + h, :, c:c + T] = _roll(w[:, c:c + T], ROT[h])
        if s > 0:
            deferred.append([DEFER, functools.partial(memory_read, s, g, _phi(q))])

    def memory_read(s, g, pq):
        r8 = _iota((8, L), 0)
        same_head = _head_of(_iota((G, T), 0)) == _head_of(_iota((G, T), 1))
        num = _dot(jnp.where(same_head, mst[g], 0.0),
                   jnp.concatenate([pq, jnp.zeros((T - G, L), f32)], axis=0).astype(bf16))
        t = pq * jnp.concatenate([zst[g]] * NT, axis=1)
        t = [t[r:r + 8] for r in range(0, G, 8)]
        ib = []
        for h in range(4):
            a, b, c = t[2 * h:2 * h + 3]
            if h > 0:
                a = jnp.where(r8 >= 2 * h, a, 0.0)
            if h < 3:
                c = jnp.where(r8 < 2 * h + 2, c, 0.0)
            den = jnp.sum(a + b + c, axis=0, keepdims=True)
            ib.append(_rcp(jnp.broadcast_to(den, (8, L)) + 1e-6))
        iv = jnp.concatenate(
            [ib[0], ib[0], jnp.where(r8 < 2, ib[0], ib[1]), ib[1],
             jnp.where(r8 < 4, ib[1], ib[2]), ib[2],
             jnp.where(r8 < 6, ib[2], ib[3]), ib[3], ib[3]], axis=0)
        gg = gcol[g * G:(g + 1) * G, :]
        res = num * iv * jnp.concatenate([gg] * NT, axis=1)
        ot[s, g * G:(g + 1) * G, :] = res
        t = None
        for c in range(0, L, T):
            for r in (0, 24, 40, 64):
                t = tie(res[r:r + 8, c:c + T], t)
        soon.append([SOON, t])

    def memory_update(s, g, v, pk, z):
        upd = _dot_nt(v, pk)
        mst[g] = upd if s == 0 else mst[g] + upd
        zst[g] = z if s == 0 else zst[g] + z

    keys = {}

    def finish_k(s, g, k):
        zpad = jnp.zeros((T - G, L), f32)
        kt = jnp.concatenate([k, zpad], axis=0).astype(bf16).T
        kn[s, g, :, :] = kt
        soon.append([SOON, pltpu.bitcast(kt[-16:], f32)])
        if s < NSEG - 1:
            pk = _phi(k)
            z = sum(pk[:, c:c + T] for c in range(T, L, T)) + pk[:, :T]
            z = jnp.broadcast_to(jnp.sum(z, axis=1, keepdims=True), (G, T))
            keys[g] = jnp.concatenate([pk, zpad], axis=0).astype(bf16), z

    def finish_v(s, g, v):
        for h in range(4):
            a = [v[16 * h + c:16 * h + c + 8] for c in (0, 8, 16)]
            c, r = divmod(ONES_ROW[h], 8)
            a[c] = jnp.where(_iota((8, L), 0) == r, 1.0, a[c])
            vl[s, 4 * g + h] = jnp.concatenate(a, axis=0)
        if s < NSEG - 1:
            deferred.append([DEFER, functools.partial(memory_update, s, g, v, *keys.pop(g))])

    attended = [0] * NSEG

    def attention(segs):
        r8 = _iota((8, T), 0)
        lane32 = _iota((32, T), 1)
        units = [(s, g, i, j) for s in segs for g in range(NG) for i, j in ORDER]
        maxes, accs, carry = {}, {}, {}

        def own_queries(s, g, i):
            w = []
            for h in range(4):
                parts = [qm[s, 4 * g + h, :, i * T:(i + 1) * T]]
                if h > 0:
                    parts.insert(0, jnp.zeros((16 * h, T), bf16))
                parts.append(jnp.zeros((T - 32 - 16 * h, T), bf16))
                w.append(jnp.concatenate(parts, axis=0))
            return jnp.concatenate(w, axis=1)

        def shared_queries(qw, *parts):
            slots = [None] * 8
            for h, quarters in parts:
                for e in range(2):
                    t = qw[h][8 * e:8 * e + 8] & lanes[QUARTERS.index(quarters)]
                    slots[h + e] = t if slots[h + e] is None else t | slots[h + e]
            slots = [jnp.zeros((8, T), u32) if t is None else t for t in slots]
            return pltpu.bitcast(jnp.concatenate(slots, axis=0), bf16)

        def diagonal_scores(s, g, i):
            k0 = i * T
            own = carry.pop("own") if i else _dot(kn[s, g, 0:32, :], own_queries(s, g, 0))
            qw = [qm.words[s, 4 * g + h, :, k0:k0 + T] for h in range(4)]
            x = _dot(kn[s, g, k0 + 32:k0 + 64, :], jnp.concatenate(
                [shared_queries(qw, (h, 15 - (2 << h)), (3, 2 << h)) for h in range(3)], axis=1))
            y = _dot(kn[s, g, k0 + 64:k0 + 96, :], jnp.concatenate(
                [shared_queries(qw, (0, 0b1001), (2, 0b0110)),
                 shared_queries(qw, (1, 0b0011), (3, 0b1100))], axis=1))
            z = _dot(kn[s, g, k0 + 96:k0 + T, :],
                     shared_queries(qw, *[(h, 1 << h) for h in range(4)]))
            xs = [x[:, h * T:(h + 1) * T] for h in range(3)]
            xs.append(jnp.where(lane32 < 64, xs[0], jnp.where(lane32 < 96, xs[1], xs[2])))
            ys = [y[:, :T], y[:, T:]] * 2
            return [jnp.concatenate([own[:, h * T:(h + 1) * T], xs[h], ys[h], z], axis=0)
                    for h in range(4)]

        def scores(s, g, i, j):
            if i == j:
                shs = diagonal_scores(s, g, i)
            else:
                more = 32 if j == i - 1 else 0
                st = _dot(kn[s, g, j * T:(j + 1) * T + more, :], own_queries(s, g, i))
                if more:
                    carry["own"] = st[T:]
                shs = [st[:T, h * T:(h + 1) * T] for h in range(4)]
            ps, alphas = [], []
            later = any(a == i for a, _ in ORDER[:ORDER.index((i, j))])
            for h in range(4):
                sh = shs[h]
                if i == j:
                    sh = sh + causal[h]
                m = jnp.max(sh, axis=0, keepdims=True)
                if later:
                    m = jnp.maximum(m, maxes[i, h])
                    alphas.append(jnp.exp2(maxes[i, h] - m))
                maxes[i, h] = m
                ps.append(jnp.exp2(sh - m).astype(bf16))
            return ps, alphas

        def values(s, g, i, j, ps, alphas):
            new = [_dot(vl[s, 4 * g + h, :, j * T:(j + 1) * T], ps[h]) for h in range(4)]
            if alphas:
                new = [a * al + b for a, al, b in zip(accs.pop(i), alphas, new)]
            if any(a == i for a, _ in ORDER[ORDER.index((i, j)) + 1:]):
                accs[i] = new
                return
            o = []
            for h in range(4):
                inv = _rcp(jnp.broadcast_to(new[h][ONES_ROW[h]:ONES_ROW[h] + 1], (8, T)))
                o.append([_roll(new[h][8 * c:8 * c + 8] * inv, -ROT[h]) for c in range(3)])
            a_dot = jnp.concatenate(
                [o[0][0], o[0][1], jnp.where(r8 < 2, o[0][2], o[1][0]), o[1][1],
                 jnp.where(r8 < 4, o[1][2], o[2][0]), o[2][1],
                 jnp.where(r8 < 6, o[2][2], o[3][0]), o[3][1], o[3][2]], axis=0)
            dst = (s, slice(g * G, (g + 1) * G), slice(i * T, (i + 1) * T))
            mix = (1.0 - gcol[g * G:(g + 1) * G, :]) * a_dot
            ot[dst] = ot[dst] + mix if s > 0 else mix
            attended[s] += 1

        pend = {}
        for t in range(len(units) + LAG):
            if t < len(units):
                pend[t] = scores(*units[t])
            if t >= LAG:
                values(*units[t - LAG], *pend.pop(t - LAG))
            yield t < len(units) and units[t][2] != units[t][3]

    def out_proj(s):
        assert attended[s] == NG * NT
        b11, b12, b21, b22 = (ot[s, k:k + HK, n:n + HK] for k in (0, HK) for n in (0, HK))
        sums = [t.astype(bf16) for t in (b11 + b22, b12 - b22, b21 - b11, b11 + b12, b21 + b22)]
        parts = [b11.astype(bf16), b22.astype(bf16)]
        rest = jnp.concatenate([ot[s, 2 * HK:D, :], hot[:, s * L:(s + 1) * L],
                                jnp.zeros((DP - D - 8, L), f32)], axis=0).astype(bf16)

        def step(n, w, o):
            d = _dot(w, o)
            if n % 3 == 2:
                yield 3 * G
            return d

        for p in range(NP):
            halves = []
            yield from strassen(3, p, parts.__getitem__, sums.__getitem__, lambda: rest,
                                step, halves.append, halves.append)
            a = jnp.concatenate(halves, axis=0)
            rows = slice(p * 2 * G, (p + 1) * 2 * G)
            for c in range(NT):
                b = s * NT + c
                res = x_v[rows, b * T:(b + 1) * T].astype(f32) + xn_v[b, rows, :].astype(f32)
                o_v[s, rows, c * T:(c + 1) * T] = (res + a[:, c * T:(c + 1) * T]).astype(bf16)
            o_cp[s][p].start()

    routed = {}

    def route():
        def both(op, a):
            return op(op(a, axis=0, keepdims=True), axis=1, keepdims=True)

        r = r_v[...]
        idx = (_iota(r.shape, 0) * T + _iota(r.shape, 1)).astype(f32)
        m1 = both(jnp.max, r)
        i1 = both(jnp.min, jnp.where(r == m1, idx, S))
        r = jnp.where(idx == i1, -jnp.inf, r)
        m2 = both(jnp.max, r)
        i2 = both(jnp.min, jnp.where((r == m2) & (idx != i1), idx, S))
        row = _iota((8, T), 0)
        routed["w"] = jnp.where(row < 2, jax.nn.sigmoid(jnp.where(row == 0, m1, m2)), 0.0)
        pick = jnp.where(row == 0, i1, jnp.where(row == 1, i2, -1.0))
        for b in range(S // T):
            hot[:, b * T:(b + 1) * T] = (pick == (lane8 + b * T).astype(f32)).astype(f32)
        for _ in range(ROUTE_WAIT):
            yield
        blocks = [jnp.broadcast_to(i.astype(jnp.int32) >> 7, (32, T)) for i in (i1, i2)]
        tiles = [[], []]
        for r0 in range(0, DP // 2, 32):
            acc = [xn_v.words[0, r0:r0 + 32, :]] * 2
            for b in range(1, S // T):
                w = xn_v.words[b, r0:r0 + 32, :]
                acc = [jnp.where(blocks[n] == b, w, acc[n]) for n in range(2)]
            for n in range(2):
                tiles[n].append(acc[n])
            if r0 % 64:
                yield
        x = None
        for n, i in enumerate((i1, i2)):
            pick = (row == n) & (lane8 == (i.astype(jnp.int32) & (T - 1)))
            d = _dot_nt(pick.astype(f32), pltpu.bitcast(jnp.concatenate(tiles[n], axis=0), bf16))
            x = d if x is None else x + d
        routed["x"] = [x[:, k:k + T] for k in range(0, DP, T)]

    def ffn_hidden():
        routed["h"] = []
        tail = routed["x"][D // T]
        tail = tail + pltpu.roll(_roll(tail, 64), 2, 0)
        for n in range(0, F, L):
            gu = []
            for w_ref in (wg_v, wu_v):
                acc = None
                for c in range(D // T):
                    d = _dot(routed["x"][c], w_ref[c * T:(c + 1) * T, n:n + L])
                    acc = d if acc is None else acc + d
                    yield
                gu.append(acc)
            d = _dot(tail, jnp.concatenate(
                [w_ref[D // T * T:D, n:n + L] for w_ref in (wg_v, wu_v)], axis=0))
            yield
            gt, up = gu[0] + d, gu[1] + pltpu.roll(d, 6, 0)
            routed["h"].append(gt * jax.nn.sigmoid(gt) * up)

    def ffn_down():
        for k in range(0, D, T):
            acc = None
            for c, n in enumerate(range(0, F, L)):
                w = wd_v[k:min(k + T, D), n:n + L]
                if k + T > D:
                    w = jnp.concatenate([w, jnp.zeros((DP - D, L), bf16)], axis=0)
                d = _dot_nt(routed["h"][c], w)
                acc = d if acc is None else acc + d
                yield
            y = jnp.concatenate([jnp.zeros((D - 4 * T, T), f32), acc * routed["w"],
                                 jnp.zeros((DP - D - 8, T), f32)], axis=0).T
            dst = (3, slice(k, min(k + T, D)), slice(4 * T, DP))
            wt[dst] = wt[dst] + y[0:min(T, D - k)]

    for c in (*c_cp, *x_cp[:2], *wq_cp, wk_cp, wv_cp):
        c.start()
    for h in range(4):
        query = (_iota((T, T), 1) - ROT[h]) & (T - 1)
        causal[h] = jnp.where(_iota((T, T), 0) <= query, 0.0, NEG)
    for n, quarters in enumerate(QUARTERS):
        lanes[n] = pltpu.bitcast(-((quarters >> (lane8 >> 5)) & 1), u32)
    for c in c_cp:
        c.wait()
    router_column()
    gate_column()
    for b in range(NT):
        if b < 2:
            x_cp[b].wait()
        fillers.append(layernorm(b, LN_ROWS[0]))
        prev = [None, None]
        while fillers:
            prev.append(fill(prev.pop(0)))
    x_cp[2].start()
    wq_cp[0].wait()
    fillers.append(transpose_w(0, 0, 2 * T))
    drain()

    def prepare(s, rows):
        fillers.extend(layernorm(b, rows) for b in range(s * NT, (s + 1) * NT))
        fillers.append(block_sums(s, rows[3]))

    def wq_arrives():
        wq_cp[1].wait()
        _run(transpose_w(0, 2 * T))

    def wk_arrives():
        wk_cp.wait()
        _run(transpose_w(1))

    def wv_arrives():
        void = kn[0, 0, 0:16, :]
        x_v[0:16, S - T:S] = void
        w_v[3, 0:16, 0:T] = void
        for ref in (wg_v, wu_v, wd_v):
            ref[0:16, 0:T] = void
        for c in (x_cp[3], wo_cp, *f_cp):
            c.start()
        for c in (wv_cp, x_cp[2]):
            c.wait()
        _run(transpose_w(2))
        prepare(1, LN_ROWS[1])

    def wo_arrives():
        for c in (x_cp[3], wo_cp):
            c.wait()
        prepare(2, LN_ROWS[2])
        prepare(3, LN_ROWS[2])
        other.append(transpose_w(3))

    def ffn_arrives():
        for c in f_cp:
            c.wait()
        _run(other.pop())
        other.append(ffn_hidden())

    arrivals.update({WAIT_Q: wq_arrives, WAIT_K: wk_arrives, WAIT_V: wv_arrives,
                     WAIT_O: wo_arrives, WAIT_F: ffn_arrives})
    finishers = tuple(enumerate((finish_q, finish_k, finish_v)))
    fillers.append(block_sums(0, LN_ROWS[0][3]))
    for i, finish in finishers:
        for p in range(NP):
            _run(project(i, 0, p, FILL_FIRST[i], finish))

    def project_segment(s):
        while prepared[0] <= s:
            assert fillers
            fill()
        for p in range(NP):
            for i, finish in finishers:
                yield from project(i, s, p, range(9), finish)

    def attend(att, steps, extra=iter(()), dense=iter(()), rows=0):
        done = 0
        for t in range(steps):
            if next(att):
                next(extra, None)
            while done < (t + 1) * rows // steps:
                done += next(dense)

    def wind_down(att, dense):
        for _ in range(LAG):
            done = 0
            while done < 4 * G:
                done += next(dense)
            next(att)
        _run(att)
        _run(dense)

    per_seg = NG * len(ORDER)
    _run(project_segment(1))
    _run(project_segment(2))
    drain()
    att, steps = attention([0]), route()
    attend(att, ROUTE_AT)
    attend(att, per_seg - ROUTE_AT, steps)
    _run(steps)
    wind_down(att, project_segment(3))
    _run(other[0])
    att, steps = attention(range(1, NSEG)), ffn_down()
    attend(att, per_seg, steps)
    _run(steps)
    outs = (n for s in range(NSEG - 1) for n in out_proj(s))
    attend(att, 2 * per_seg, dense=outs, rows=((NSEG - 1) * NP * 9 - TAIL) * G)
    wind_down(att, outs)
    _run(out_proj(NSEG - 1))
    assert not deferred and not arrivals
    for cs in o_cp:
        for c in cs:
            c.wait()


@jax.jit
def pallas_parallel_sum__memory_aug_infini_attn__moe_arch_mod__prompt_kernel(
    A_x: jax.Array,
    A_wq: jax.Array,
    A_wk: jax.Array,
    A_wv: jax.Array,
    A_wo: jax.Array,
    A_beta: jax.Array,
    B_x: jax.Array,
    B_w_r: jax.Array,
    B_w_gate: jax.Array,
    B_w_up: jax.Array,
    B_w_down: jax.Array,
):
    del B_x
    hbm = pl.BlockSpec(memory_space=pltpu.HBM)
    out = pl.pallas_call(
        _kernel,
        out_shape=jax.ShapeDtypeStruct((D, S), A_x.dtype),
        in_specs=[hbm] * 10,
        out_specs=hbm,
        scratch_shapes=[
            pltpu.VMEM((D, S), bf16),
            pltpu.VMEM((4, D, D), bf16),
            pltpu.VMEM((1, H), bf16),
            pltpu.VMEM((D,), bf16),
            pltpu.VMEM((D, F), bf16),
            pltpu.VMEM((D, F), bf16),
            pltpu.VMEM((D, F), bf16),
            pltpu.VMEM((4, D, DP), f32),
            pltpu.VMEM((D, T), f32),
            pltpu.VMEM((S // T, DP // 2, T), u32),
            pltpu.VMEM((NSEG, 5, HK // 2, HK), u32),
            pltpu.VMEM((NSEG, H, 16, L), u32),
            pltpu.VMEM((NSEG, H, 24, L), f32),
            pltpu.VMEM((NSEG, NG, L // 2, T), u32),
            pltpu.VMEM((NSEG, D, L), f32),
            pltpu.VMEM((NG, G, T), f32),
            pltpu.VMEM((NG, G, T), f32),
            pltpu.VMEM((D, T), f32),
            pltpu.VMEM((S // T, T), f32),
            pltpu.VMEM((8, S), f32),
            pltpu.VMEM((NSEG, D, L), bf16),
            pltpu.VMEM((4, T, T), f32),
            pltpu.VMEM((len(QUARTERS), 8, T), u32),
            pltpu.SemaphoreType.DMA((8 + len(XPARTS),)),
        ],
        compiler_params=pltpu.CompilerParams(vmem_limit_bytes=100 * 2**20),
    )(A_x.reshape(S, D).T, A_wq, A_wk, A_wv, A_wo, A_beta.reshape(1, H), B_w_r,
      B_w_gate, B_w_up, B_w_down.T)
    return out.T.reshape(A_x.shape)
```
